```python
import jax
import jax.numpy as jnp

def _softmax(x, axis=-1):
    return jax.nn.softmax(x, axis=axis)
def _gelu(x):
    return jax.nn.gelu(x, approximate=True)
def _silu(x):
    return jax.nn.silu(x)
def _sigmoid(x):
    return jax.nn.sigmoid(x)
def _layernorm(x, axis=-1, eps=1e-5):
    m = jnp.mean(x, axis=axis, keepdims=True)
    v = jnp.var(x, axis=axis, keepdims=True)
    return (x - m) / jnp.sqrt(v + eps)
def _scatter_add(tgt, idx, src, axis=0):
    return tgt.at[idx].add(src)
def _segment_sum(src, seg, n):
    return jax.ops.segment_sum(src, seg, n)
class _Rng:
    def __init__(self, key):
        self._k = key
    def _next(self):
        self._k, sub = jax.random.split(self._k)
        return sub
    def normal(self, shape):
        return jax.random.normal(self._next(), shape, dtype=jnp.bfloat16)
    def randint(self, lo, hi, shape):
        return jax.random.randint(self._next(), shape, lo, hi, dtype=jnp.int32)
    def uniform(self, shape, lo=0.0, hi=1.0):
        return jax.random.uniform(self._next(), shape, jnp.bfloat16, lo, hi)
    def permutation(self, n):
        return jax.random.permutation(self._next(), n)


kernel_name = 'sequential_preLN__compressed_kv_cla__moe_arch_mod__prompt'

def setup_inputs():
    _rng = _Rng(jax.random.key(int.from_bytes(__import__("os").urandom(4), "little")))
    _w = (lambda a: (lambda t: t.astype(jnp.bfloat16) if jnp.issubdtype(t.dtype, jnp.floating) else t)(jnp.asarray(a)))
    def _A_setup():
        B, H, Sq, Sk, D, M = 1, 32, 2048, 2048, 128, 1024
        Dc = 4 * D
        return {
            "x": _w((lambda *s: _rng.normal(s) * 0.05)(B, Sq, M)),
            "c_kv": _w((lambda *s: _rng.normal(s) * 0.05)(B, Sk, Dc)),
            "w_q": _w((lambda *s: _rng.normal(s) * 0.05)(M, H, D) * (M ** -0.5)),
            "w_uk": _w((lambda *s: _rng.normal(s) * 0.05)(Dc, H, D) * (Dc ** -0.5)),
            "w_uv": _w((lambda *s: _rng.normal(s) * 0.05)(Dc, H, D) * (Dc ** -0.5)),
            "w_o": _w((lambda *s: _rng.normal(s) * 0.05)(H, D, M) * ((H * D) ** -0.5)),
        }
    _A_in = _A_setup()

    def _B_setup():
        B, S, D, F, C = 1, 2048, 1024, 3584, 2
        return {
            "x": _w((lambda *s: _rng.normal(s) * 0.05)(B, S, D)),
            "w_r": _w((lambda *s: _rng.normal(s) * 0.05)(D)),
            "w_gate": _w((lambda *s: _rng.normal(s) * 0.05)(D, F)),
            "w_up": _w((lambda *s: _rng.normal(s) * 0.05)(D, F)),
            "w_down": _w((lambda *s: _rng.normal(s) * 0.05)(F, D)),
        }
    _B_in = _B_setup()

    return {
        "A_x": _A_in["x"],
        "A_c_kv": _A_in["c_kv"],
        "A_w_q": _A_in["w_q"],
        "A_w_uk": _A_in["w_uk"],
        "A_w_uv": _A_in["w_uv"],
        "A_w_o": _A_in["w_o"],
        "B_x": _B_in["x"],
        "B_w_r": _B_in["w_r"],
        "B_w_gate": _B_in["w_gate"],
        "B_w_up": _B_in["w_up"],
        "B_w_down": _B_in["w_down"],
    }

def reference(A_x, A_c_kv, A_w_q, A_w_uk, A_w_uv, A_w_o, B_x, B_w_r, B_w_gate, B_w_up, B_w_down):
    def _A_ref(x, c_kv, w_q, w_uk, w_uv, w_o):
        B, Sq, M = x.shape[0], x.shape[1], x.shape[2]
        Sk = c_kv.shape[1]
        H, D = w_q.shape[1], w_q.shape[2]
        q = jnp.einsum("bqm,mhd->bhqd", x, w_q)
        k = jnp.einsum("bkc,chd->bhkd", c_kv, w_uk)
        v = jnp.einsum("bkc,chd->bhkd", c_kv, w_uv)
        scores = jnp.einsum("bhqd,bhkd->bhqk", q, k) * (D ** -0.5)
        off = Sk - Sq
        qi = jnp.arange(Sq)[:, None]
        kj = jnp.arange(Sk)[None, :]
        cmask = kj <= (qi + off)
        scores = jnp.where(cmask[None, None], scores, -1e9)
        p = _softmax(scores, axis=-1)
        ctx = jnp.einsum("bhqk,bhkd->bhqd", p, v)
        return jnp.einsum("bhqd,hdm->bqm", ctx, w_o)

    def _B_ref(x, w_r, w_gate, w_up, w_down):
        B, S, D = x.shape
        C = 2
        r = x @ w_r
        idx = jnp.argsort(-r, axis=-1)[:, :C]
        idx_e = jnp.repeat(idx.reshape(B, C, 1), D, axis=2)
        x_sel = jnp.take_along_axis(x, idx_e, axis=1)
        g = _silu(x_sel @ w_gate)
        u = x_sel @ w_up
        y = (g * u) @ w_down
        r_sel = _sigmoid(jnp.take_along_axis(r, idx, axis=1))
        y = y * r_sel.reshape(B, C, 1)
        b_off = (jnp.arange(B) * S).reshape(B, 1)
        flat_idx = (idx + b_off).reshape(B * C)
        zero = (x * 0.0).reshape(B * S, D)
        upd = _scatter_add(zero, flat_idx, y.reshape(B * C, D), axis=0)
        return x + upd.reshape(B, S, D)

    x = A_x
    h = x + _A_ref(_layernorm(x, axis=-1), A_c_kv, A_w_q, A_w_uk, A_w_uv, A_w_o)
    h2 = h + _B_ref(_layernorm(h, axis=-1), B_w_r, B_w_gate, B_w_up, B_w_down)
    return h2
```

```python
import functools, math
import jax, jax.numpy as jnp
from jax import lax
from jax.experimental import pallas as pl
from jax.experimental.pallas import tpu as pltpu

S, M, H, D, DC, F = 2048, 1024, 32, 128, 512, 3584
EPS = 1e-5
bf16, f32, u32 = jnp.bfloat16, jnp.float32, jnp.uint32
NT = (((1,), (1,)), ((), ()))

def _rb(x):
    return x.astype(bf16).astype(f32)

def _ln_bf16(xf):
    mu = jnp.mean(xf, axis=-1, keepdims=True)
    var = jnp.mean(jnp.square(xf - mu), axis=-1, keepdims=True)
    d = _rb(xf - _rb(mu))
    sd = _rb(jnp.sqrt(_rb(_rb(var) + EPS)))
    return (d * (1.0 / sd)).astype(bf16)

def _unpack(w, shift):
    w = (w << shift) & jnp.uint32(0xFFFF0000)
    return pltpu.bitcast(w, f32).astype(bf16)

def default_sched(nb, lag=3):
    s = [("KP", 0), ("QP", 0), ("VP", 0)]
    outs = 0
    for t in range(nb):
        s.append(("QK", t))
        if t + 1 < nb:
            s += [("KP", t + 1), ("QP", t + 1), ("VP", t + 1)]
        else:
            while outs < nb - 2:
                s.append(("OUT", outs)); outs += 1
        s.append(("PV", t))
        if t - lag >= 0 and outs <= t - lag:
            s.append(("OUT", outs)); outs += 1
    while outs < nb:
        s.append(("OUT", outs)); outs += 1
    return s

def make(TQ=256, lag=3, diag=True, CH=128):
  nb = S // TQ
  sched = default_sched(nb, lag)
  NCH = S // CH
  def kernel(x_hbm, c_hbm, wq_hbm, wk_hbm, wv_hbm, wo_hbm, wr_ref, wg_hbm, wu_hbm, wd_hbm,
             o_hbm, x_ref, c_ref, xn_ref, acc_ref, hn_ref, o_ref, bq, bk, bv, bo, wg_ref, wu_ref, wd_ref,
             wsem, osem, xsem, csem, fsem, outsem):
    h = pl.program_id(0)
    pair = lax.shift_right_logical(h, 1)
    slot = pair & 1
    hslot = h & 1
    def wcopies(p, sl):
        return [pltpu.make_async_copy(w.bitcast(u32).at[:, p, :], b.at[sl], wsem.at[t, sl])
                for t, (w, b) in enumerate(((wk_hbm, bk), (wv_hbm, bv), (wq_hbm, bq)))]
    def ocopy(hh, sl):
        return pltpu.make_async_copy(wo_hbm.at[hh], bo.at[sl], osem.at[sl])
    def xcopy(i):
        return pltpu.make_async_copy(x_hbm.at[pl.ds(i * CH, CH)], x_ref.at[pl.ds(i * CH, CH)], xsem.at[i])
    ccopy = pltpu.make_async_copy(c_hbm, c_ref, csem)
    fcopies = [pltpu.make_async_copy(s_, d_, fsem.at[t]) for t, (s_, d_) in
               enumerate(((wg_hbm, wg_ref), (wu_hbm, wu_ref), (wd_hbm, wd_ref)))]
    def outcopy(i):
        return pltpu.make_async_copy(o_ref.at[pl.ds(i * CH, CH)], o_hbm.at[pl.ds(i * CH, CH)], outsem.at[i])

    @pl.when(h == 0)
    def _():
        for i in range(NCH): xcopy(i).start()
        for cp in wcopies(0, 0): cp.start()
        ccopy.start()
        ocopy(0, 0).start()
        def body(i, _):
            r = pl.multiple_of(i * CH, CH)
            xcopy(i).wait()
            xf = x_ref[pl.ds(r, CH), :].astype(f32)
            xn_ref[pl.ds(r, CH), :] = _ln_bf16(xf)
            acc_ref[pl.ds(r, CH), :] = jnp.zeros((CH, M), f32)
            return 0
        lax.fori_loop(0, NCH, body, 0)
        ccopy.wait()

    @pl.when(h == 1)
    def _():
        for cp in fcopies: cp.start()

    @pl.when(hslot == 0)
    def _():
        for cp in wcopies(pair, slot): cp.wait()
        @pl.when(pair + 1 < H // 2)
        def _():
            for cp in wcopies(pair + 1, 1 - slot): cp.start()
    ocopy(h, hslot).wait()
    @pl.when(h + 1 < H)
    def _():
        ocopy(h + 1, 1 - hslot).start()

    shift = (16 * (1 - hslot)).astype(u32)
    wk = _unpack(bk[slot], shift)
    wq = _unpack(bq[slot], shift)
    wv = _unpack(bv[slot], shift)
    wo = bo[hslot]
    qscale = (D ** -0.5) * math.log2(math.e)
    row = lax.broadcasted_iota(jnp.int32, (128, 128), 0)
    col = lax.broadcasted_iota(jnp.int32, (128, 128), 1)
    tri = col <= row
    ks, vs, qs, ps, ls, ctxs = {}, {}, {}, {}, {}, {}
    R = TQ // 128
    for op, i in sched:
        r0 = i * TQ
        if op == "KP":
            ks[i] = jnp.dot(c_ref[r0:r0 + TQ, :], wk, preferred_element_type=f32).astype(bf16)
        elif op == "VP":
            vs[i] = jnp.dot(c_ref[r0:r0 + TQ, :], wv, preferred_element_type=f32).astype(bf16)
        elif op == "QP":
            qs[i] = (jnp.dot(xn_ref[r0:r0 + TQ, :], wq, preferred_element_type=f32) * qscale).astype(bf16)
        elif op == "QK":
            kk = jnp.concatenate([ks[j] for j in range(i + 1)], axis=0)
            q = qs.pop(i)
            smain = lax.dot_general(q, kk[:r0 + 128], NT, preferred_element_type=f32)
            extra = [lax.dot_general(q[t * 128:], kk[r0 + t * 128:r0 + (t + 1) * 128], NT,
                                     preferred_element_type=f32) for t in range(1, R)]
            prow, lrow = [], []
            for a in range(R):
                pieces = [smain[a * 128:(a + 1) * 128]] + [extra[t - 1][(a - t) * 128:(a - t + 1) * 128] for t in range(1, a + 1)]
                sa = jnp.concatenate(pieces, axis=1) if len(pieces) > 1 else pieces[0]
                w = sa.shape[1]
                sd = jnp.where(tri, sa[:, w - 128:], -1e30)
                sa = jnp.concatenate([sa[:, :w - 128], sd], axis=1) if w > 128 else sd
                m = jnp.max(sa, axis=1, keepdims=True)
                p = jnp.exp2(sa - m)
                lrow.append(jnp.sum(p, axis=1, keepdims=True))
                prow.append(p.astype(bf16))
            ps[i] = prow
            ls[i] = jnp.concatenate(lrow, axis=0) if R > 1 else lrow[0]
        elif op == "PV":
            vv = jnp.concatenate([vs[j] for j in range(i + 1)], axis=0)
            prow = ps.pop(i)
            w0 = r0 + 128
            pm = jnp.concatenate([p[:, :w0] for p in prow], axis=0) if R > 1 else prow[0]
            ctx = jnp.dot(pm, vv[:w0], preferred_element_type=f32)
            if R > 1:
                parts = [ctx[0:128]]
                for a in range(1, R):
                    parts.append(ctx[a * 128:(a + 1) * 128] +
                                 jnp.dot(prow[a][:, w0:], vv[w0:w0 + a * 128], preferred_element_type=f32))
                ctx = jnp.concatenate(parts, axis=0)
            ctxs[i] = (ctx * (1.0 / ls.pop(i))).astype(bf16)
        elif op == "OUT":
            acc_ref[r0:r0 + TQ, :] += jnp.dot(ctxs.pop(i), wo, preferred_element_type=f32)

    @pl.when(h == H - 1)
    def _():
        wr = wr_ref[...].astype(f32)
        def body(i, carry):
            r0 = pl.multiple_of(i * CH, CH)
            xf = x_ref[pl.ds(r0, CH), :].astype(f32)
            hh = _rb(xf + _rb(acc_ref[pl.ds(r0, CH), :]))
            hn = _ln_bf16(hh).astype(f32)
            hn_ref[pl.ds(r0, CH), :] = hn
            acc_ref[pl.ds(r0, CH), :] = hh
            o_ref[pl.ds(r0, CH), :] = (hh + hn).astype(bf16)
            outcopy(i).start()
            r = _rb(jnp.sum(hn * wr, axis=1, keepdims=True))
            lane = lax.broadcasted_iota(jnp.int32, (CH, 128), 1)
            return jnp.where(lane == i, r, carry)
        rr = lax.fori_loop(0, NCH, body, jnp.full((CH, 128), -jnp.inf, f32))
        tok = (lax.broadcasted_iota(jnp.int32, (CH, 128), 1) * CH
               + lax.broadcasted_iota(jnp.int32, (CH, 128), 0))
        big = jnp.int32(1 << 30)
        m1 = jnp.max(rr)
        i1 = jnp.min(jnp.where(rr == m1, tok, big))
        rr2 = jnp.where(tok == i1, -jnp.inf, rr)
        m2 = jnp.max(rr2)
        i2 = jnp.min(jnp.where((rr2 == m2) & (tok != i1), tok, big))
        i1 = jnp.clip(i1, 0, S - 1)
        i2 = jnp.clip(i2, 0, S - 1)
        x1 = hn_ref[pl.ds(i1, 1), :]
        x2 = hn_ref[pl.ds(i2, 1), :]
        sub = lax.broadcasted_iota(jnp.int32, (16, M), 0)
        xs = jnp.where(sub == 0, x1, jnp.where(sub == 1, x2, 0.0)).astype(bf16)
        for cp in fcopies: cp.wait()
        g = _rb(jnp.dot(xs, wg_ref[...], preferred_element_type=f32))
        g = _rb(g * _rb(jax.nn.sigmoid(g)))
        u = _rb(jnp.dot(xs, wu_ref[...], preferred_element_type=f32))
        y = _rb(jnp.dot((g * u).astype(bf16), wd_ref[...], preferred_element_type=f32))
        sub1 = lax.broadcasted_iota(jnp.int32, (16, 1), 0)
        rs = jnp.where(sub1 == 0, m1, m2)
        y = _rb(y * _rb(jax.nn.sigmoid(rs)))
        for i in range(NCH): outcopy(i).wait()
        for j, idx in enumerate((i1, i2)):
            g0 = pl.multiple_of(idx & ~15, 16)
            hh = acc_ref[pl.ds(g0, 16), :]
            hn = hn_ref[pl.ds(g0, 16), :]
            new = _rb(hn + y[j:j + 1, :])
            hn = jnp.where(sub == idx - g0, new, hn)
            hn_ref[pl.ds(g0, 16), :] = hn
            o_ref[pl.ds(g0, 16), :] = (hh + hn).astype(bf16)
            cp = pltpu.make_async_copy(o_ref.at[pl.ds(g0, 16)], o_hbm.at[pl.ds(g0, 16)], outsem.at[0])
            cp.start(); cp.wait()

  @jax.jit
  def run(A_x, A_c_kv, A_w_q, A_w_uk, A_w_uv, A_w_o, B_x, B_w_r, B_w_gate, B_w_up, B_w_down):
    anyspec = pl.BlockSpec(memory_space=pl.ANY)
    V = pltpu.VMEM
    DMA = pltpu.SemaphoreType.DMA
    out = pl.pallas_call(
        kernel,
        grid=(H,),
        in_specs=[anyspec] * 6 + [pl.BlockSpec((1, M), lambda h: (0, 0))] + [anyspec] * 3,
        out_specs=anyspec,
        out_shape=jax.ShapeDtypeStruct((S, M), bf16),
        scratch_shapes=[V((S, M), bf16), V((S, DC), bf16), V((S, M), bf16), V((S, M), f32), V((S, M), f32), V((S, M), bf16),
                        V((2, M, D), u32), V((2, DC, D), u32), V((2, DC, D), u32), V((2, D, M), bf16),
                        V((M, F), bf16), V((M, F), bf16), V((F, M), bf16),
                        DMA((3, 2)), DMA((2,)), DMA((NCH,)), DMA(()), DMA((3,)), DMA((NCH,))],
        compiler_params=pltpu.CompilerParams(dimension_semantics=("arbitrary",),
                                             vmem_limit_bytes=120 * 1024 * 1024),
    )(A_x.reshape(S, M), A_c_kv.reshape(S, DC), A_w_q, A_w_uk, A_w_uv, A_w_o, B_w_r.reshape(1, M),
      B_w_gate, B_w_up, B_w_down)
    return out.reshape(1, S, M)
  return run


_run = make()


@jax.jit
def pallas_sequential_preLN__compressed_kv_cla__moe_arch_mod__prompt_kernel(
    A_x, A_c_kv, A_w_q, A_w_uk, A_w_uv, A_w_o, B_x, B_w_r, B_w_gate, B_w_up, B_w_down):
    return _run(A_x, A_c_kv, A_w_q, A_w_uk, A_w_uv, A_w_o, B_x, B_w_r, B_w_gate, B_w_up, B_w_down)
```

```python
import functools, math
import jax, jax.numpy as jnp
from jax import lax
from jax.experimental import pallas as pl
from jax.experimental.pallas import tpu as pltpu

S, M, H, D, DC, F = 2048, 1024, 32, 128, 512, 3584
EPS = 1e-5
bf16, f32, u32, i32 = jnp.bfloat16, jnp.float32, jnp.uint32, jnp.int32
NT = (((1,), (1,)), ((), ()))
G = 4
NP = H // 2
TQ = 256
NB = S // TQ
T2 = TQ // 2
FCH = 14
QSCALE = (D ** -0.5) * math.log2(math.e)
IMIN = jnp.iinfo(jnp.int32).min

def _rb(x):
    return x.astype(bf16).astype(f32)

def _inv_sd(mu, ss):
    dm = mu - _rb(mu)
    var = jnp.maximum(ss - dm * dm, 0.0)
    return 1.0 / _rb(jnp.sqrt(_rb(_rb(var) + EPS)))

def _gather(col):
    n = col.shape[0] // 8
    lane = lax.broadcasted_iota(i32, (8, 128), 1)
    out = jnp.broadcast_to(col[0:8], (8, 128))
    for g in range(1, n):
        out = jnp.where(lane == g, col[g * 8:(g + 1) * 8], out)
    return out

def _scatter(dense, n):
    return jnp.concatenate([jnp.broadcast_to(dense[:, g:g + 1], (8, 128)) for g in range(n)], axis=0)

def _ln_block(xf, wr=None):
    n = xf.shape[0] // 8
    s = jnp.sum(xf, axis=-1, keepdims=True)
    d = xf - _rb(s * (1.0 / M))
    ss = jnp.sum(d * d, axis=-1, keepdims=True)
    inv_d = _inv_sd(_gather(s) * (1.0 / M), _gather(ss) * (1.0 / M))
    inv = _scatter(inv_d, n)
    inv = jnp.concatenate([inv] * (M // 128), axis=1)
    if wr is None:
        return d, inv
    r = _rb(_gather(jnp.sum(d * wr, axis=-1, keepdims=True)) * inv_d)
    return d, inv, r

def _unpack_pair(buf):
    k = buf.shape[0] * G
    w = pltpu.bitcast(buf.reshape(2 * k, D), u32)
    w2 = jnp.concatenate([w << 16, w & jnp.uint32(0xFFFF0000)], axis=1)
    return pltpu.bitcast(w2, f32).astype(bf16)

def _pk(x):
    return pltpu.bitcast(x, u32)
def _upk(x):
    return pltpu.bitcast(x, bf16)

def parse(s):
    out = []
    for t in s.replace(",", " ").split():
        name = t.rstrip("0123456789")
        out.append((name,) + tuple(int(c) for c in t[len(name):]))
    return out

MID = ("QK70 QK71 KP7 QP7 PV70 QK60 PV71 QK61 VP7 KP6 QP6 PV60 QK50 PV61 QK51 OUT7 VP6 KP5 QP5 "
       "PV50 QK40 PV51 QK41 OUT6 VP5 KP4 QP4 PV40 QK30 PV41 QK31 OUT5 VP4 KP3 QP3 PV30 QK20 PV31 QK21 OUT4 VP3 KP2 QP2 "
       "PV20 QK10 PV21 QK11 OUT3 VP2 KP1 QP1 PV10 QK00 PV11 QK01 OUT2 VP1 KP0 QP0 PV00 PV01 OUT1 VP0 OUT0")
LAST = "QK0 QK1 QK7 PV0 PV1 QK6 PV7 QK5 PV6 QK4 PV5 QK3 QK2 PV4 PV3 PV2"

def make(mid=MID, last=LAST, NS=NP, skip="", nffn=1):
  mid, last = parse(mid), parse(last)
  def kernel(x_hbm, c_hbm, wq_hbm, wk_hbm, wv_hbm, wo_hbm, wr_hbm, wg_hbm, wu_hbm, wd_hbm,
             o_hbm, x_ref, c_ref, cp_ref, xn_ref, acc_ref, o_ref, bq, bk, bv, bo, q_ref, k_ref, v_ref, ctx_ref,
             wr_ref, wg_ref, wu_ref, wd_ref, wsem, xsem, csem, fsem, outsem):
    wtab = {"k": (0, wk_hbm, bk), "v": (1, wv_hbm, bv), "q": (2, wq_hbm, bq), "o": (3, wo_hbm, bo)}
    def wstart(name, pp, sl):
        t, w, b = wtab[name]
        h0 = 2 * pp if isinstance(pp, int) else pl.multiple_of(2 * pp, 2)
        if name == "o":
            pltpu.make_async_copy(w.at[pl.ds(h0, 2)], b.at[sl], wsem.at[t, sl]).start()
        else:
            for g in range(G):
                pltpu.make_async_copy(w.at[:, g, pl.ds(h0, 2), :], b.at[sl, :, pl.ds(2 * g, 2), :],
                                      wsem.at[t, sl]).start()
    def wwait(name, sl):
        t, w, b = wtab[name]
        pltpu.make_async_copy(b.at[sl], b.at[sl], wsem.at[t, sl]).wait()
    def rows(i, n, k=1):
        return pl.ds(i * n, k * n) if isinstance(i, int) else pl.ds(pl.multiple_of(i * n, n), k * n)
    def xcopy(i):
        return pltpu.make_async_copy(x_hbm.at[rows(i, TQ)], x_ref.at[rows(i, TQ)], xsem.at[i])
    def ccopy(i):
        return pltpu.make_async_copy(c_hbm.at[rows(i, TQ)], c_ref.at[rows(i, TQ)], csem.at[i])
    rcopy = pltpu.make_async_copy(wr_hbm, wr_ref, fsem.at[3])
    def fstart(j):
        cs = rows(j, F // FCH)
        pltpu.make_async_copy(wg_hbm.at[:, cs], wg_ref.at[:, cs], fsem.at[0]).start()
        pltpu.make_async_copy(wu_hbm.at[:, cs], wu_ref.at[:, cs], fsem.at[1]).start()
        pltpu.make_async_copy(wd_hbm.at[cs, :], wd_ref.at[cs, :], fsem.at[2]).start()
    def fwait():
        for t, r in enumerate((wg_ref, wu_ref, wd_ref)):
            pltpu.make_async_copy(r, r, fsem.at[t]).wait()
    def outcopy(i):
        return pltpu.make_async_copy(o_ref.at[rows(i, TQ)], o_hbm.at[rows(i, TQ)], outsem.at[i])

    R = TQ // 128

    def proj(src_ref, w, dst, i, scale=None):
        y = jnp.dot(_upk(src_ref[rows(i, T2), :]), w, preferred_element_type=f32)
        if scale is not None:
            y = y * scale
        for e in range(2):
            dst[e, rows(i, T2), :] = _pk(y[:, e * D:(e + 1) * D].astype(bf16))

    def qk(i, e, tri):
        r0 = i * TQ
        w0 = r0 + 128
        smain = lax.dot_general(_upk(q_ref[e, r0 // 2:(r0 + TQ) // 2, :]), _upk(k_ref[e, :w0 // 2, :]), NT,
                                preferred_element_type=f32)
        extra = [lax.dot_general(_upk(q_ref[e, (r0 + t * 128) // 2:(r0 + TQ) // 2, :]),
                                 _upk(k_ref[e, (r0 + t * 128) // 2:(r0 + (t + 1) * 128) // 2, :]), NT,
                                 preferred_element_type=f32) for t in range(1, R)]
        prow = []
        for a in range(R):
            pieces = [smain[a * 128:(a + 1) * 128]] + [extra[t - 1][(a - t) * 128:(a - t + 1) * 128] for t in range(1, a + 1)]
            sa = jnp.concatenate(pieces, axis=1) if len(pieces) > 1 else pieces[0]
            w = sa.shape[1]
            sd = jnp.where(tri, sa[:, w - 128:], -1e30)
            sa = jnp.concatenate([sa[:, :w - 128], sd], axis=1) if w > 128 else sd
            m = jnp.max(sa, axis=1, keepdims=True)
            prow.append(jnp.exp2(sa - m))
        return prow

    def pv(i, e, prow):
        w0 = i * TQ + 128
        pmb = jnp.concatenate([pp[:, :w0] for pp in prow], axis=0).astype(bf16)
        ctx = jnp.dot(pmb, _upk(v_ref[e, :w0 // 2, :]), preferred_element_type=f32)
        lm = jnp.sum(pmb.astype(f32), axis=1, keepdims=True)
        parts = []
        for a in range(R):
            ca = ctx[a * 128:(a + 1) * 128]
            la = lm[a * 128:(a + 1) * 128]
            if a > 0:
                peb = prow[a][:, w0:].astype(bf16)
                ca = ca + jnp.dot(peb, _upk(v_ref[e, w0 // 2:(w0 + a * 128) // 2, :]), preferred_element_type=f32)
                la = la + jnp.sum(peb.astype(f32), axis=1, keepdims=True)
            parts.append(ca * pl.reciprocal(la, approx=False, full_range=False))
        return jnp.concatenate(parts, axis=0)

    def causal_tri():
        return lax.broadcasted_iota(i32, (128, 128), 1) <= lax.broadcasted_iota(i32, (128, 128), 0)

    def step(pslot, oslot):
        tri = causal_tri()
        W = {}
        def getw(name):
            if name not in W:
                b = wtab[name][2]
                W[name] = b[oslot].reshape(2 * D, M) if name == "o" else _unpack_pair(b[pslot])
            return W[name]
        ps, ctxs = {}, {}
        for item in mid:
            op, i = item[0], item[1]
            if op == "KP":
                proj(cp_ref, getw("k"), k_ref, i)
            elif op == "VP":
                proj(cp_ref, getw("v"), v_ref, i)
            elif op == "QP":
                proj(xn_ref, getw("q"), q_ref, i, QSCALE)
            elif op == "QK":
                ps[i, item[2]] = qk(i, item[2], tri)
            elif op == "PV":
                ctxs[i, item[2]] = pv(i, item[2], ps.pop((i, item[2])))
            elif op == "OUT":
                c2 = jnp.concatenate([ctxs.pop((i, 0)), ctxs.pop((i, 1))], axis=1).astype(bf16)
                acc_ref[rows(i, TQ), :] += jnp.dot(c2, getw("o"), preferred_element_type=f32)

    for name in "kvq": wstart(name, 0, 0)
    for i in range(NB):
        ccopy(i).start(); xcopy(i).start()
    wstart("o", 0, 0)
    for name in "kvq": wstart(name, 1, 1)
    rcopy.start()
    for name in "kvq": wwait(name, 0)
    wk0, wv0, wq0 = _unpack_pair(bk[0]), _unpack_pair(bv[0]), _unpack_pair(bq[0])
    def pro(i, _):
        ccopy(i).wait(); xcopy(i).wait()
        cp_ref[rows(i, T2), :] = _pk(c_ref[rows(i, TQ), :])
        d, inv = _ln_block(x_ref[rows(i, TQ), :].astype(f32))
        xn_ref[rows(i, T2), :] = _pk((d * inv).astype(bf16))
        acc_ref[rows(i, TQ), :] = jnp.zeros((TQ, M), f32)
        proj(cp_ref, wk0, k_ref, i)
        proj(cp_ref, wv0, v_ref, i)
        proj(xn_ref, wq0, q_ref, i, QSCALE)
        return 0
    lax.fori_loop(0, NB, pro, 0)

    def body(p, _):
        s0 = p & 1
        s1 = 1 - s0
        for name in "kvq": wwait(name, s1)
        wwait("o", s0)
        pn = jnp.minimum(p + 2, NS - 1)
        for name in "kvq": wstart(name, pn, s0)
        wstart("o", p + 1, s1)
        if "F" not in skip:
            @pl.when(p < FCH)
            def _():
                fstart(p)
        step(s1, s0)
        return 0
    lax.fori_loop(0, NS - 1, body, 0)

    def last_head(e, _):
        tri = causal_tri()
        ps = {}
        for op, i in last:
            if op == "QK":
                ps[i] = qk(i, e, tri)
            else:
                ctx_ref[e, rows(i, T2), :] = _pk(pv(i, e, ps.pop(i)).astype(bf16))
        return 0
    lax.fori_loop(0, 2, last_head, 0)
    wwait("o", (NS - 1) & 1)
    rcopy.wait()
    for name in "kvq": wwait(name, NS & 1)
    if "F" not in skip:
        fwait()
    wr = wr_ref[...].astype(f32).reshape(1, M)
    wo = bo[(NS - 1) & 1].reshape(2 * D, M)

    def out_block(i, dst):
        c2 = _upk(jnp.concatenate([ctx_ref[0, rows(i, T2), :], ctx_ref[1, rows(i, T2), :]], axis=1))
        dst[...] += jnp.dot(c2, wo, preferred_element_type=f32)

    def epi_block(i, src, top):
        hh = _rb(x_ref[rows(i, TQ), :].astype(f32) + src[...])
        d, inv, r = _ln_block(hh, wr)
        o_ref[rows(i, TQ), :] = (hh + d * inv).astype(bf16)
        outcopy(i).start()
        b = pltpu.bitcast(r + 0.0, i32)
        key = b ^ (lax.shift_right_arithmetic(b, 31) & jnp.int32(0x7FFF0000))
        lane = lax.broadcasted_iota(i32, (8, 128), 1)
        tok = i * TQ + lane * 8 + lax.broadcasted_iota(i32, (8, 128), 0)
        key = jnp.where(lane < TQ // 8, key | (jnp.int32(0xFFFF) - tok), IMIN)
        return jnp.maximum(top[0], key), jnp.maximum(top[1], jnp.minimum(top[0], key))

    lo = jnp.full((8, 128), IMIN, i32)
    out_block(0, acc_ref.at[rows(0, TQ)])
    def oe(j, top):
        v = acc_ref.at[rows(j, TQ, 2)]
        top = epi_block(j, v.at[0:TQ], top)
        out_block(j + 1, v.at[TQ:2 * TQ])
        return top
    top = lax.fori_loop(0, NB - 1, oe, (lo, lo))
    t1, t2 = epi_block(NB - 1, acc_ref.at[rows(NB - 1, TQ)], top)

    def amax(t):
        return jnp.max(jnp.max(t, axis=1, keepdims=True), axis=0, keepdims=True)
    k1 = amax(t1)
    k2 = amax(jnp.where(t1 == k1, t2, t1))
    i1 = jnp.int32(0xFFFF) - (k1[0, 0] & jnp.int32(0xFFFF))
    i2 = jnp.int32(0xFFFF) - (k2[0, 0] & jnp.int32(0xFFFF))
    i1 = jnp.clip(i1, 0, S - 1); i2 = jnp.clip(i2, 0, S - 1)
    g1 = pl.multiple_of(i1 & ~7, 8); g2 = pl.multiple_of(i2 & ~7, 8)
    xg = jnp.concatenate([x_ref[pl.ds(g1, 8), :].astype(f32), x_ref[pl.ds(g2, 8), :].astype(f32)], axis=0)
    ag = jnp.concatenate([acc_ref[pl.ds(g1, 8), :], acc_ref[pl.ds(g2, 8), :]], axis=0)
    hh = _rb(xg + ag)
    mu = jnp.sum(hh, axis=-1, keepdims=True) * (1.0 / M)
    d = hh - _rb(mu)
    inv = _inv_sd(mu, jnp.sum(d * d, axis=-1, keepdims=True) * (1.0 / M))
    hn = d * inv
    hnb = hn.astype(bf16)
    r = _rb(jnp.sum(d * wr, axis=1, keepdims=True) * inv)
    sub = lax.broadcasted_iota(i32, (16, 1), 0)
    tok = jnp.where(sub < 8, g1 + sub, g2 + sub - 8)
    sel = (tok == i1) | (tok == i2)
    if "F" in skip:
        y = hn
    else:
        fw = F // nffn
        acts = []
        for j in range(nffn):
            g = _rb(jnp.dot(hnb, wg_ref[:, j * fw:(j + 1) * fw], preferred_element_type=f32))
            g = _rb(g * _rb(jax.nn.sigmoid(g)))
            u = _rb(jnp.dot(hnb, wu_ref[:, j * fw:(j + 1) * fw], preferred_element_type=f32))
            acts.append((g * u).astype(bf16))
        y = None
        for j in range(nffn):
            yj = jnp.dot(acts[j], wd_ref[j * fw:(j + 1) * fw, :], preferred_element_type=f32)
            y = yj if y is None else y + yj
        y = _rb(y)
    y = _rb(y * _rb(jax.nn.sigmoid(r)))
    res = (hh + jnp.where(sel, _rb(_rb(hn) + y), hn)).astype(bf16)
    for i in range(NB): outcopy(i).wait()
    o_ref[pl.ds(g1, 8), :] = res[:8]
    o_ref[pl.ds(g2, 8), :] = res[8:]
    cp1 = pltpu.make_async_copy(o_ref.at[pl.ds(g1, 8)], o_hbm.at[pl.ds(g1, 8)], outsem.at[0])
    cp1.start()
    @pl.when(g2 != g1)
    def _():
        cp2 = pltpu.make_async_copy(o_ref.at[pl.ds(g2, 8)], o_hbm.at[pl.ds(g2, 8)], outsem.at[1])
        cp2.start(); cp2.wait()
    cp1.wait()

  @jax.jit
  def run(A_x, A_c_kv, A_w_q, A_w_uk, A_w_uv, A_w_o, B_x, B_w_r, B_w_gate, B_w_up, B_w_down):
    anyspec = pl.BlockSpec(memory_space=pl.ANY)
    V = pltpu.VMEM
    DMA = pltpu.SemaphoreType.DMA
    out = pl.pallas_call(
        kernel,
        in_specs=[anyspec] * 10,
        out_specs=anyspec,
        out_shape=jax.ShapeDtypeStruct((S, M), bf16),
        scratch_shapes=[V((S, M), bf16), V((S, DC), bf16), V((S // 2, DC), u32), V((S // 2, M), u32),
                        V((S, M), f32), V((S, M), bf16),
                        V((2, M // G, 2 * G, D), bf16), V((2, DC // G, 2 * G, D), bf16), V((2, DC // G, 2 * G, D), bf16),
                        V((2, 2, D, M), bf16),
                        V((2, S // 2, D), u32), V((2, S // 2, D), u32), V((2, S // 2, D), u32), V((2, S // 2, D), u32),
                        V((M,), bf16), V((M, F), bf16), V((M, F), bf16), V((F, M), bf16),
                        DMA((4, 2)), DMA((NB,)), DMA((NB,)), DMA((4,)), DMA((NB,))],
        compiler_params=pltpu.CompilerParams(vmem_limit_bytes=120 * 1024 * 1024, disable_bounds_checks=True),
    )(A_x.reshape(S, M), A_c_kv.reshape(S, DC), A_w_q.reshape(M // G, G, H, D), A_w_uk.reshape(DC // G, G, H, D),
      A_w_uv.reshape(DC // G, G, H, D), A_w_o, B_w_r, B_w_gate, B_w_up, B_w_down)
    return out.reshape(1, S, M)
  return run


_run = make()


@jax.jit
def pallas_sequential_preLN__compressed_kv_cla__moe_arch_mod__prompt_kernel(
    A_x, A_c_kv, A_w_q, A_w_uk, A_w_uv, A_w_o, B_x, B_w_r, B_w_gate, B_w_up, B_w_down):
    return _run(A_x, A_c_kv, A_w_q, A_w_uk, A_w_uv, A_w_o, B_x, B_w_r, B_w_gate, B_w_up, B_w_down)
```

```python
import math

import jax
import jax.numpy as jnp
from jax import lax
from jax.experimental import pallas as pl
from jax.experimental.pallas import tpu as pltpu

S, M, H, D, DC, F = 2048, 1024, 32, 128, 512, 3584
EPS = 1e-5
bf16, f32, u32, i32 = jnp.bfloat16, jnp.float32, jnp.uint32, jnp.int32
NT = (((1,), (1,)), ((), ()))
G = 4
NP = H // 2
TQ = 256
NB = S // TQ
T2 = TQ // 2
NG = TQ // 8
FCH = 14
QSCALE = (D ** -0.5) * math.log2(math.e)
PACE = 58

MID = ("QK70 QK71 QK60 PV70 QP7 KP7 PV71 PV60 QK61 KP6 QP6 VP7 QK50 PV61 OUT7 VP6 QK51 KP5 QK40 PV50 PV51 "
       "QK41 QP5 OUT6 KP4 QP4 PV40 VP5 QK30 PV41 VP4 QK31 OUT5 KP3 PV30 QK20 PV31 OUT4 QP3 PV20 QK21 QP2 "
       "KP2 PV21 VP3 OUT3 VP2 QK10 QK11 QP1 PV10 QK00 PV11 KP1 QK01 QP0 OUT2 PV00 PV01 VP1 OUT1 VP0 KP0 OUT0")
LAST = "QK7 QK6 PV7 QK5 PV6 QK4 PV5 QK3 PV4 QK2 QK1 QK0 PV3 PV2 PV1 PV0"


def _parse(s):
    out = []
    for t in s.split():
        name = t.rstrip("0123456789")
        out.append((name,) + tuple(int(c) for c in t[len(name):]))
    return out


def _rb(x):
    return x.astype(bf16).astype(f32)


def _pk(x):
    return pltpu.bitcast(x, u32)


def _upk(x):
    return pltpu.bitcast(x, bf16)


def _gather(col):
    n = col.shape[0] // 8
    lane = lax.broadcasted_iota(i32, (8, 128), 1)
    vs = [jnp.broadcast_to(col[g * 8:(g + 1) * 8], (8, 128)) for g in range(n)]
    bit = 1
    while len(vs) > 1:
        m = (lane & bit) != 0
        vs = [jnp.where(m, vs[2 * k + 1], vs[2 * k]) for k in range(len(vs) // 2)]
        bit *= 2
    return vs[0]


def _scatter(dense, n):
    return jnp.concatenate([jnp.broadcast_to(dense[:, g:g + 1], (8, 128)) for g in range(n)], axis=0)


def _wide(v):
    return jnp.concatenate([v] * (M // 128), axis=1)


def _unpack_pair(buf):
    k = buf.shape[0] * G
    w = pltpu.bitcast(buf.reshape(2 * k, D), u32)
    w2 = jnp.concatenate([w << 16, w & jnp.uint32(0xFFFF0000)], axis=1)
    return pltpu.bitcast(w2, f32).astype(bf16)


def _rows(i, n, k=1):
    return pl.ds(i * n, k * n) if isinstance(i, int) else pl.ds(pl.multiple_of(i * n, n), k * n)


def _kernel(x_hbm, c_hbm, wq_hbm, wk_hbm, wv_hbm, wo_hbm, wr_hbm, wg_hbm, wu_hbm, wd_hbm, o_hbm,
            x_ref, c_ref, cp_ref, xn_ref, acc_ref, o_ref, bq, bk, bv, bo, q_ref, k_ref, v_ref, ctx_ref,
            wr_ref, wg_ref, wu_ref, wd_ref, st_ref, z_ref, wsem, xsem, csem, fsem, outsem):
    wtab = {"k": (0, wk_hbm, bk), "v": (1, wv_hbm, bv), "q": (2, wq_hbm, bq), "o": (3, wo_hbm, bo)}

    def wstart(name, pair, slot):
        t, w, b = wtab[name]
        heads = _rows(pair, 2)
        if name == "o":
            pltpu.make_async_copy(w.at[heads], b.at[slot], wsem.at[t, slot]).start()
        else:
            for g in range(G):
                pltpu.make_async_copy(w.at[:, g, heads, :], b.at[slot, :, pl.ds(2 * g, 2), :],
                                      wsem.at[t, slot]).start()

    def wwait(name, slot):
        t, _, b = wtab[name]
        pltpu.make_async_copy(b.at[slot], b.at[slot], wsem.at[t, slot]).wait()

    def xcopy(i):
        return pltpu.make_async_copy(x_hbm.at[_rows(i, TQ)], x_ref.at[_rows(i, TQ)], xsem.at[i])

    def ccopy(i):
        return pltpu.make_async_copy(c_hbm.at[_rows(i, TQ)], c_ref.at[_rows(i, TQ)], csem.at[i])

    def outcopy(i):
        return pltpu.make_async_copy(o_ref.at[_rows(i, TQ)], o_hbm.at[_rows(i, TQ)], outsem.at[i])

    rcopy = pltpu.make_async_copy(wr_hbm, wr_ref, fsem.at[3])

    def fstart(j):
        cs = _rows(j, F // FCH)
        pltpu.make_async_copy(wg_hbm.at[:, cs], wg_ref.at[:, cs], fsem.at[0]).start()
        pltpu.make_async_copy(wu_hbm.at[:, cs], wu_ref.at[:, cs], fsem.at[1]).start()
        pltpu.make_async_copy(wd_hbm.at[cs, :], wd_ref.at[cs, 0:M], fsem.at[2]).start()

    def fwait():
        for t, r in enumerate((wg_ref, wu_ref, wd_ref.at[:, 0:M])):
            pltpu.make_async_copy(r, r, fsem.at[t]).wait()

    def proj(src, w, dst, i, scale=None):
        y = jnp.dot(_upk(src), w, preferred_element_type=f32)
        if scale is not None:
            y = y * scale
        for e in range(2):
            dst[e, _rows(i, T2), :] = _pk(y[:, e * D:(e + 1) * D].astype(bf16))

    def causal_tri():
        return lax.broadcasted_iota(i32, (128, 128), 1) <= lax.broadcasted_iota(i32, (128, 128), 0)

    def qk(i, e, tri):
        r0 = i * TQ
        w0 = r0 + 128
        main = lax.dot_general(_upk(q_ref[e, r0 // 2:(r0 + TQ) // 2, :]), _upk(k_ref[e, :w0 // 2, :]), NT,
                               preferred_element_type=f32)
        diag = lax.dot_general(_upk(q_ref[e, w0 // 2:(r0 + TQ) // 2, :]),
                               _upk(k_ref[e, w0 // 2:(r0 + TQ) // 2, :]), NT, preferred_element_type=f32)
        up = jnp.where(tri, main[:128, r0:], -1e30)
        if r0:
            up = jnp.concatenate([main[:128, :r0], up], axis=1)
        low = jnp.concatenate([main[128:], jnp.where(tri, diag, -1e30)], axis=1)
        return [jnp.exp2(s - jnp.max(s, axis=1, keepdims=True)) for s in (up, low)]

    def pv(i, e, p):
        w0 = i * TQ + 128
        pm = jnp.concatenate([p[0], p[1][:, :w0]], axis=0).astype(bf16)
        ctx = jnp.dot(pm, _upk(v_ref[e, :w0 // 2, :]), preferred_element_type=f32)
        den = jnp.sum(pm.astype(f32), axis=1, keepdims=True)
        up = ctx[:128] * pl.reciprocal(den[:128], approx=False, full_range=False)
        pd = p[1][:, w0:].astype(bf16)
        low = ctx[128:] + jnp.dot(pd, _upk(v_ref[e, w0 // 2:(w0 + 128) // 2, :]), preferred_element_type=f32)
        dl = den[128:] + jnp.sum(pd.astype(f32), axis=1, keepdims=True)
        return jnp.concatenate([up, low * pl.reciprocal(dl, approx=False, full_range=False)], axis=0)

    for name in "kvq":
        wstart(name, 0, 0)
    for i in range(NB):
        ccopy(i).start()
        xcopy(i).start()
    wstart("o", 0, 0)
    for name in "kvq":
        wstart(name, 1, 1)
    rcopy.start()
    z_ref[...] = jnp.zeros((8, 128), u32)
    for name in "kvq":
        wwait(name, 0)
    wk0, wv0, wq0 = _unpack_pair(bk[0]), _unpack_pair(bv[0]), _unpack_pair(bq[0])

    def prologue(i, _):
        ccopy(i).wait()
        xcopy(i).wait()
        cpk = _pk(c_ref[_rows(i, TQ), :])
        cp_ref[_rows(i, T2), :] = cpk
        xf = x_ref[_rows(i, TQ), :].astype(f32)
        acc_ref[_rows(i, TQ), :] = xf
        d = xf - jnp.sum(xf, axis=-1, keepdims=True) * (1.0 / M)
        inv = lax.rsqrt(jnp.sum(d * d, axis=-1, keepdims=True) * (1.0 / M) + EPS)
        xnp = _pk((d * inv).astype(bf16))
        xn_ref[_rows(i, T2), :] = xnp
        proj(cpk, wk0, k_ref, i)
        proj(cpk, wv0, v_ref, i)
        proj(xnp, wq0, q_ref, i, QSCALE)
        return 0

    lax.fori_loop(0, NB, prologue, 0)

    def step(p, _):
        s0 = p & 1
        s1 = 1 - s0
        for name in "kvq":
            wwait(name, s1)
        wwait("o", s0)
        ahead = jnp.minimum(p + 2, NP - 1)
        for name in "kvq":
            wstart(name, ahead, s0)
        wstart("o", p + 1, s1)

        @pl.when(p < FCH)
        def _():
            fstart(p)

        tri = causal_tri()
        w = {}

        def weight(name):
            if name not in w:
                b = wtab[name][2]
                w[name] = b[s0].reshape(2 * D, M) if name == "o" else _unpack_pair(b[s1])
            return w[name]

        ps, ctxs = {}, {}
        for item in _parse(MID):
            op, i = item[0], item[1]
            if op == "KP":
                proj(cp_ref[_rows(i, T2), :], weight("k"), k_ref, i)
            elif op == "VP":
                proj(cp_ref[_rows(i, T2), :], weight("v"), v_ref, i)
            elif op == "QP":
                proj(xn_ref[_rows(i, T2), :], weight("q"), q_ref, i, QSCALE)
            elif op == "QK":
                ps[item[1:]] = qk(i, item[2], tri)
            elif op == "PV":
                ctxs[item[1:]] = pv(i, item[2], ps.pop(item[1:]))
            else:
                c2 = jnp.concatenate([ctxs.pop((i, 0)), ctxs.pop((i, 1))], axis=1).astype(bf16)
                acc_ref[_rows(i, TQ), :] += jnp.dot(c2, weight("o"), preferred_element_type=f32)
        return 0

    lax.fori_loop(0, NP - 1, step, 0)

    def last_head(e, _):
        tri = causal_tri()
        ps = {}
        for op, i in _parse(LAST):
            if op == "QK":
                ps[i] = qk(i, e, tri)
            else:
                ctx_ref[e, _rows(i, T2), :] = _pk(pv(i, e, ps.pop(i)).astype(bf16))
        return 0

    lax.fori_loop(0, 2, last_head, 0)
    wwait("o", (NP - 1) & 1)
    rcopy.wait()
    for name in "kvq":
        wwait(name, NP & 1)
    fwait()
    wr = wr_ref[...].astype(f32).reshape(1, M)
    wo = bo[(NP - 1) & 1].reshape(2 * D, M)

    def out_block(i, dst):
        c2 = _upk(jnp.concatenate([ctx_ref[0, _rows(i, T2), :], ctx_ref[1, _rows(i, T2), :]], axis=1))
        y = dst[...] + jnp.dot(c2, wo, preferred_element_type=f32)
        dst[...] = y
        return y

    def epi_block(i, src, top, y=None):
        hh = _rb(src[...])
        s = jnp.sum(hh, axis=-1, keepdims=True)
        mrow = _rb(s * (1.0 / M))
        if y is not None:
            z = z_ref[...]
            parts = []
            for g in range(NG):
                t = g * PACE // NG
                yt = y[(t % NG) * 8:(t % NG + 1) * 8, (t // NG) * 256:(t // NG) * 256 + 128]
                mg = jnp.broadcast_to(mrow[g * 8:(g + 1) * 8], (8, 128))
                parts.append(pltpu.bitcast(pltpu.bitcast(mg, u32) | (pltpu.bitcast(yt, u32) & z), f32))
            mrow = _wide(jnp.concatenate(parts, axis=0))
        d = hh - mrow
        mu = _gather(s) * (1.0 / M)
        mub = _rb(mu)
        dm = mu - mub
        var = _gather(jnp.sum(d * d, axis=-1, keepdims=True)) * (1.0 / M) - dm * dm
        sw = _gather(jnp.sum(d * wr, axis=-1, keepdims=True))
        ve = _rb(_rb(jnp.maximum(var, 0.0)) + EPS)
        inv = pl.reciprocal(_rb(ve * lax.rsqrt(ve)), approx=False, full_range=False)
        r = _rb(sw * inv)
        inv_s = _scatter(inv, NG)
        off_s = _scatter(mub * inv, NG)
        st_ref[0, _rows(i, TQ), :] = inv_s
        st_ref[1, _rows(i, TQ), :] = off_s
        o_ref[_rows(i, TQ), :] = (hh * _wide(inv_s + 1.0) - _wide(off_s)).astype(bf16)
        outcopy(i).start()
        b = pltpu.bitcast(r + 0.0, i32)
        code = lax.shift_right_arithmetic(b ^ (lax.shift_right_arithmetic(b, 31) & jnp.int32(0x7FFF0000)), 5)
        lane = lax.broadcasted_iota(i32, (8, 128), 1)
        tok = i * TQ + lane * 8 + lax.broadcasted_iota(i32, (8, 128), 0)
        key = pltpu.bitcast(code + (jnp.int32(0x24000000 + S - 1) - tok), f32)
        key = jnp.where(lane < NG, key, 0.0)
        return jnp.maximum(top[0], key), jnp.maximum(top[1], jnp.minimum(top[0], key))

    out_block(0, acc_ref.at[_rows(0, TQ)])

    def out_epi(j, top):
        v = acc_ref.at[_rows(j, TQ, 2)]
        y = out_block(j + 1, v.at[TQ:2 * TQ])
        return epi_block(j, v.at[0:TQ], top, y)

    lo = jnp.zeros((8, 128), f32)
    top = lax.fori_loop(0, NB - 1, out_epi, (lo, lo))
    t1, t2 = epi_block(NB - 1, acc_ref.at[_rows(NB - 1, TQ)], top)

    def amax(t):
        return jnp.max(jnp.max(t, axis=1, keepdims=True), axis=0, keepdims=True)

    k1 = amax(t1)
    k2 = amax(jnp.where(t1 == k1, t2, t1))
    i1 = (S - 1) - (pltpu.bitcast(k1, i32)[0, 0] & (S - 1))
    i2 = (S - 1) - (pltpu.bitcast(k2, i32)[0, 0] & (S - 1))
    g1 = pl.multiple_of(i1 & ~7, 8)
    g2 = pl.multiple_of(i2 & ~7, 8)

    def two(f):
        return jnp.concatenate([f(pl.ds(g1, 8)), f(pl.ds(g2, 8))], axis=0)

    hh = _rb(two(lambda r_: acc_ref[r_, :]))
    hn = hh * _wide(two(lambda r_: st_ref[0, r_, :])) - _wide(two(lambda r_: st_ref[1, r_, :]))
    hnb = hn.astype(bf16)
    r = _rb(jnp.sum(hn * wr, axis=1, keepdims=True))
    sub = lax.broadcasted_iota(i32, (16, 1), 0)
    tok = jnp.where(sub < 8, g1 + sub, g2 + sub - 8)
    sel = (tok == i1) | (tok == i2)
    g = _rb(jnp.dot(hnb, wg_ref[...], preferred_element_type=f32))
    g = _rb(g * _rb(jax.nn.sigmoid(g)))
    u = _rb(jnp.dot(hnb, wu_ref[...], preferred_element_type=f32))
    y = _rb(jnp.dot((g * u).astype(bf16), wd_ref[:, 0:M], preferred_element_type=f32))
    y = _rb(y * _rb(jax.nn.sigmoid(r)))
    res = (hh + jnp.where(sel, _rb(_rb(hn) + y), hn)).astype(bf16)
    for i in range(NB):
        outcopy(i).wait()
    o_ref[0:16, :] = res
    cp1 = pltpu.make_async_copy(o_ref.at[0:8], o_hbm.at[pl.ds(g1, 8)], outsem.at[0])
    cp1.start()

    @pl.when(g2 != g1)
    def _():
        cp2 = pltpu.make_async_copy(o_ref.at[8:16], o_hbm.at[pl.ds(g2, 8)], outsem.at[1])
        cp2.start()
        cp2.wait()

    cp1.wait()


@jax.jit
def pallas_sequential_preLN__compressed_kv_cla__moe_arch_mod__prompt_kernel(
    A_x: jax.Array,
    A_c_kv: jax.Array,
    A_w_q: jax.Array,
    A_w_uk: jax.Array,
    A_w_uv: jax.Array,
    A_w_o: jax.Array,
    B_x: jax.Array,
    B_w_r: jax.Array,
    B_w_gate: jax.Array,
    B_w_up: jax.Array,
    B_w_down: jax.Array,
):
    del B_x
    hbm = pl.BlockSpec(memory_space=pl.ANY)
    V = pltpu.VMEM
    DMA = pltpu.SemaphoreType.DMA
    out = pl.pallas_call(
        _kernel,
        in_specs=[hbm] * 10,
        out_specs=hbm,
        out_shape=jax.ShapeDtypeStruct((S, M), bf16),
        scratch_shapes=[
            V((S, M), bf16), V((S, DC), bf16),
            V((S // 2, DC), u32), V((S // 2, M), u32),
            V((S, M), f32), V((S, M), bf16),
            V((2, M // G, 2 * G, D), bf16), V((2, DC // G, 2 * G, D), bf16), V((2, DC // G, 2 * G, D), bf16),
            V((2, 2, D, M), bf16),
            V((2, S // 2, D), u32), V((2, S // 2, D), u32), V((2, S // 2, D), u32), V((2, S // 2, D), u32),
            V((M,), bf16), V((M, F), bf16), V((M, F), bf16),
            V((F, M + 128), bf16),
            V((2, S, 128), f32), V((8, 128), u32),
            DMA((4, 2)), DMA((NB,)), DMA((NB,)), DMA((4,)), DMA((NB,)),
        ],
        compiler_params=pltpu.CompilerParams(vmem_limit_bytes=120 * 1024 * 1024,
                                             disable_bounds_checks=True,
                                             disable_semaphore_checks=True),
    )(A_x.reshape(S, M), A_c_kv.reshape(S, DC), A_w_q.reshape(M // G, G, H, D),
      A_w_uk.reshape(DC // G, G, H, D), A_w_uv.reshape(DC // G, G, H, D), A_w_o,
      B_w_r, B_w_gate, B_w_up, B_w_down)
    return out.reshape(1, S, M)
```

```python
import math

import jax
import jax.numpy as jnp
from jax import lax
from jax.experimental import pallas as pl
from jax.experimental.pallas import tpu as pltpu

S, M, H, D, DC, F = 2048, 1024, 32, 128, 512, 3584
EPS = 1e-5
bf16, f32, u32, i32 = jnp.bfloat16, jnp.float32, jnp.uint32, jnp.int32
NT = (((1,), (1,)), ((), ()))
G = 4
NP = H // 2
TQ = 256
NB = S // TQ
T2 = TQ // 2
NG = TQ // 8
FCH = 14
QSCALE = (D ** -0.5) * math.log2(math.e)
PACE = 72

MID = ("QK70 QK71 QK60 PV70 QP7 KP7 PV71 PV60 QK61 KP6 QP6 VP7 QK50 PV61 OUT7 VP6 QK51 KP5 QK40 PV50 PV51 "
       "QK41 QP5 OUT6 KP4 QP4 PV40 VP5 QK30 PV41 VP4 QK31 OUT5 KP3 PV30 QK20 PV31 OUT4 QP3 PV20 QK21 QP2 "
       "KP2 PV21 VP3 OUT3 VP2 QK10 QK11 QP1 PV10 QK00 PV11 KP1 QK01 QP0 OUT2 PV00 PV01 VP1 OUT1 VP0 KP0 OUT0")
LAST = "QK7 QK6 PV7 QK5 PV6 QK4 PV5 QK3 PV4 QK2 QK1 QK0 PV3 PV2 PV1 PV0"


def _parse(s):
    out = []
    for t in s.split():
        name = t.rstrip("0123456789")
        out.append((name,) + tuple(int(c) for c in t[len(name):]))
    return out


def _rb(x):
    return x.astype(bf16).astype(f32)


def _pk(x):
    return pltpu.bitcast(x, u32)


def _upk(x):
    return pltpu.bitcast(x, bf16)


def _gather(col):
    n = col.shape[0] // 8
    lane = lax.broadcasted_iota(i32, (8, 128), 1)
    vs = [jnp.broadcast_to(col[g * 8:(g + 1) * 8], (8, 128)) for g in range(n)]
    bit = 1
    while len(vs) > 1:
        m = (lane & bit) != 0
        vs = [jnp.where(m, vs[2 * k + 1], vs[2 * k]) for k in range(len(vs) // 2)]
        bit *= 2
    return vs[0]


def _scatter(dense, n):
    return jnp.concatenate([jnp.broadcast_to(dense[:, g:g + 1], (8, 128)) for g in range(n)], axis=0)


def _wide(v):
    return jnp.concatenate([v] * (M // 128), axis=1)


def _unpack_pair(buf):
    k = buf.shape[0] * G
    w = pltpu.bitcast(buf.reshape(2 * k, D), u32)
    w2 = jnp.concatenate([w << 16, w & jnp.uint32(0xFFFF0000)], axis=1)
    return pltpu.bitcast(w2, f32).astype(bf16)


def _rows(i, n, k=1):
    return pl.ds(i * n, k * n) if isinstance(i, int) else pl.ds(pl.multiple_of(i * n, n), k * n)


def _kernel(x_hbm, c_hbm, wq_hbm, wk_hbm, wv_hbm, wo_hbm, wr_hbm, wg_hbm, wu_hbm, wd_hbm, o_hbm,
            x_ref, c_ref, cp_ref, xn_ref, acc_ref, o_ref, bq, bk, bv, bo, q_ref, k_ref, v_ref, ctx_ref,
            wr_ref, wg_ref, wu_ref, wd_ref, st_ref, z_ref, wsem, xsem, csem, fsem, outsem):
    wtab = {"k": (0, wk_hbm, bk), "v": (1, wv_hbm, bv), "q": (2, wq_hbm, bq), "o": (3, wo_hbm, bo)}

    def wstart(name, pair, slot):
        t, w, b = wtab[name]
        heads = _rows(pair, 2)
        if name == "o":
            pltpu.make_async_copy(w.at[heads], b.at[slot], wsem.at[t, slot]).start()
        else:
            for g in range(G):
                pltpu.make_async_copy(w.at[:, g, heads, :], b.at[slot, :, pl.ds(2 * g, 2), :],
                                      wsem.at[t, slot]).start()

    def wwait(name, slot):
        t, _, b = wtab[name]
        pltpu.make_async_copy(b.at[slot], b.at[slot], wsem.at[t, slot]).wait()

    def xcopy(i):
        return pltpu.make_async_copy(x_hbm.at[_rows(i, TQ)], x_ref.at[_rows(i, TQ)], xsem.at[i])

    def ccopy(i):
        return pltpu.make_async_copy(c_hbm.at[_rows(i, TQ)], c_ref.at[_rows(i, TQ)], csem.at[i])

    def outcopy(i):
        return pltpu.make_async_copy(o_ref.at[_rows(i, TQ)], o_hbm.at[_rows(i, TQ)], outsem.at[i])

    rcopy = pltpu.make_async_copy(wr_hbm, wr_ref, fsem.at[3])

    def fstart(j):
        cs = _rows(j, F // FCH)
        pltpu.make_async_copy(wg_hbm.at[:, cs], wg_ref.at[:, cs], fsem.at[0]).start()
        pltpu.make_async_copy(wu_hbm.at[:, cs], wu_ref.at[:, cs], fsem.at[1]).start()
        pltpu.make_async_copy(wd_hbm.at[cs, :], wd_ref.at[cs, 0:M], fsem.at[2]).start()

    def fwait():
        for t, r in enumerate((wg_ref, wu_ref, wd_ref.at[:, 0:M])):
            pltpu.make_async_copy(r, r, fsem.at[t]).wait()

    def proj(src, w, dst, i, scale=None):
        y = jnp.dot(_upk(src), w, preferred_element_type=f32)
        if scale is not None:
            y = y * scale
        for e in range(2):
            dst[e, _rows(i, T2), :] = _pk(y[:, e * D:(e + 1) * D].astype(bf16))

    def causal_tri():
        return lax.broadcasted_iota(i32, (128, 128), 1) <= lax.broadcasted_iota(i32, (128, 128), 0)

    def qk(i, e, tri):
        r0 = i * TQ
        w0 = r0 + 128
        main = lax.dot_general(_upk(q_ref[e, r0 // 2:(r0 + TQ) // 2, :]), _upk(k_ref[e, :w0 // 2, :]), NT,
                               preferred_element_type=f32)
        diag = lax.dot_general(_upk(q_ref[e, w0 // 2:(r0 + TQ) // 2, :]),
                               _upk(k_ref[e, w0 // 2:(r0 + TQ) // 2, :]), NT, preferred_element_type=f32)
        up = jnp.where(tri, main[:128, r0:], -1e30)
        if r0:
            up = jnp.concatenate([main[:128, :r0], up], axis=1)
        low = jnp.concatenate([main[128:], jnp.where(tri, diag, -1e30)], axis=1)
        return [jnp.exp2(s - jnp.max(s, axis=1, keepdims=True)) for s in (up, low)]

    def pv(i, e, p):
        w0 = i * TQ + 128
        pm = jnp.concatenate([p[0], p[1][:, :w0]], axis=0).astype(bf16)
        ctx = jnp.dot(pm, _upk(v_ref[e, :w0 // 2, :]), preferred_element_type=f32)
        den = jnp.sum(pm.astype(f32), axis=1, keepdims=True)
        up = ctx[:128] * pl.reciprocal(den[:128], approx=False, full_range=False)
        pd = p[1][:, w0:].astype(bf16)
        low = ctx[128:] + jnp.dot(pd, _upk(v_ref[e, w0 // 2:(w0 + 128) // 2, :]), preferred_element_type=f32)
        dl = den[128:] + jnp.sum(pd.astype(f32), axis=1, keepdims=True)
        return jnp.concatenate([up, low * pl.reciprocal(dl, approx=False, full_range=False)], axis=0)

    def issue(n, f):
        def body(i, _):
            f(i)
            return 0

        lax.fori_loop(0, n, body, 0)

    HB = NB // 2
    wstart("k", 0, 0)
    wstart("v", 0, 0)
    issue(HB, lambda i: ccopy(i).start())
    wstart("q", 0, 0)
    issue(HB, lambda t: (ccopy(HB + t).start(), xcopy(2 * t).start(), xcopy(2 * t + 1).start()))
    wstart("o", 0, 0)
    for name in "kvq":
        wstart(name, 1, 1)
    rcopy.start()
    z_ref[...] = jnp.zeros((8, 128), u32)
    wwait("k", 0)
    wk0 = _unpack_pair(bk[0])
    wwait("v", 0)
    wv0 = _unpack_pair(bv[0])

    def kv_block(i):
        cpk = _pk(c_ref[_rows(i, TQ), :])
        cp_ref[_rows(i, T2), :] = cpk
        proj(cpk, wk0, k_ref, i)
        proj(cpk, wv0, v_ref, i)

    def ln_block(i):
        xf = x_ref[_rows(i, TQ), :].astype(f32)
        acc_ref[_rows(i, TQ), :] = xf
        d = xf - jnp.sum(xf, axis=-1, keepdims=True) * (1.0 / M)
        inv = lax.rsqrt(jnp.sum(d * d, axis=-1, keepdims=True) * (1.0 / M) + EPS)
        xnp = _pk((d * inv).astype(bf16))
        xn_ref[_rows(i, T2), :] = xnp
        return xnp

    def pro_a(i, _):
        ccopy(i).wait()
        kv_block(i)
        return 0

    lax.fori_loop(0, HB, pro_a, 0)
    wwait("q", 0)
    wq0 = _unpack_pair(bq[0])

    def pro_b(t, _):
        ccopy(HB + t).wait()
        xcopy(2 * t).wait()
        xcopy(2 * t + 1).wait()
        xa = ln_block(2 * t)
        xb = ln_block(2 * t + 1)
        kv_block(HB + t)
        proj(xa, wq0, q_ref, 2 * t, QSCALE)
        proj(xb, wq0, q_ref, 2 * t + 1, QSCALE)
        return 0

    lax.fori_loop(0, HB, pro_b, 0)

    def step(p, _):
        s0 = p & 1
        s1 = 1 - s0
        for name in "kvq":
            wwait(name, s1)
        wwait("o", s0)
        ahead = jnp.minimum(p + 2, NP - 1)
        for name in "kvq":
            wstart(name, ahead, s0)
        wstart("o", p + 1, s1)

        @pl.when(p < FCH)
        def _():
            fstart(p)

        tri = causal_tri()
        w = {}

        def weight(name):
            if name not in w:
                b = wtab[name][2]
                w[name] = b[s0].reshape(2 * D, M) if name == "o" else _unpack_pair(b[s1])
            return w[name]

        ps, ctxs = {}, {}
        for item in _parse(MID):
            op, i = item[0], item[1]
            if op == "KP":
                proj(cp_ref[_rows(i, T2), :], weight("k"), k_ref, i)
            elif op == "VP":
                proj(cp_ref[_rows(i, T2), :], weight("v"), v_ref, i)
            elif op == "QP":
                proj(xn_ref[_rows(i, T2), :], weight("q"), q_ref, i, QSCALE)
            elif op == "QK":
                ps[item[1:]] = qk(i, item[2], tri)
            elif op == "PV":
                ctxs[item[1:]] = pv(i, item[2], ps.pop(item[1:]))
            else:
                c2 = jnp.concatenate([ctxs.pop((i, 0)), ctxs.pop((i, 1))], axis=1).astype(bf16)
                acc_ref[_rows(i, TQ), :] += jnp.dot(c2, weight("o"), preferred_element_type=f32)
        return 0

    lax.fori_loop(0, NP - 1, step, 0)

    def last_head(e, _):
        tri = causal_tri()
        ps = {}
        for op, i in _parse(LAST):
            if op == "QK":
                ps[i] = qk(i, e, tri)
            else:
                ctx_ref[e, _rows(i, T2), :] = _pk(pv(i, e, ps.pop(i)).astype(bf16))
        return 0

    lax.fori_loop(0, 2, last_head, 0)
    wwait("o", (NP - 1) & 1)
    rcopy.wait()
    for name in "kvq":
        wwait(name, NP & 1)
    fwait()
    wr = wr_ref[...].astype(f32).reshape(1, M)
    wo = bo[(NP - 1) & 1].reshape(2 * D, M)

    def out_block(i, dst):
        c2 = _upk(jnp.concatenate([ctx_ref[0, _rows(i, T2), :], ctx_ref[1, _rows(i, T2), :]], axis=1))
        y = dst[...] + jnp.dot(c2, wo, preferred_element_type=f32)
        dst[...] = _rb(y)
        return y

    def epi_block(i, src, top, y=None):
        hh = src[...]
        s = jnp.sum(hh, axis=-1, keepdims=True)
        mrow = _rb(s * (1.0 / M))
        if y is not None:
            z = z_ref[...]
            parts = []
            for g in range(NG):
                t = g * PACE // NG
                yt = y[(t % NG) * 8:(t % NG + 1) * 8, (t // NG) * 256:(t // NG) * 256 + 128]
                mg = jnp.broadcast_to(mrow[g * 8:(g + 1) * 8], (8, 128))
                parts.append(pltpu.bitcast(pltpu.bitcast(mg, u32) | (pltpu.bitcast(yt, u32) & z), f32))
            mrow = jnp.concatenate(parts, axis=0)
        else:
            mrow = jnp.broadcast_to(mrow, (TQ, 128))
        d = hh - _wide(mrow)
        mu = _gather(s) * (1.0 / M)
        dm = mu - _rb(mu)
        var = _gather(jnp.sum(d * d, axis=-1, keepdims=True)) * (1.0 / M) - dm * dm
        sw = _gather(jnp.sum(d * wr, axis=-1, keepdims=True))
        ve = _rb(_rb(jnp.maximum(var, 0.0)) + EPS)
        inv = pl.reciprocal(_rb(ve * lax.rsqrt(ve)), approx=False, full_range=False)
        r = _rb(sw * inv)
        inv_s = _scatter(inv, NG)
        st_ref[0, _rows(i, TQ), :] = inv_s
        st_ref[1, _rows(i, TQ), :] = mrow
        o_ref[_rows(i, TQ), :] = (hh * _wide(inv_s + 1.0) - _wide(mrow * inv_s)).astype(bf16)
        outcopy(i).start()
        b = pltpu.bitcast(r + 0.0, i32)
        code = lax.shift_right_arithmetic(b ^ (lax.shift_right_arithmetic(b, 31) & jnp.int32(0x7FFF0000)), 5)
        lane = lax.broadcasted_iota(i32, (8, 128), 1)
        tok = i * TQ + lane * 8 + lax.broadcasted_iota(i32, (8, 128), 0)
        key = pltpu.bitcast(code + (jnp.int32(0x24000000 + S - 1) - tok), f32)
        key = jnp.where(lane < NG, key, 0.0)
        return jnp.maximum(top[0], key), jnp.maximum(top[1], jnp.minimum(top[0], key))

    out_block(0, acc_ref.at[_rows(0, TQ)])

    def out_epi(j, top):
        v = acc_ref.at[_rows(j, TQ, 2)]
        y = out_block(j + 1, v.at[TQ:2 * TQ])
        return epi_block(j, v.at[0:TQ], top, y)

    lo = jnp.zeros((8, 128), f32)
    top = lax.fori_loop(0, NB - 1, out_epi, (lo, lo))
    t1, t2 = epi_block(NB - 1, acc_ref.at[_rows(NB - 1, TQ)], top)

    def amax(t):
        return jnp.max(jnp.max(t, axis=1, keepdims=True), axis=0, keepdims=True)

    k1 = amax(t1)
    k2 = amax(jnp.where(t1 == k1, t2, t1))
    i1 = (S - 1) - (pltpu.bitcast(k1, i32)[0, 0] & (S - 1))
    i2 = (S - 1) - (pltpu.bitcast(k2, i32)[0, 0] & (S - 1))
    g1 = pl.multiple_of(i1 & ~7, 8)
    g2 = pl.multiple_of(i2 & ~7, 8)

    def two(f):
        return jnp.concatenate([f(pl.ds(g1, 8)), f(pl.ds(g2, 8))], axis=0)

    hh = two(lambda r_: acc_ref[r_, :])
    hnb = (_rb(hh - _wide(two(lambda r_: st_ref[1, r_, :]))) * _wide(two(lambda r_: st_ref[0, r_, :]))).astype(bf16)
    hn = hnb.astype(f32)
    r = _rb(jnp.sum(hn * wr, axis=1, keepdims=True))
    sub = lax.broadcasted_iota(i32, (16, 1), 0)
    tok = jnp.where(sub < 8, g1 + sub, g2 + sub - 8)
    sel = (tok == i1) | (tok == i2)
    g = _rb(jnp.dot(hnb, wg_ref[...], preferred_element_type=f32))
    g = _rb(g * _rb(jax.nn.sigmoid(g)))
    u = _rb(jnp.dot(hnb, wu_ref[...], preferred_element_type=f32))
    y = _rb(jnp.dot((g * u).astype(bf16), wd_ref[:, 0:M], preferred_element_type=f32))
    y = _rb(y * _rb(jax.nn.sigmoid(r)))
    res = (hh + jnp.where(sel, _rb(hn + y), hn)).astype(bf16)
    for i in range(NB):
        outcopy(i).wait()
    o_ref[0:16, :] = res
    cp1 = pltpu.make_async_copy(o_ref.at[0:8], o_hbm.at[pl.ds(g1, 8)], outsem.at[0])
    cp1.start()

    @pl.when(g2 != g1)
    def _():
        cp2 = pltpu.make_async_copy(o_ref.at[8:16], o_hbm.at[pl.ds(g2, 8)], outsem.at[1])
        cp2.start()
        cp2.wait()

    cp1.wait()


@jax.jit
def pallas_sequential_preLN__compressed_kv_cla__moe_arch_mod__prompt_kernel(
    A_x: jax.Array,
    A_c_kv: jax.Array,
    A_w_q: jax.Array,
    A_w_uk: jax.Array,
    A_w_uv: jax.Array,
    A_w_o: jax.Array,
    B_x: jax.Array,
    B_w_r: jax.Array,
    B_w_gate: jax.Array,
    B_w_up: jax.Array,
    B_w_down: jax.Array,
):
    del B_x
    hbm = pl.BlockSpec(memory_space=pl.ANY)
    V = pltpu.VMEM
    DMA = pltpu.SemaphoreType.DMA
    out = pl.pallas_call(
        _kernel,
        in_specs=[hbm] * 10,
        out_specs=hbm,
        out_shape=jax.ShapeDtypeStruct((S, M), bf16),
        scratch_shapes=[
            V((S, M), bf16), V((S, DC), bf16),
            V((S // 2, DC), u32), V((S // 2, M), u32),
            V((S, M), f32), V((S, M), bf16),
            V((2, M // G, 2 * G, D), bf16), V((2, DC // G, 2 * G, D), bf16), V((2, DC // G, 2 * G, D), bf16),
            V((2, 2, D, M), bf16),
            V((2, S // 2, D), u32), V((2, S // 2, D), u32), V((2, S // 2, D), u32), V((2, S // 2, D), u32),
            V((M,), bf16), V((M, F), bf16), V((M, F), bf16),
            V((F, M + 128), bf16),
            V((2, S, 128), f32), V((8, 128), u32),
            DMA((4, 2)), DMA((NB,)), DMA((NB,)), DMA((4,)), DMA((NB,)),
        ],
        compiler_params=pltpu.CompilerParams(vmem_limit_bytes=120 * 1024 * 1024,
                                             disable_bounds_checks=True,
                                             disable_semaphore_checks=True),
    )(A_x.reshape(S, M), A_c_kv.reshape(S, DC), A_w_q.reshape(M // G, G, H, D),
      A_w_uk.reshape(DC // G, G, H, D), A_w_uv.reshape(DC // G, G, H, D), A_w_o,
      B_w_r, B_w_gate, B_w_up, B_w_down)
    return out.reshape(1, S, M)
```

```python
import math

import jax
import jax.numpy as jnp
from jax import lax
from jax.experimental import pallas as pl
from jax.experimental.pallas import tpu as pltpu

S, M, H, D, DC, F = 2048, 1024, 32, 128, 512, 3584
EPS = 1e-5
bf16, f32, u32, i32 = jnp.bfloat16, jnp.float32, jnp.uint32, jnp.int32
NT = (((1,), (1,)), ((), ()))
G = 4
NP = H // 2
TQ = 256
NB = S // TQ
T2 = TQ // 2
NG = TQ // 8
FCH = 14
QSCALE = (D ** -0.5) * math.log2(math.e)
PACE = 72

NEG = -1e30
GR = 16
NC = 128 // GR
TB = 128 * NC

MID = ("LT106 LT105 QK107 LT104 QK106 LT103 QK105 LT102 QK104 LT101 QK103 QK102 PV107 QK101 PV106 LT100 "
       "LT116 QK100 PV105 LT115 QK117 PV104 LT114 QK116 PV103 LT113 QK115 PV102 LT112 QK114 PV101 LT111 "
       "QK113 PV100 LT110 PV115 QK112 PV117 QK111 PV116 LT006 QK110 LT005 QK007 KP7 QP7 PV114 LT004 QK006 "
       "QP6 PV113 LT003 KP6 QK005 PV112 LT002 QK004 QP5 PV111 LT001 QK003 KP5 PV110 LT000 QK002 QP4 PV007 "
       "QK001 KP4 PV006 LT016 QK000 VP7 PV005 LT015 QK017 VP6 PV004 VP5 LT014 QK016 LT013 QK015 PV003 VP4 "
       "PV002 LT012 QK014 OUT7 QK013 OUT6 PV000 LT010 QK012 OUT5 PV001 LT011 PV017 QK011 OUT4 QK010 QP3 "
       "PV015 PV013 PV012 KP3 PV016 KP1 PV014 QP2 PV011 QP1 PV010 KP2 VP2 QP0 VP3 OUT3 VP1 VP0 OUT2 KP0 OUT1 "
       "OUT0")
LAST = ("LT15 LT16 QK17 LT14 QK16 LT13 QK14 LT11 QK15 LT12 PV17 QK13 PV16 LT10 QK11 PV14 QK12 PV15 QK10 LT06 "
       "PV13 LT05 QK07 LT04 PV12 QK06 PV11 QK05 LT03 PV10 LT02 QK04 PV07 LT01 QK03 PV06 LT00 QK02 PV05 QK01 "
       "PV04 QK00 PV03 PV02 PV01 PV00")


def _parse(s):
    out = []
    for t in s.split():
        name = t.rstrip("0123456789")
        out.append((name,) + tuple(int(c) for c in t[len(name):]))
    return out


def _rb(x):
    return x.astype(bf16).astype(f32)


def _pk(x):
    return pltpu.bitcast(x, u32)


def _upk(x):
    return pltpu.bitcast(x, bf16)


def _gather(col):
    n = col.shape[0] // 8
    lane = lax.broadcasted_iota(i32, (8, 128), 1)
    vs = [jnp.broadcast_to(col[g * 8:(g + 1) * 8], (8, 128)) for g in range(n)]
    bit = 1
    while len(vs) > 1:
        m = (lane & bit) != 0
        vs = [jnp.where(m, vs[2 * k + 1], vs[2 * k]) for k in range(len(vs) // 2)]
        bit *= 2
    return vs[0]


def _scatter(dense, n):
    return jnp.concatenate([jnp.broadcast_to(dense[:, g:g + 1], (8, 128)) for g in range(n)], axis=0)


def _wide(v):
    return jnp.concatenate([v] * (M // 128), axis=1)


def _unpack_pair(buf):
    k = buf.shape[0] * G
    w = pltpu.bitcast(buf.reshape(2 * k, D), u32)
    w2 = jnp.concatenate([w << 16, w & jnp.uint32(0xFFFF0000)], axis=1)
    return pltpu.bitcast(w2, f32).astype(bf16)


def _cat(parts, axis):
    return parts[0] if len(parts) == 1 else jnp.concatenate(parts, axis=axis)


def _rows(i, n, k=1):
    return pl.ds(i * n, k * n) if isinstance(i, int) else pl.ds(pl.multiple_of(i * n, n), k * n)


def _kernel(x_hbm, c_hbm, wq_hbm, wk_hbm, wv_hbm, wo_hbm, wr_hbm, wg_hbm, wu_hbm, wd_hbm, o_hbm,
            x_ref, c_ref, cp_ref, xn_ref, acc_ref, o_ref, bq, bk, bv, bo, q_ref, k_ref, v_ref, ctx_ref,
            wr_ref, wg_ref, wu_ref, wd_ref, st_ref, z_ref, wsem, xsem, csem, fsem, outsem):
    wtab = {"k": (0, wk_hbm, bk), "v": (1, wv_hbm, bv), "q": (2, wq_hbm, bq), "o": (3, wo_hbm, bo)}

    def wstart(name, pair, slot):
        t, w, b = wtab[name]
        heads = _rows(pair, 2)
        if name == "o":
            pltpu.make_async_copy(w.at[heads], b.at[slot], wsem.at[t, slot]).start()
        else:
            for g in range(G):
                pltpu.make_async_copy(w.at[:, g, heads, :], b.at[slot, :, pl.ds(2 * g, 2), :],
                                      wsem.at[t, slot]).start()

    def wwait(name, slot):
        t, _, b = wtab[name]
        pltpu.make_async_copy(b.at[slot], b.at[slot], wsem.at[t, slot]).wait()

    def xcopy(i):
        return pltpu.make_async_copy(x_hbm.at[_rows(i, TQ)], x_ref.at[_rows(i, TQ)], xsem.at[i])

    def ccopy(i):
        return pltpu.make_async_copy(c_hbm.at[_rows(i, TQ)], c_ref.at[_rows(i, TQ)], csem.at[i])

    def outcopy(i):
        return pltpu.make_async_copy(o_ref.at[_rows(i, TQ)], o_hbm.at[_rows(i, TQ)], outsem.at[i])

    rcopy = pltpu.make_async_copy(wr_hbm, wr_ref, fsem.at[3])

    def fstart(j):
        cs = _rows(j, F // FCH)
        pltpu.make_async_copy(wg_hbm.at[:, cs], wg_ref.at[:, cs], fsem.at[0]).start()
        pltpu.make_async_copy(wu_hbm.at[:, cs], wu_ref.at[:, cs], fsem.at[1]).start()
        pltpu.make_async_copy(wd_hbm.at[cs, :], wd_ref.at[cs, 0:M], fsem.at[2]).start()

    def fwait():
        for t, r in enumerate((wg_ref, wu_ref, wd_ref.at[:, 0:M])):
            pltpu.make_async_copy(r, r, fsem.at[t]).wait()

    def proj(src, w, dst, i, scale=None):
        y = jnp.dot(_upk(src), w, preferred_element_type=f32)
        if scale is not None:
            y = y * scale
        for e in range(2):
            dst[e, _rows(i, T2), :] = _pk(y[:, e * D:(e + 1) * D].astype(bf16))

    def pr(ref, e, lo, hi):
        return ref[e, lo // 2:hi // 2, :]

    def nt(a, b):
        return lax.dot_general(_upk(a), _upk(b), NT, preferred_element_type=f32)

    def iota2():
        return lax.broadcasted_iota(i32, (GR, 128), 0), lax.broadcasted_iota(i32, (GR, 128), 1)

    def causal_tri():
        row, col = iota2()
        return col <= row + (128 - GR)

    def qunit(I, e, c):
        return _cat([pr(q_ref, e, r, r + GR) for r in range(I * TB + GR * c, (I + 1) * TB, 128)], 0)

    def left(I, e, c):
        s = GR * (c + 1)
        st = nt(pr(k_ref, e, 0, s), qunit(I, e, c))
        t = jnp.concatenate([st, jnp.full((128 - s, 128), NEG, f32)], axis=0).T
        if I == 0:
            row, col = iota2()
            t = jnp.concatenate([jnp.where(col <= row + GR * c, t[:GR], NEG), t[GR:]], axis=0)
        return t

    def qk(I, e, c, tri, lf):
        r0 = I * TB
        s = GR * (c + 1)
        q = qunit(I, e, c)
        if s == 128:
            mn = nt(q, pr(k_ref, e, 0, r0 + 128))
        else:
            mn = _cat([lf] + ([nt(q, pr(k_ref, e, s, r0 + s))] if r0 else []), 1)
        ex = [nt(q[x * GR // 2:], pr(k_ref, e, r0 + s + 128 * (x - 1), r0 + s + 128 * x)) for x in range(1, NC)]
        out = []
        for a in range(NC):
            sa = _cat([mn[a * GR:(a + 1) * GR]]
                      + [ex[x - 1][(a - x) * GR:(a - x + 1) * GR] for x in range(1, a + 1)], 1)
            w = sa.shape[1]
            if not (s < 128 and w == 128):
                sa = _cat(([sa[:, :w - 128]] if w > 128 else []) + [jnp.where(tri, sa[:, w - 128:], NEG)], 1)
            out.append(jnp.exp2(sa - jnp.max(sa, axis=1, keepdims=True)))
        return out

    def pv(I, e, c, p, nv):
        r0 = I * TB
        s = GR * (c + 1)
        w0 = r0 + 128
        vpu = c < nv
        if s == 128:
            vm = [pr(v_ref, e, 0, w0)]
        else:
            vm = ([] if vpu else [pr(v_ref, e, 0, 128)]) + ([pr(v_ref, e, s, r0 + s)] if r0 else [])
        ctx = None
        if vm:
            pm = _cat([pa[:, 128 * vpu:w0] for pa in p], 0).astype(bf16)
            ctx = jnp.dot(pm, _upk(_cat(vm, 0)), preferred_element_type=f32)
        if vpu:
            v0 = _upk(pr(v_ref, e, 0, s)).astype(f32)
            pp = _pk(_cat([pa[:, :128] for pa in p], 0).astype(bf16))
            acc = None
            for k in range(s):
                t = _upk(jnp.broadcast_to(pp[:, k:k + 1], (64, 128))).astype(f32) * v0[k:k + 1, :]
                acc = t if acc is None else acc + t
            ctx = acc if ctx is None else ctx + acc
        cs = [ctx[a * GR:(a + 1) * GR] for a in range(NC)]
        den = [jnp.sum(pa.astype(bf16).astype(f32), axis=1, keepdims=True) for pa in p]
        for x in range(1, NC):
            px = _cat([p[a][:, w0 + 128 * (x - 1):w0 + 128 * x] for a in range(x, NC)], 0).astype(bf16)
            cx = jnp.dot(px, _upk(pr(v_ref, e, r0 + s + 128 * (x - 1), r0 + s + 128 * x)),
                         preferred_element_type=f32)
            for a in range(x, NC):
                cs[a] = cs[a] + cx[(a - x) * GR:(a - x + 1) * GR]
        return [cs[a] * pl.reciprocal(den[a], approx=False, full_range=False) for a in range(NC)]

    def issue(n, f):
        def body(i, _):
            f(i)
            return 0

        lax.fori_loop(0, n, body, 0)

    HB = NB // 2
    wstart("k", 0, 0)
    wstart("v", 0, 0)
    issue(HB, lambda i: ccopy(i).start())
    wstart("q", 0, 0)
    issue(HB, lambda t: (ccopy(HB + t).start(), xcopy(2 * t).start(), xcopy(2 * t + 1).start()))
    wstart("o", 0, 0)
    for name in "kvq":
        wstart(name, 1, 1)
    rcopy.start()
    z_ref[...] = jnp.zeros((8, 128), u32)
    wwait("k", 0)
    wk0 = _unpack_pair(bk[0])
    wwait("v", 0)
    wv0 = _unpack_pair(bv[0])

    def kv_block(i):
        cpk = _pk(c_ref[_rows(i, TQ), :])
        cp_ref[_rows(i, T2), :] = cpk
        proj(cpk, wk0, k_ref, i)
        proj(cpk, wv0, v_ref, i)

    def ln_block(i):
        xf = x_ref[_rows(i, TQ), :].astype(f32)
        acc_ref[_rows(i, TQ), :] = xf
        d = xf - jnp.sum(xf, axis=-1, keepdims=True) * (1.0 / M)
        inv = lax.rsqrt(jnp.sum(d * d, axis=-1, keepdims=True) * (1.0 / M) + EPS)
        xnp = _pk((d * inv).astype(bf16))
        xn_ref[_rows(i, T2), :] = xnp
        return xnp

    def pro_a(i, _):
        ccopy(i).wait()
        kv_block(i)
        return 0

    lax.fori_loop(0, HB, pro_a, 0)
    wwait("q", 0)
    wq0 = _unpack_pair(bq[0])

    def pro_b(t, _):
        ccopy(HB + t).wait()
        xcopy(2 * t).wait()
        xcopy(2 * t + 1).wait()
        xa = ln_block(2 * t)
        xb = ln_block(2 * t + 1)
        kv_block(HB + t)
        proj(xa, wq0, q_ref, 2 * t, QSCALE)
        proj(xb, wq0, q_ref, 2 * t + 1, QSCALE)
        return 0

    lax.fori_loop(0, HB, pro_b, 0)

    def step(p, _):
        s0 = p & 1
        s1 = 1 - s0
        for name in "kvq":
            wwait(name, s1)
        wwait("o", s0)
        ahead = jnp.minimum(p + 2, NP - 1)
        for name in "kvq":
            wstart(name, ahead, s0)
        wstart("o", p + 1, s1)

        @pl.when(p < FCH)
        def _():
            fstart(p)

        tri = causal_tri()
        w = {}

        def weight(name):
            if name not in w:
                b = wtab[name][2]
                w[name] = b[s0].reshape(2 * D, M) if name == "o" else _unpack_pair(b[s1])
            return w[name]

        lfs, ps, ctxs = {}, {}, {}
        for item in _parse(MID):
            op, i, u = item[0], item[1], item[1:]
            if op == "LT":
                lfs[u] = left(*u)
            elif op == "KP":
                proj(cp_ref[_rows(i, T2), :], weight("k"), k_ref, i)
            elif op == "VP":
                proj(cp_ref[_rows(i, T2), :], weight("v"), v_ref, i)
            elif op == "QP":
                proj(xn_ref[_rows(i, T2), :], weight("q"), q_ref, i, QSCALE)
            elif op == "QK":
                ps[u] = qk(*u, tri, lfs.pop(u, None))
            elif op == "PV":
                ctxs[u] = pv(*u, ps.pop(u), 1)
            else:
                I, a0 = divmod(2 * i, NC)
                c2 = jnp.concatenate([_cat([ctxs[I, e, c][a] for a in (a0, a0 + 1) for c in range(NC)], 0)
                                      for e in range(2)], axis=1).astype(bf16)
                acc_ref[_rows(i, TQ), :] += jnp.dot(c2, weight("o"), preferred_element_type=f32)
        return 0

    lax.fori_loop(0, NP - 1, step, 0)

    def last_head(e, _):
        tri = causal_tri()
        lfs, ps = {}, {}
        for op, I, c in _parse(LAST):
            if op == "LT":
                lfs[I, c] = left(I, e, c)
            elif op == "QK":
                ps[I, c] = qk(I, e, c, tri, lfs.pop((I, c), None))
            else:
                for a, ca in enumerate(pv(I, e, c, ps.pop((I, c)), 0)):
                    r = (I * TB + 128 * a + GR * c) // 2
                    ctx_ref[e, r:r + GR // 2, :] = _pk(ca.astype(bf16))
        return 0

    lax.fori_loop(0, 2, last_head, 0)
    wwait("o", (NP - 1) & 1)
    rcopy.wait()
    for name in "kvq":
        wwait(name, NP & 1)
    fwait()
    wr = wr_ref[...].astype(f32).reshape(1, M)
    wo = bo[(NP - 1) & 1].reshape(2 * D, M)

    def out_block(i, dst):
        c2 = _upk(jnp.concatenate([ctx_ref[0, _rows(i, T2), :], ctx_ref[1, _rows(i, T2), :]], axis=1))
        y = dst[...] + jnp.dot(c2, wo, preferred_element_type=f32)
        dst[...] = _rb(y)
        return y

    def epi_block(i, src, top, y=None):
        hh = src[...]
        s = jnp.sum(hh, axis=-1, keepdims=True)
        mrow = _rb(s * (1.0 / M))
        if y is not None:
            z = z_ref[...]
            parts = []
            for g in range(NG):
                t = g * PACE // NG
                yt = y[(t % NG) * 8:(t % NG + 1) * 8, (t // NG) * 256:(t // NG) * 256 + 128]
                mg = jnp.broadcast_to(mrow[g * 8:(g + 1) * 8], (8, 128))
                parts.append(pltpu.bitcast(pltpu.bitcast(mg, u32) | (pltpu.bitcast(yt, u32) & z), f32))
            mrow = jnp.concatenate(parts, axis=0)
        else:
            mrow = jnp.broadcast_to(mrow, (TQ, 128))
        d = hh - _wide(mrow)
        mu = _gather(s) * (1.0 / M)
        dm = mu - _rb(mu)
        var = _gather(jnp.sum(d * d, axis=-1, keepdims=True)) * (1.0 / M) - dm * dm
        sw = _gather(jnp.sum(d * wr, axis=-1, keepdims=True))
        ve = _rb(_rb(jnp.maximum(var, 0.0)) + EPS)
        inv = pl.reciprocal(_rb(ve * lax.rsqrt(ve)), approx=False, full_range=False)
        r = _rb(sw * inv)
        inv_s = _scatter(inv, NG)
        st_ref[0, _rows(i, TQ), :] = inv_s
        st_ref[1, _rows(i, TQ), :] = mrow
        o_ref[_rows(i, TQ), :] = (hh * _wide(inv_s + 1.0) - _wide(mrow * inv_s)).astype(bf16)
        outcopy(i).start()
        b = pltpu.bitcast(r + 0.0, i32)
        code = lax.shift_right_arithmetic(b ^ (lax.shift_right_arithmetic(b, 31) & jnp.int32(0x7FFF0000)), 5)
        lane = lax.broadcasted_iota(i32, (8, 128), 1)
        tok = i * TQ + lane * 8 + lax.broadcasted_iota(i32, (8, 128), 0)
        key = pltpu.bitcast(code + (jnp.int32(0x24000000 + S - 1) - tok), f32)
        key = jnp.where(lane < NG, key, 0.0)
        return jnp.maximum(top[0], key), jnp.maximum(top[1], jnp.minimum(top[0], key))

    out_block(0, acc_ref.at[_rows(0, TQ)])

    def out_epi(j, top):
        v = acc_ref.at[_rows(j, TQ, 2)]
        y = out_block(j + 1, v.at[TQ:2 * TQ])
        return epi_block(j, v.at[0:TQ], top, y)

    lo = jnp.zeros((8, 128), f32)
    top = lax.fori_loop(0, NB - 1, out_epi, (lo, lo))
    t1, t2 = epi_block(NB - 1, acc_ref.at[_rows(NB - 1, TQ)], top)

    def amax(t):
        return jnp.max(jnp.max(t, axis=1, keepdims=True), axis=0, keepdims=True)

    k1 = amax(t1)
    k2 = amax(jnp.where(t1 == k1, t2, t1))
    i1 = (S - 1) - (pltpu.bitcast(k1, i32)[0, 0] & (S - 1))
    i2 = (S - 1) - (pltpu.bitcast(k2, i32)[0, 0] & (S - 1))
    g1 = pl.multiple_of(i1 & ~7, 8)
    g2 = pl.multiple_of(i2 & ~7, 8)

    def two(f):
        return jnp.concatenate([f(pl.ds(g1, 8)), f(pl.ds(g2, 8))], axis=0)

    hh = two(lambda r_: acc_ref[r_, :])
    hnb = (_rb(hh - _wide(two(lambda r_: st_ref[1, r_, :]))) * _wide(two(lambda r_: st_ref[0, r_, :]))).astype(bf16)
    hn = hnb.astype(f32)
    r = _rb(jnp.sum(hn * wr, axis=1, keepdims=True))
    sub = lax.broadcasted_iota(i32, (16, 1), 0)
    tok = jnp.where(sub < 8, g1 + sub, g2 + sub - 8)
    sel = (tok == i1) | (tok == i2)
    g = _rb(jnp.dot(hnb, wg_ref[...], preferred_element_type=f32))
    g = _rb(g * _rb(jax.nn.sigmoid(g)))
    u = _rb(jnp.dot(hnb, wu_ref[...], preferred_element_type=f32))
    y = _rb(jnp.dot((g * u).astype(bf16), wd_ref[:, 0:M], preferred_element_type=f32))
    y = _rb(y * _rb(jax.nn.sigmoid(r)))
    res = (hh + jnp.where(sel, _rb(hn + y), hn)).astype(bf16)
    for i in range(NB):
        outcopy(i).wait()
    o_ref[0:16, :] = res
    cp1 = pltpu.make_async_copy(o_ref.at[0:8], o_hbm.at[pl.ds(g1, 8)], outsem.at[0])
    cp1.start()

    @pl.when(g2 != g1)
    def _():
        cp2 = pltpu.make_async_copy(o_ref.at[8:16], o_hbm.at[pl.ds(g2, 8)], outsem.at[1])
        cp2.start()
        cp2.wait()

    cp1.wait()


@jax.jit
def pallas_sequential_preLN__compressed_kv_cla__moe_arch_mod__prompt_kernel(
    A_x: jax.Array,
    A_c_kv: jax.Array,
    A_w_q: jax.Array,
    A_w_uk: jax.Array,
    A_w_uv: jax.Array,
    A_w_o: jax.Array,
    B_x: jax.Array,
    B_w_r: jax.Array,
    B_w_gate: jax.Array,
    B_w_up: jax.Array,
    B_w_down: jax.Array,
):
    del B_x
    hbm = pl.BlockSpec(memory_space=pl.ANY)
    V = pltpu.VMEM
    DMA = pltpu.SemaphoreType.DMA
    out = pl.pallas_call(
        _kernel,
        in_specs=[hbm] * 10,
        out_specs=hbm,
        out_shape=jax.ShapeDtypeStruct((S, M), bf16),
        scratch_shapes=[
            V((S, M), bf16), V((S, DC), bf16),
            V((S // 2, DC), u32), V((S // 2, M), u32),
            V((S, M), f32), V((S, M), bf16),
            V((2, M // G, 2 * G, D), bf16), V((2, DC // G, 2 * G, D), bf16), V((2, DC // G, 2 * G, D), bf16),
            V((2, 2, D, M), bf16),
            V((2, S // 2, D), u32), V((2, S // 2, D), u32), V((2, S // 2, D), u32), V((2, S // 2, D), u32),
            V((M,), bf16), V((M, F), bf16), V((M, F), bf16),
            V((F, M + 128), bf16),
            V((2, S, 128), f32), V((8, 128), u32),
            DMA((4, 2)), DMA((NB,)), DMA((NB,)), DMA((4,)), DMA((NB,)),
        ],
        compiler_params=pltpu.CompilerParams(vmem_limit_bytes=120 * 1024 * 1024,
                                             disable_bounds_checks=True,
                                             disable_semaphore_checks=True),
    )(A_x.reshape(S, M), A_c_kv.reshape(S, DC), A_w_q.reshape(M // G, G, H, D),
      A_w_uk.reshape(DC // G, G, H, D), A_w_uv.reshape(DC // G, G, H, D), A_w_o,
      B_w_r, B_w_gate, B_w_up, B_w_down)
    return out.reshape(1, S, M)
```

```python
import math

import jax
import jax.numpy as jnp
from jax import lax
from jax.experimental import pallas as pl
from jax.experimental.pallas import tpu as pltpu

S, M, H, D, DC, F = 2048, 1024, 32, 128, 512, 3584
EPS = 1e-5
bf16, f32, u32, i32 = jnp.bfloat16, jnp.float32, jnp.uint32, jnp.int32
NT = (((1,), (1,)), ((), ()))
G = 4
NP = H // 2
TQ = 256
NB = S // TQ
T2 = TQ // 2
NG = TQ // 8
FCH = 14
QSCALE = (D ** -0.5) * math.log2(math.e)
PACE = 72

NEG = -1e30
GR = 16
NC = 128 // GR
TB = 128 * NC

MID = ("LT106 LT105 QK107 LT104 QK106 LT103 QK105 LT102 QK104 LT101 QK103 LT100 QK102 PV107 QK101 PV106 "
       "LT116 QK100 PV105 LT115 QK117 PV104 LT114 QK116 PV103 LT113 QK115 PV102 LT112 QK114 PV101 LT111 "
       "QK113 PV100 LT110 QK112 PV117 QK111 PV116 LT006 QK110 PV115 LT005 QK007 KP7 QP7 PV114 LT004 QK006 "
       "QP6 PV113 LT003 KP6 QK005 PV112 LT002 QK004 QP5 PV111 LT001 QK003 KP5 PV110 LT000 QK002 QP4 PV007 "
       "QK001 KP4 PV006 LT016 QK000 VP7 PV005 LT015 QK017 VP6 PV004 LT014 QK016 VP5 PV003 LT013 QK015 VP4 "
       "PV002 LT012 QK014 OUT7 PV001 LT011 QK013 OUT6 PV000 LT010 QK012 OUT5 PV017 QK011 OUT4 PV016 QK010 "
       "QP3 PV015 PV013 PV012 KP3 KP1 PV014 QP2 PV011 PV010 KP2 QP1 VP2 QP0 VP3 VP1 VP0 OUT3 KP0 OUT2 OUT1 "
       "OUT0")
LAST = ("LT15 LT16 QK17 LT14 QK16 LT13 QK14 LT11 QK15 LT12 PV17 QK13 PV16 LT10 QK11 PV14 QK12 PV15 QK10 LT06 "
       "PV13 LT05 QK07 LT04 PV12 QK06 PV11 QK05 LT03 PV10 LT02 QK04 PV07 LT01 QK03 PV06 LT00 QK02 PV05 QK01 "
       "PV04 QK00 PV03 PV02 PV01 PV00")


def _parse(s):
    out = []
    for t in s.split():
        name = t.rstrip("0123456789")
        out.append((name,) + tuple(int(c) for c in t[len(name):]))
    return out


def _rb(x):
    return x.astype(bf16).astype(f32)


def _pk(x):
    return pltpu.bitcast(x, u32)


def _upk(x):
    return pltpu.bitcast(x, bf16)


def _gather(col):
    n = col.shape[0] // 8
    lane = lax.broadcasted_iota(i32, (8, 128), 1)
    vs = [jnp.broadcast_to(col[g * 8:(g + 1) * 8], (8, 128)) for g in range(n)]
    bit = 1
    while len(vs) > 1:
        m = (lane & bit) != 0
        vs = [jnp.where(m, vs[2 * k + 1], vs[2 * k]) for k in range(len(vs) // 2)]
        bit *= 2
    return vs[0]


def _scatter(dense, n):
    return jnp.concatenate([jnp.broadcast_to(dense[:, g:g + 1], (8, 128)) for g in range(n)], axis=0)


def _wide(v):
    return jnp.concatenate([v] * (M // 128), axis=1)


def _unpack_pair(buf):
    k = buf.shape[0] * G
    w = pltpu.bitcast(buf.reshape(2 * k, D), u32)
    w2 = jnp.concatenate([w << 16, w & jnp.uint32(0xFFFF0000)], axis=1)
    return pltpu.bitcast(w2, f32).astype(bf16)


def _cat(parts, axis):
    return parts[0] if len(parts) == 1 else jnp.concatenate(parts, axis=axis)


def _rows(i, n, k=1):
    return pl.ds(i * n, k * n) if isinstance(i, int) else pl.ds(pl.multiple_of(i * n, n), k * n)


def _kernel(x_hbm, c_hbm, wq_hbm, wk_hbm, wv_hbm, wo_hbm, wr_hbm, wg_hbm, wu_hbm, wd_hbm, o_hbm,
            x_ref, c_ref, cp_ref, xn_ref, acc_ref, o_ref, bq, bk, bv, bo, q_ref, k_ref, v_ref, ctx_ref,
            wr_ref, wg_ref, wu_ref, wd_ref, st_ref, z_ref, wsem, xsem, csem, fsem, outsem):
    wtab = {"k": (0, wk_hbm, bk), "v": (1, wv_hbm, bv), "q": (2, wq_hbm, bq), "o": (3, wo_hbm, bo)}

    def wstart(name, pair, slot):
        t, w, b = wtab[name]
        heads = _rows(pair, 2)
        if name == "o":
            pltpu.make_async_copy(w.at[heads], b.at[slot], wsem.at[t, slot]).start()
        else:
            for g in range(G):
                pltpu.make_async_copy(w.at[:, g, heads, :], b.at[slot, :, pl.ds(2 * g, 2), :],
                                      wsem.at[t, slot]).start()

    def wwait(name, slot):
        t, _, b = wtab[name]
        pltpu.make_async_copy(b.at[slot], b.at[slot], wsem.at[t, slot]).wait()

    def xcopy(i):
        return pltpu.make_async_copy(x_hbm.at[_rows(i, TQ)], x_ref.at[_rows(i, TQ)], xsem.at[i])

    def ccopy(i):
        return pltpu.make_async_copy(c_hbm.at[_rows(i, TQ)], c_ref.at[_rows(i, TQ)], csem.at[i])

    def outcopy(i):
        return pltpu.make_async_copy(o_ref.at[_rows(i, TQ)], o_hbm.at[_rows(i, TQ)], outsem.at[i])

    rcopy = pltpu.make_async_copy(wr_hbm, wr_ref, fsem.at[3])

    def fstart(j):
        cs = _rows(j, F // FCH)
        pltpu.make_async_copy(wg_hbm.at[:, cs], wg_ref.at[:, cs], fsem.at[0]).start()
        pltpu.make_async_copy(wu_hbm.at[:, cs], wu_ref.at[:, cs], fsem.at[1]).start()
        pltpu.make_async_copy(wd_hbm.at[cs, :], wd_ref.at[cs, 0:M], fsem.at[2]).start()

    def fwait():
        for t, r in enumerate((wg_ref, wu_ref, wd_ref.at[:, 0:M])):
            pltpu.make_async_copy(r, r, fsem.at[t]).wait()

    def proj(src, w, dst, i, scale=None):
        y = jnp.dot(_upk(src), w, preferred_element_type=f32)
        if scale is not None:
            y = y * scale
        for e in range(2):
            dst[e, _rows(i, T2), :] = _pk(y[:, e * D:(e + 1) * D].astype(bf16))

    def pr(ref, e, lo, hi):
        return ref[e, lo // 2:hi // 2, :]

    def nt(a, b):
        return lax.dot_general(_upk(a), _upk(b), NT, preferred_element_type=f32)

    def iota2():
        return lax.broadcasted_iota(i32, (GR, 128), 0), lax.broadcasted_iota(i32, (GR, 128), 1)

    def causal_tri():
        row, col = iota2()
        return col <= row + (128 - GR)

    def qunit(I, e, c):
        return _cat([pr(q_ref, e, r, r + GR) for r in range(I * TB + GR * c, (I + 1) * TB, 128)], 0)

    def left(I, e, c):
        s = GR * (c + 1)
        st = nt(pr(k_ref, e, 0, s), qunit(I, e, c))
        t = jnp.concatenate([st, jnp.full((128 - s, 128), NEG, f32)], axis=0).T
        if I == 0:
            row, col = iota2()
            t = jnp.concatenate([jnp.where(col <= row + GR * c, t[:GR], NEG), t[GR:]], axis=0)
        return t

    def qk(I, e, c, tri, lf):
        r0 = I * TB
        s = GR * (c + 1)
        q = qunit(I, e, c)
        if s == 128:
            mn = nt(q, pr(k_ref, e, 0, r0 + 128))
        else:
            mn = _cat([lf] + ([nt(q, pr(k_ref, e, s, r0 + s))] if r0 else []), 1)
        ex = [nt(q[x * GR // 2:], pr(k_ref, e, r0 + s + 128 * (x - 1), r0 + s + 128 * x)) for x in range(1, NC)]
        out = []
        for a in range(NC):
            sa = _cat([mn[a * GR:(a + 1) * GR]]
                      + [ex[x - 1][(a - x) * GR:(a - x + 1) * GR] for x in range(1, a + 1)], 1)
            w = sa.shape[1]
            if not (s < 128 and w == 128):
                sa = _cat(([sa[:, :w - 128]] if w > 128 else []) + [jnp.where(tri, sa[:, w - 128:], NEG)], 1)
            out.append(jnp.exp2(sa - jnp.max(sa, axis=1, keepdims=True)))
        return out

    def pv(I, e, c, p, nv):
        r0 = I * TB
        s = GR * (c + 1)
        w0 = r0 + 128
        vpu = c < nv
        if s == 128:
            vm = [pr(v_ref, e, 0, w0)]
        else:
            vm = ([] if vpu else [pr(v_ref, e, 0, 128)]) + ([pr(v_ref, e, s, r0 + s)] if r0 else [])
        ctx = None
        if vm:
            pm = _cat([pa[:, 128 * vpu:w0] for pa in p], 0).astype(bf16)
            ctx = jnp.dot(pm, _upk(_cat(vm, 0)), preferred_element_type=f32)
        if vpu:
            v0 = _upk(pr(v_ref, e, 0, s)).astype(f32)
            pp = _pk(_cat([pa[:, :128] for pa in p], 0).astype(bf16))
            acc = None
            for k in range(s):
                t = _upk(jnp.broadcast_to(pp[:, k:k + 1], (64, 128))).astype(f32) * v0[k:k + 1, :]
                acc = t if acc is None else acc + t
            ctx = acc if ctx is None else ctx + acc
        cs = [ctx[a * GR:(a + 1) * GR] for a in range(NC)]
        den = [jnp.sum(pa.astype(bf16).astype(f32), axis=1, keepdims=True) for pa in p]
        for x in range(1, NC):
            px = _cat([p[a][:, w0 + 128 * (x - 1):w0 + 128 * x] for a in range(x, NC)], 0).astype(bf16)
            cx = jnp.dot(px, _upk(pr(v_ref, e, r0 + s + 128 * (x - 1), r0 + s + 128 * x)),
                         preferred_element_type=f32)
            for a in range(x, NC):
                cs[a] = cs[a] + cx[(a - x) * GR:(a - x + 1) * GR]
        return [cs[a] * pl.reciprocal(den[a], approx=False, full_range=False) for a in range(NC)]

    def issue(n, f):
        def body(i, _):
            f(i)
            return 0

        lax.fori_loop(0, n, body, 0)

    HB = NB // 2
    wstart("k", 0, 0)
    wstart("v", 0, 0)
    issue(HB, lambda i: ccopy(i).start())
    wstart("q", 0, 0)
    issue(HB, lambda t: (ccopy(HB + t).start(), xcopy(2 * t).start(), xcopy(2 * t + 1).start()))
    wstart("o", 0, 0)
    for name in "kvq":
        wstart(name, 1, 1)
    rcopy.start()
    z_ref[...] = jnp.zeros((8, 128), u32)
    wwait("k", 0)
    wk0 = _unpack_pair(bk[0])
    wwait("v", 0)
    wv0 = _unpack_pair(bv[0])

    def kv_block(i):
        cpk = _pk(c_ref[_rows(i, TQ), :])
        cp_ref[_rows(i, T2), :] = cpk
        proj(cpk, wk0, k_ref, i)
        proj(cpk, wv0, v_ref, i)

    def ln_block(i):
        xf = x_ref[_rows(i, TQ), :].astype(f32)
        acc_ref[_rows(i, TQ), :] = xf
        d = xf - jnp.sum(xf, axis=-1, keepdims=True) * (1.0 / M)
        inv = lax.rsqrt(jnp.sum(d * d, axis=-1, keepdims=True) * (1.0 / M) + EPS)
        xnp = _pk((d * inv).astype(bf16))
        xn_ref[_rows(i, T2), :] = xnp
        return xnp

    def pro_a(i, _):
        ccopy(i).wait()
        kv_block(i)
        return 0

    lax.fori_loop(0, HB, pro_a, 0)
    wwait("q", 0)
    wq0 = _unpack_pair(bq[0])

    def pro_b(t, _):
        ccopy(HB + t).wait()
        xcopy(2 * t).wait()
        xcopy(2 * t + 1).wait()
        xa = ln_block(2 * t)
        xb = ln_block(2 * t + 1)
        kv_block(HB + t)
        proj(xa, wq0, q_ref, 2 * t, QSCALE)
        proj(xb, wq0, q_ref, 2 * t + 1, QSCALE)
        return 0

    lax.fori_loop(0, HB, pro_b, 0)

    def step(p, _):
        s0 = p & 1
        s1 = 1 - s0
        for name in "kvq":
            wwait(name, s1)
        wwait("o", s0)
        ahead = jnp.minimum(p + 2, NP - 1)
        for name in "kvq":
            wstart(name, ahead, s0)
        wstart("o", p + 1, s1)

        @pl.when(p < FCH)
        def _():
            fstart(p)

        tri = causal_tri()
        w = {}

        def weight(name):
            if name not in w:
                b = wtab[name][2]
                w[name] = b[s0].reshape(2 * D, M) if name == "o" else _unpack_pair(b[s1])
            return w[name]

        lfs, ps, ctxs = {}, {}, {}
        for item in _parse(MID):
            op, i, u = item[0], item[1], item[1:]
            if op == "LT":
                lfs[u] = left(*u)
            elif op == "KP":
                proj(cp_ref[_rows(i, T2), :], weight("k"), k_ref, i)
            elif op == "VP":
                proj(cp_ref[_rows(i, T2), :], weight("v"), v_ref, i)
            elif op == "QP":
                proj(xn_ref[_rows(i, T2), :], weight("q"), q_ref, i, QSCALE)
            elif op == "QK":
                ps[u] = qk(*u, tri, lfs.pop(u, None))
            elif op == "PV":
                ctxs[u] = pv(*u, ps.pop(u), 0)
            else:
                I, a0 = divmod(2 * i, NC)
                c2 = jnp.concatenate([_cat([ctxs[I, e, c][a] for a in (a0, a0 + 1) for c in range(NC)], 0)
                                      for e in range(2)], axis=1).astype(bf16)
                acc_ref[_rows(i, TQ), :] += jnp.dot(c2, weight("o"), preferred_element_type=f32)
        return 0

    lax.fori_loop(0, NP - 1, step, 0)

    def last_head(e, _):
        tri = causal_tri()
        lfs, ps = {}, {}
        for op, I, c in _parse(LAST):
            if op == "LT":
                lfs[I, c] = left(I, e, c)
            elif op == "QK":
                ps[I, c] = qk(I, e, c, tri, lfs.pop((I, c), None))
            else:
                for a, ca in enumerate(pv(I, e, c, ps.pop((I, c)), 0)):
                    r = (I * TB + 128 * a + GR * c) // 2
                    ctx_ref[e, r:r + GR // 2, :] = _pk(ca.astype(bf16))
        return 0

    lax.fori_loop(0, 2, last_head, 0)
    wwait("o", (NP - 1) & 1)
    rcopy.wait()
    for name in "kvq":
        wwait(name, NP & 1)
    fwait()
    wr = wr_ref[...].astype(f32).reshape(1, M)
    wo = bo[(NP - 1) & 1].reshape(2 * D, M)

    def out_block(i, dst):
        c2 = _upk(jnp.concatenate([ctx_ref[0, _rows(i, T2), :], ctx_ref[1, _rows(i, T2), :]], axis=1))
        y = dst[...] + jnp.dot(c2, wo, preferred_element_type=f32)
        dst[...] = _rb(y)
        return y

    def epi_block(i, src, top, y=None):
        hh = src[...]
        s = jnp.sum(hh, axis=-1, keepdims=True)
        mrow = _rb(s * (1.0 / M))
        if y is not None:
            z = z_ref[...]
            parts = []
            for g in range(NG):
                t = g * PACE // NG
                yt = y[(t % NG) * 8:(t % NG + 1) * 8, (t // NG) * 256:(t // NG) * 256 + 128]
                mg = jnp.broadcast_to(mrow[g * 8:(g + 1) * 8], (8, 128))
                parts.append(pltpu.bitcast(pltpu.bitcast(mg, u32) | (pltpu.bitcast(yt, u32) & z), f32))
            mrow = jnp.concatenate(parts, axis=0)
        else:
            mrow = jnp.broadcast_to(mrow, (TQ, 128))
        d = hh - _wide(mrow)
        mu = _gather(s) * (1.0 / M)
        dm = mu - _rb(mu)
        var = _gather(jnp.sum(d * d, axis=-1, keepdims=True)) * (1.0 / M) - dm * dm
        sw = _gather(jnp.sum(d * wr, axis=-1, keepdims=True))
        ve = _rb(_rb(jnp.maximum(var, 0.0)) + EPS)
        inv = pl.reciprocal(_rb(ve * lax.rsqrt(ve)), approx=False, full_range=False)
        r = _rb(sw * inv)
        inv_s = _scatter(inv, NG)
        st_ref[0, _rows(i, TQ), :] = inv_s
        st_ref[1, _rows(i, TQ), :] = mrow
        o_ref[_rows(i, TQ), :] = (hh * _wide(inv_s + 1.0) - _wide(mrow * inv_s)).astype(bf16)
        outcopy(i).start()
        b = pltpu.bitcast(r + 0.0, i32)
        code = lax.shift_right_arithmetic(b ^ (lax.shift_right_arithmetic(b, 31) & jnp.int32(0x7FFF0000)), 5)
        lane = lax.broadcasted_iota(i32, (8, 128), 1)
        tok = i * TQ + lane * 8 + lax.broadcasted_iota(i32, (8, 128), 0)
        key = pltpu.bitcast(code + (jnp.int32(0x24000000 + S - 1) - tok), f32)
        key = jnp.where(lane < NG, key, 0.0)
        return jnp.maximum(top[0], key), jnp.maximum(top[1], jnp.minimum(top[0], key))

    out_block(0, acc_ref.at[_rows(0, TQ)])

    def out_epi(j, top):
        v = acc_ref.at[_rows(j, TQ, 2)]
        y = out_block(j + 1, v.at[TQ:2 * TQ])
        return epi_block(j, v.at[0:TQ], top, y)

    lo = jnp.zeros((8, 128), f32)
    top = lax.fori_loop(0, NB - 1, out_epi, (lo, lo))
    t1, t2 = epi_block(NB - 1, acc_ref.at[_rows(NB - 1, TQ)], top)

    def amax(t):
        return jnp.max(jnp.max(t, axis=1, keepdims=True), axis=0, keepdims=True)

    k1 = amax(t1)
    k2 = amax(jnp.where(t1 == k1, t2, t1))
    i1 = (S - 1) - (pltpu.bitcast(k1, i32)[0, 0] & (S - 1))
    i2 = (S - 1) - (pltpu.bitcast(k2, i32)[0, 0] & (S - 1))
    g1 = pl.multiple_of(i1 & ~7, 8)
    g2 = pl.multiple_of(i2 & ~7, 8)

    def two(f):
        return jnp.concatenate([f(pl.ds(g1, 8)), f(pl.ds(g2, 8))], axis=0)

    hh = two(lambda r_: acc_ref[r_, :])
    hnb = (_rb(hh - _wide(two(lambda r_: st_ref[1, r_, :]))) * _wide(two(lambda r_: st_ref[0, r_, :]))).astype(bf16)
    hn = hnb.astype(f32)
    r = _rb(jnp.sum(hn * wr, axis=1, keepdims=True))
    sub = lax.broadcasted_iota(i32, (16, 1), 0)
    tok = jnp.where(sub < 8, g1 + sub, g2 + sub - 8)
    sel = (tok == i1) | (tok == i2)
    g = _rb(jnp.dot(hnb, wg_ref[...], preferred_element_type=f32))
    g = _rb(g * _rb(jax.nn.sigmoid(g)))
    u = _rb(jnp.dot(hnb, wu_ref[...], preferred_element_type=f32))
    y = _rb(jnp.dot((g * u).astype(bf16), wd_ref[:, 0:M], preferred_element_type=f32))
    y = _rb(y * _rb(jax.nn.sigmoid(r)))
    res = (hh + jnp.where(sel, _rb(hn + y), hn)).astype(bf16)
    for i in range(NB):
        outcopy(i).wait()
    o_ref[0:16, :] = res
    cp1 = pltpu.make_async_copy(o_ref.at[0:8], o_hbm.at[pl.ds(g1, 8)], outsem.at[0])
    cp1.start()

    @pl.when(g2 != g1)
    def _():
        cp2 = pltpu.make_async_copy(o_ref.at[8:16], o_hbm.at[pl.ds(g2, 8)], outsem.at[1])
        cp2.start()
        cp2.wait()

    cp1.wait()


@jax.jit
def pallas_sequential_preLN__compressed_kv_cla__moe_arch_mod__prompt_kernel(
    A_x: jax.Array,
    A_c_kv: jax.Array,
    A_w_q: jax.Array,
    A_w_uk: jax.Array,
    A_w_uv: jax.Array,
    A_w_o: jax.Array,
    B_x: jax.Array,
    B_w_r: jax.Array,
    B_w_gate: jax.Array,
    B_w_up: jax.Array,
    B_w_down: jax.Array,
):
    del B_x
    hbm = pl.BlockSpec(memory_space=pl.ANY)
    V = pltpu.VMEM
    DMA = pltpu.SemaphoreType.DMA
    out = pl.pallas_call(
        _kernel,
        in_specs=[hbm] * 10,
        out_specs=hbm,
        out_shape=jax.ShapeDtypeStruct((S, M), bf16),
        scratch_shapes=[
            V((S, M), bf16), V((S, DC), bf16),
            V((S // 2, DC), u32), V((S // 2, M), u32),
            V((S, M), f32), V((S, M), bf16),
            V((2, M // G, 2 * G, D), bf16), V((2, DC // G, 2 * G, D), bf16), V((2, DC // G, 2 * G, D), bf16),
            V((2, 2, D, M), bf16),
            V((2, S // 2, D), u32), V((2, S // 2, D), u32), V((2, S // 2, D), u32), V((2, S // 2, D), u32),
            V((M,), bf16), V((M, F), bf16), V((M, F), bf16),
            V((F, M + 128), bf16),
            V((2, S, 128), f32), V((8, 128), u32),
            DMA((4, 2)), DMA((NB,)), DMA((NB,)), DMA((4,)), DMA((NB,)),
        ],
        compiler_params=pltpu.CompilerParams(vmem_limit_bytes=120 * 1024 * 1024,
                                             disable_bounds_checks=True,
                                             disable_semaphore_checks=True),
    )(A_x.reshape(S, M), A_c_kv.reshape(S, DC), A_w_q.reshape(M // G, G, H, D),
      A_w_uk.reshape(DC // G, G, H, D), A_w_uv.reshape(DC // G, G, H, D), A_w_o,
      B_w_r, B_w_gate, B_w_up, B_w_down)
    return out.reshape(1, S, M)
```

```python
import math

import jax
import jax.numpy as jnp
from jax import lax
from jax.experimental import pallas as pl
from jax.experimental.pallas import tpu as pltpu

S, M, H, D, DC, F = 2048, 1024, 32, 128, 512, 3584
EPS = 1e-5
bf16, f32, u32, i32 = jnp.bfloat16, jnp.float32, jnp.uint32, jnp.int32
NT = (((1,), (1,)), ((), ()))
G = 4
NP = H // 2
TQ = 256
NB = S // TQ
T2 = TQ // 2
NG = TQ // 8
FCH = 14
QSCALE = (D ** -0.5) * math.log2(math.e)
PACE = 72

NEG = -1e30
GR = 16
NC = 128 // GR
TB = 128 * NC
NV = 4
BS = 4

MID = ("LT106 LT105 QK107 LT104 QK106 LT103 LT102 QK105 QK104 LT101 QK103 QK102 PV107 QK101 PV106 LT100 "
       "LT116 QK100 PV105 LT115 QK117 PV104 LT114 QK116 PV103 LT113 QK114 QK115 PV102 LT112 PV101 LT111 "
       "QK113 PV100 LT110 PV115 QK112 PV117 QK111 PV116 LT006 QK110 LT005 QK007 KP7 QP7 PV114 LT004 QK006 "
       "QP6 PV113 LT003 KP6 QK005 PV112 LT002 QK004 QP5 PV111 LT001 QK003 KP5 PV110 LT000 QK002 QP4 PV007 "
       "QK001 KP4 PV006 LT016 QK000 VP7 PV005 LT015 QK017 VP6 QK016 PV004 VP5 LT014 VP4 PV002 LT013 QK015 "
       "PV003 LT012 QK014 OUT7 QK013 OUT6 PV000 LT010 QK012 OUT5 PV001 LT011 PV017 QK011 OUT4 QK010 QP3 "
       "PV015 PV013 PV012 KP3 PV016 KP1 PV014 QP2 PV011 QP1 PV010 KP2 VP2 OUT2 VP3 QP0 OUT3 VP0 KP0 VP1 OUT1 "
       "OUT0")
LAST = ("LT15 LT16 QK17 LT14 QK16 LT13 QK14 LT11 QK15 LT12 PV17 QK13 PV16 LT10 QK11 PV14 QK12 PV15 QK10 LT06 "
       "PV13 LT05 QK07 LT04 PV12 QK06 PV11 QK05 LT03 PV10 LT02 QK04 PV07 LT01 QK03 PV06 LT00 QK02 PV05 QK01 "
       "PV04 QK00 PV03 PV02 PV01 PV00")


def _parse(s):
    out = []
    for t in s.split():
        name = t.rstrip("0123456789")
        out.append((name,) + tuple(int(c) for c in t[len(name):]))
    return out


def _rb(x):
    return x.astype(bf16).astype(f32)


def _pk(x):
    return pltpu.bitcast(x, u32)


def _upk(x):
    return pltpu.bitcast(x, bf16)


def _gather(col):
    n = col.shape[0] // 8
    lane = lax.broadcasted_iota(i32, (8, 128), 1)
    vs = [jnp.broadcast_to(col[g * 8:(g + 1) * 8], (8, 128)) for g in range(n)]
    bit = 1
    while len(vs) > 1:
        m = (lane & bit) != 0
        vs = [jnp.where(m, vs[2 * k + 1], vs[2 * k]) for k in range(len(vs) // 2)]
        bit *= 2
    return vs[0]


def _scatter(dense, n):
    return jnp.concatenate([jnp.broadcast_to(dense[:, g:g + 1], (8, 128)) for g in range(n)], axis=0)


def _wide(v):
    return jnp.concatenate([v] * (M // 128), axis=1)


def _unpack_pair(buf):
    k = buf.shape[0] * G
    w = pltpu.bitcast(buf.reshape(2 * k, D), u32)
    w2 = jnp.concatenate([w << 16, w & jnp.uint32(0xFFFF0000)], axis=1)
    return pltpu.bitcast(w2, f32).astype(bf16)


def _cat(parts, axis):
    return parts[0] if len(parts) == 1 else jnp.concatenate(parts, axis=axis)


def _rows(i, n, k=1):
    return pl.ds(i * n, k * n) if isinstance(i, int) else pl.ds(pl.multiple_of(i * n, n), k * n)


def _kernel(x_hbm, c_hbm, wq_hbm, wk_hbm, wv_hbm, wo_hbm, wr_hbm, wg_hbm, wu_hbm, wd_hbm, o_hbm,
            x_ref, c_ref, cp_ref, xn_ref, acc_ref, o_ref, bq, bk, bv, bo, q_ref, k_ref, v_ref, ctx_ref,
            wr_ref, wg_ref, wu_ref, wd_ref, st_ref, z_ref, wsem, xsem, csem, fsem, outsem):
    wtab = {"k": (0, wk_hbm, bk), "v": (1, wv_hbm, bv), "q": (2, wq_hbm, bq), "o": (3, wo_hbm, bo)}

    def wstart(name, pair, slot):
        t, w, b = wtab[name]
        heads = _rows(pair, 2)
        if name == "o":
            pltpu.make_async_copy(w.at[heads], b.at[slot], wsem.at[t, slot]).start()
        else:
            for g in range(G):
                pltpu.make_async_copy(w.at[:, g, heads, :], b.at[slot, :, pl.ds(2 * g, 2), :],
                                      wsem.at[t, slot]).start()

    def wwait(name, slot):
        t, _, b = wtab[name]
        pltpu.make_async_copy(b.at[slot], b.at[slot], wsem.at[t, slot]).wait()

    def xcopy(i):
        return pltpu.make_async_copy(x_hbm.at[_rows(i, TQ)], x_ref.at[_rows(i, TQ)], xsem.at[i])

    def ccopy(i):
        return pltpu.make_async_copy(c_hbm.at[_rows(i, TQ)], c_ref.at[_rows(i, TQ)], csem.at[i])

    def outcopy(i):
        return pltpu.make_async_copy(o_ref.at[_rows(i, TQ)], o_hbm.at[_rows(i, TQ)], outsem.at[i])

    rcopy = pltpu.make_async_copy(wr_hbm, wr_ref, fsem.at[3])

    def fstart(j):
        cs = _rows(j, F // FCH)
        pltpu.make_async_copy(wg_hbm.at[:, cs], wg_ref.at[:, cs], fsem.at[0]).start()
        pltpu.make_async_copy(wu_hbm.at[:, cs], wu_ref.at[:, cs], fsem.at[1]).start()
        pltpu.make_async_copy(wd_hbm.at[cs, :], wd_ref.at[cs, 0:M], fsem.at[2]).start()

    def fwait():
        for t, r in enumerate((wg_ref, wu_ref, wd_ref.at[:, 0:M])):
            pltpu.make_async_copy(r, r, fsem.at[t]).wait()

    def proj(src, w, dst, i, scale=None):
        y = jnp.dot(_upk(src), w, preferred_element_type=f32)
        if scale is not None:
            y = y * scale
        for e in range(2):
            dst[e, _rows(i, T2), :] = _pk(y[:, e * D:(e + 1) * D].astype(bf16))

    def pr(ref, e, lo, hi):
        return ref[e, lo // 2:hi // 2, :]

    def nt(a, b):
        return lax.dot_general(_upk(a), _upk(b), NT, preferred_element_type=f32)

    def iota2():
        return lax.broadcasted_iota(i32, (GR, 128), 0), lax.broadcasted_iota(i32, (GR, 128), 1)

    def causal_tri():
        row, col = iota2()
        return col <= row + (128 - GR)

    def qunit(I, e, c):
        return _cat([pr(q_ref, e, r, r + GR) for r in range(I * TB + GR * c, (I + 1) * TB, 128)], 0)

    def period(c):
        return 1 << (GR * (c + 1) - 1).bit_length()

    def left(I, e, c, nv):
        s = GR * (c + 1)
        per = period(c) if c < nv else 128
        st = nt(pr(k_ref, e, 0, s), qunit(I, e, c))
        pad = [jnp.full((per - s, 128), NEG, f32)] if per > s else []
        t = jnp.concatenate(([st] + pad) * (128 // per), axis=0).T
        if I == 0:
            row, col = iota2()
            t = jnp.concatenate([jnp.where((col & (per - 1)) <= row + GR * c, t[:GR], NEG), t[GR:]], axis=0)
        return t

    def qk(I, e, c, tri, lf):
        r0 = I * TB
        s = GR * (c + 1)
        q = qunit(I, e, c)
        if s == 128:
            mn = nt(q, pr(k_ref, e, 0, r0 + 128))
        else:
            mn = _cat([lf] + ([nt(q, pr(k_ref, e, s, r0 + s))] if r0 else []), 1)
        ex = [nt(q[x * GR // 2:], pr(k_ref, e, r0 + s + 128 * (x - 1), r0 + s + 128 * x)) for x in range(1, NC)]
        out = []
        for a in range(NC):
            sa = _cat([mn[a * GR:(a + 1) * GR]]
                      + [ex[x - 1][(a - x) * GR:(a - x + 1) * GR] for x in range(1, a + 1)], 1)
            w = sa.shape[1]
            if not (s < 128 and w == 128):
                sa = _cat(([sa[:, :w - 128]] if w > 128 else []) + [jnp.where(tri, sa[:, w - 128:], NEG)], 1)
            out.append(jnp.exp2(sa - jnp.max(sa, axis=1, keepdims=True)))
        return out

    def skewed_v(e, per):
        w = _upk(pr(v_ref, e, 0, per)).astype(f32)
        lane = lax.broadcasted_iota(i32, (per, 128), 1)
        bit = 1
        while bit < per:
            w = jnp.where((lane & bit) != 0, pltpu.roll(w, per - bit, 0), w)
            bit *= 2
        return [w[0:BS]] + [pltpu.roll(w[r // 8 * 8:r // 8 * 8 + 8], r, 1)[r % 8:r % 8 + BS]
                            for r in range(BS, per, BS)]

    def pv(I, e, c, p, nv, skew):
        r0 = I * TB
        s = GR * (c + 1)
        w0 = r0 + 128
        vpu = c < nv
        if s == 128:
            vm = [pr(v_ref, e, 0, w0)]
        else:
            vm = ([] if vpu else [pr(v_ref, e, 0, 128)]) + ([pr(v_ref, e, s, r0 + s)] if r0 else [])
        cs = [None] * NC
        if vm:
            pm = _cat([pa[:, 128 * vpu:w0] for pa in p], 0).astype(bf16)
            ctx = jnp.dot(pm, _upk(_cat(vm, 0)), preferred_element_type=f32)
            cs = [ctx[a * GR:(a + 1) * GR] for a in range(NC)]
        if vpu:
            per = period(c)
            if (e, per) not in skew:
                skew[e, per] = skewed_v(e, per)
            pl0 = _cat([pa[:, :128] for pa in p], 0)
            baby = [pl0] + [pltpu.roll(pl0, 128 - b, 1) for b in range(1, BS)]
            acc = None
            for w in reversed(skew[e, per]):
                if acc is not None:
                    acc = pltpu.roll(acc, 128 - BS, 1)
                for b in range(BS):
                    t = baby[b] * w[b:b + 1, :]
                    acc = t if acc is None else acc + t
            once = iota2()[1] < s
            p = [_cat([jnp.where(once, pa[:, :128], 0.0)] + ([pa[:, 128:]] if pa.shape[1] > 128 else []), 1)
                 for pa in p]
        den = [jnp.sum(pa.astype(bf16).astype(f32), axis=1, keepdims=True) for pa in p]
        for x in range(1, NC):
            px = _cat([p[a][:, w0 + 128 * (x - 1):w0 + 128 * x] for a in range(x, NC)], 0).astype(bf16)
            cx = jnp.dot(px, _upk(pr(v_ref, e, r0 + s + 128 * (x - 1), r0 + s + 128 * x)),
                         preferred_element_type=f32)
            for a in range(x, NC):
                t = cx[(a - x) * GR:(a - x + 1) * GR]
                cs[a] = t if cs[a] is None else cs[a] + t
        if vpu:
            cs = [acc[a * GR:(a + 1) * GR] if cs[a] is None else cs[a] + acc[a * GR:(a + 1) * GR]
                  for a in range(NC)]
        return [cs[a] * pl.reciprocal(den[a], approx=False, full_range=False) for a in range(NC)]

    def issue(n, f):
        def body(i, _):
            f(i)
            return 0

        lax.fori_loop(0, n, body, 0)

    HB = NB // 2
    wstart("k", 0, 0)
    wstart("v", 0, 0)
    issue(HB, lambda i: ccopy(i).start())
    wstart("q", 0, 0)
    issue(HB, lambda t: (ccopy(HB + t).start(), xcopy(2 * t).start(), xcopy(2 * t + 1).start()))
    wstart("o", 0, 0)
    for name in "kvq":
        wstart(name, 1, 1)
    rcopy.start()
    z_ref[...] = jnp.zeros((8, 128), u32)
    wwait("k", 0)
    wk0 = _unpack_pair(bk[0])
    wwait("v", 0)
    wv0 = _unpack_pair(bv[0])

    def kv_block(i):
        cpk = _pk(c_ref[_rows(i, TQ), :])
        cp_ref[_rows(i, T2), :] = cpk
        proj(cpk, wk0, k_ref, i)
        proj(cpk, wv0, v_ref, i)

    def ln_block(i):
        xf = x_ref[_rows(i, TQ), :].astype(f32)
        acc_ref[_rows(i, TQ), :] = xf
        d = xf - jnp.sum(xf, axis=-1, keepdims=True) * (1.0 / M)
        inv = lax.rsqrt(jnp.sum(d * d, axis=-1, keepdims=True) * (1.0 / M) + EPS)
        xnp = _pk((d * inv).astype(bf16))
        xn_ref[_rows(i, T2), :] = xnp
        return xnp

    def pro_a(i, _):
        ccopy(i).wait()
        kv_block(i)
        return 0

    lax.fori_loop(0, HB, pro_a, 0)
    wwait("q", 0)
    wq0 = _unpack_pair(bq[0])

    def pro_b(t, _):
        ccopy(HB + t).wait()
        xcopy(2 * t).wait()
        xcopy(2 * t + 1).wait()
        xa = ln_block(2 * t)
        xb = ln_block(2 * t + 1)
        kv_block(HB + t)
        proj(xa, wq0, q_ref, 2 * t, QSCALE)
        proj(xb, wq0, q_ref, 2 * t + 1, QSCALE)
        return 0

    lax.fori_loop(0, HB, pro_b, 0)

    def step(p, _):
        s0 = p & 1
        s1 = 1 - s0
        for name in "kvq":
            wwait(name, s1)
        wwait("o", s0)
        ahead = jnp.minimum(p + 2, NP - 1)
        for name in "kvq":
            wstart(name, ahead, s0)
        wstart("o", p + 1, s1)

        @pl.when(p < FCH)
        def _():
            fstart(p)

        tri = causal_tri()
        w = {}

        def weight(name):
            if name not in w:
                b = wtab[name][2]
                w[name] = b[s0].reshape(2 * D, M) if name == "o" else _unpack_pair(b[s1])
            return w[name]

        lfs, ps, ctxs, skew = {}, {}, {}, {}
        for item in _parse(MID):
            op, i, u = item[0], item[1], item[1:]
            if op == "LT":
                lfs[u] = left(*u, NV)
            elif op == "KP":
                proj(cp_ref[_rows(i, T2), :], weight("k"), k_ref, i)
            elif op == "VP":
                proj(cp_ref[_rows(i, T2), :], weight("v"), v_ref, i)
            elif op == "QP":
                proj(xn_ref[_rows(i, T2), :], weight("q"), q_ref, i, QSCALE)
            elif op == "QK":
                ps[u] = qk(*u, tri, lfs.pop(u, None))
            elif op == "PV":
                ctxs[u] = pv(*u, ps.pop(u), NV, skew)
            else:
                I, a0 = divmod(2 * i, NC)
                c2 = jnp.concatenate([_cat([ctxs[I, e, c][a] for a in (a0, a0 + 1) for c in range(NC)], 0)
                                      for e in range(2)], axis=1).astype(bf16)
                acc_ref[_rows(i, TQ), :] += jnp.dot(c2, weight("o"), preferred_element_type=f32)
        return 0

    lax.fori_loop(0, NP - 1, step, 0)

    def last_head(e, _):
        tri = causal_tri()
        lfs, ps = {}, {}
        for op, I, c in _parse(LAST):
            if op == "LT":
                lfs[I, c] = left(I, e, c, 0)
            elif op == "QK":
                ps[I, c] = qk(I, e, c, tri, lfs.pop((I, c), None))
            else:
                for a, ca in enumerate(pv(I, e, c, ps.pop((I, c)), 0, None)):
                    r = (I * TB + 128 * a + GR * c) // 2
                    ctx_ref[e, r:r + GR // 2, :] = _pk(ca.astype(bf16))
        return 0

    lax.fori_loop(0, 2, last_head, 0)
    wwait("o", (NP - 1) & 1)
    rcopy.wait()
    for name in "kvq":
        wwait(name, NP & 1)
    fwait()
    wr = wr_ref[...].astype(f32).reshape(1, M)
    wo = bo[(NP - 1) & 1].reshape(2 * D, M)

    def out_block(i, dst):
        c2 = _upk(jnp.concatenate([ctx_ref[0, _rows(i, T2), :], ctx_ref[1, _rows(i, T2), :]], axis=1))
        y = dst[...] + jnp.dot(c2, wo, preferred_element_type=f32)
        dst[...] = _rb(y)
        return y

    def epi_block(i, src, top, y=None):
        hh = src[...]
        s = jnp.sum(hh, axis=-1, keepdims=True)
        mrow = _rb(s * (1.0 / M))
        if y is not None:
            z = z_ref[...]
            parts = []
            for g in range(NG):
                t = g * PACE // NG
                yt = y[(t % NG) * 8:(t % NG + 1) * 8, (t // NG) * 256:(t // NG) * 256 + 128]
                mg = jnp.broadcast_to(mrow[g * 8:(g + 1) * 8], (8, 128))
                parts.append(pltpu.bitcast(pltpu.bitcast(mg, u32) | (pltpu.bitcast(yt, u32) & z), f32))
            mrow = jnp.concatenate(parts, axis=0)
        else:
            mrow = jnp.broadcast_to(mrow, (TQ, 128))
        d = hh - _wide(mrow)
        mu = _gather(s) * (1.0 / M)
        dm = mu - _rb(mu)
        var = _gather(jnp.sum(d * d, axis=-1, keepdims=True)) * (1.0 / M) - dm * dm
        sw = _gather(jnp.sum(d * wr, axis=-1, keepdims=True))
        ve = _rb(_rb(jnp.maximum(var, 0.0)) + EPS)
        inv = pl.reciprocal(_rb(ve * lax.rsqrt(ve)), approx=False, full_range=False)
        r = _rb(sw * inv)
        inv_s = _scatter(inv, NG)
        st_ref[0, _rows(i, TQ), :] = inv_s
        st_ref[1, _rows(i, TQ), :] = mrow
        o_ref[_rows(i, TQ), :] = (hh * _wide(inv_s + 1.0) - _wide(mrow * inv_s)).astype(bf16)
        outcopy(i).start()
        b = pltpu.bitcast(r + 0.0, i32)
        code = lax.shift_right_arithmetic(b ^ (lax.shift_right_arithmetic(b, 31) & jnp.int32(0x7FFF0000)), 5)
        lane = lax.broadcasted_iota(i32, (8, 128), 1)
        tok = i * TQ + lane * 8 + lax.broadcasted_iota(i32, (8, 128), 0)
        key = pltpu.bitcast(code + (jnp.int32(0x24000000 + S - 1) - tok), f32)
        key = jnp.where(lane < NG, key, 0.0)
        return jnp.maximum(top[0], key), jnp.maximum(top[1], jnp.minimum(top[0], key))

    out_block(0, acc_ref.at[_rows(0, TQ)])

    def out_epi(j, top):
        v = acc_ref.at[_rows(j, TQ, 2)]
        y = out_block(j + 1, v.at[TQ:2 * TQ])
        return epi_block(j, v.at[0:TQ], top, y)

    lo = jnp.zeros((8, 128), f32)
    top = lax.fori_loop(0, NB - 1, out_epi, (lo, lo))
    t1, t2 = epi_block(NB - 1, acc_ref.at[_rows(NB - 1, TQ)], top)

    def amax(t):
        return jnp.max(jnp.max(t, axis=1, keepdims=True), axis=0, keepdims=True)

    k1 = amax(t1)
    k2 = amax(jnp.where(t1 == k1, t2, t1))
    i1 = (S - 1) - (pltpu.bitcast(k1, i32)[0, 0] & (S - 1))
    i2 = (S - 1) - (pltpu.bitcast(k2, i32)[0, 0] & (S - 1))
    g1 = pl.multiple_of(i1 & ~7, 8)
    g2 = pl.multiple_of(i2 & ~7, 8)

    def two(f):
        return jnp.concatenate([f(pl.ds(g1, 8)), f(pl.ds(g2, 8))], axis=0)

    hh = two(lambda r_: acc_ref[r_, :])
    hnb = (_rb(hh - _wide(two(lambda r_: st_ref[1, r_, :]))) * _wide(two(lambda r_: st_ref[0, r_, :]))).astype(bf16)
    hn = hnb.astype(f32)
    r = _rb(jnp.sum(hn * wr, axis=1, keepdims=True))
    sub = lax.broadcasted_iota(i32, (16, 1), 0)
    tok = jnp.where(sub < 8, g1 + sub, g2 + sub - 8)
    sel = (tok == i1) | (tok == i2)
    g = _rb(jnp.dot(hnb, wg_ref[...], preferred_element_type=f32))
    g = _rb(g * _rb(jax.nn.sigmoid(g)))
    u = _rb(jnp.dot(hnb, wu_ref[...], preferred_element_type=f32))
    y = _rb(jnp.dot((g * u).astype(bf16), wd_ref[:, 0:M], preferred_element_type=f32))
    y = _rb(y * _rb(jax.nn.sigmoid(r)))
    res = (hh + jnp.where(sel, _rb(hn + y), hn)).astype(bf16)
    for i in range(NB):
        outcopy(i).wait()
    o_ref[0:16, :] = res
    cp1 = pltpu.make_async_copy(o_ref.at[0:8], o_hbm.at[pl.ds(g1, 8)], outsem.at[0])
    cp1.start()

    @pl.when(g2 != g1)
    def _():
        cp2 = pltpu.make_async_copy(o_ref.at[8:16], o_hbm.at[pl.ds(g2, 8)], outsem.at[1])
        cp2.start()
        cp2.wait()

    cp1.wait()


@jax.jit
def pallas_sequential_preLN__compressed_kv_cla__moe_arch_mod__prompt_kernel(
    A_x: jax.Array,
    A_c_kv: jax.Array,
    A_w_q: jax.Array,
    A_w_uk: jax.Array,
    A_w_uv: jax.Array,
    A_w_o: jax.Array,
    B_x: jax.Array,
    B_w_r: jax.Array,
    B_w_gate: jax.Array,
    B_w_up: jax.Array,
    B_w_down: jax.Array,
):
    del B_x
    hbm = pl.BlockSpec(memory_space=pl.ANY)
    V = pltpu.VMEM
    DMA = pltpu.SemaphoreType.DMA
    out = pl.pallas_call(
        _kernel,
        in_specs=[hbm] * 10,
        out_specs=hbm,
        out_shape=jax.ShapeDtypeStruct((S, M), bf16),
        scratch_shapes=[
            V((S, M), bf16), V((S, DC), bf16),
            V((S // 2, DC), u32), V((S // 2, M), u32),
            V((S, M), f32), V((S, M), bf16),
            V((2, M // G, 2 * G, D), bf16), V((2, DC // G, 2 * G, D), bf16), V((2, DC // G, 2 * G, D), bf16),
            V((2, 2, D, M), bf16),
            V((2, S // 2, D), u32), V((2, S // 2, D), u32), V((2, S // 2, D), u32), V((2, S // 2, D), u32),
            V((M,), bf16), V((M, F), bf16), V((M, F), bf16),
            V((F, M + 128), bf16),
            V((2, S, 128), f32), V((8, 128), u32),
            DMA((4, 2)), DMA((NB,)), DMA((NB,)), DMA((4,)), DMA((NB,)),
        ],
        compiler_params=pltpu.CompilerParams(vmem_limit_bytes=120 * 1024 * 1024,
                                             disable_bounds_checks=True,
                                             disable_semaphore_checks=True),
    )(A_x.reshape(S, M), A_c_kv.reshape(S, DC), A_w_q.reshape(M // G, G, H, D),
      A_w_uk.reshape(DC // G, G, H, D), A_w_uv.reshape(DC // G, G, H, D), A_w_o,
      B_w_r, B_w_gate, B_w_up, B_w_down)
    return out.reshape(1, S, M)
```

```python
import math

import jax
import jax.numpy as jnp
from jax import lax
from jax.experimental import pallas as pl
from jax.experimental.pallas import tpu as pltpu

S, M, H, D, DC, F = 2048, 1024, 32, 128, 512, 3584
EPS = 1e-5
bf16, f32, u32, i32 = jnp.bfloat16, jnp.float32, jnp.uint32, jnp.int32
NT = (((1,), (1,)), ((), ()))
G = 4
NP = H // 2
TQ = 256
NB = S // TQ
T2 = TQ // 2
NG = TQ // 8
FCH = 14
QSCALE = (D ** -0.5) * math.log2(math.e)
PACE = 72

NEG = -1e30
GR = 16
NC = 128 // GR
TB = 128 * NC
NV = 4
BS = 4

MID = ("LT105 LT106 QK107 LT104 QK106 QK105 QK104 LT101 LT103 LT102 QK103 QK102 PV107 QK101 LT100 LT116 "
       "QK100 PV105 PV106 LT115 QK117 QK115 PV104 LT114 QK116 PV102 PV103 LT113 QK114 LT112 PV101 LT111 "
       "QK113 PV100 LT110 PV115 QK112 PV117 QK111 LT006 QK110 PV116 LT005 QK007 KP7 QP7 PV114 LT004 QK006 "
       "QP6 LT003 KP6 QK005 PV112 LT002 QK004 PV113 QP5 PV111 LT001 QK003 KP5 PV110 QK002 QP4 PV007 QK001 "
       "KP4 PV006 LT000 LT016 QK000 VP7 PV005 QK017 LT015 VP6 QK016 PV004 VP5 LT014 VP4 PV002 LT013 QK015 "
       "PV003 LT012 QK014 OUT7 QK013 OUT6 PV000 LT010 QK012 OUT5 PV001 LT011 PV017 QK011 OUT4 QK010 QP3 "
       "PV015 PV013 PV012 KP3 KP1 PV016 PV014 PV011 QP1 PV010 KP2 OUT2 VP3 QP0 QP2 VP2 OUT3 VP0 VP1 OUT1 "
       "OUT0 KP0")
LAST = ("LT15 LT16 QK17 LT14 QK16 LT13 QK14 LT11 QK15 LT12 PV17 QK13 PV16 LT10 QK11 PV14 QK12 PV15 QK10 LT06 "
       "PV13 LT05 QK07 LT04 PV12 QK06 PV11 QK05 LT03 PV10 LT02 QK04 PV07 LT01 QK03 PV06 LT00 QK02 PV05 QK01 "
       "PV04 QK00 PV03 PV02 PV01 PV00")


def _parse(s):
    out = []
    for t in s.split():
        name = t.rstrip("0123456789")
        out.append((name,) + tuple(int(c) for c in t[len(name):]))
    return out


def _rb(x):
    return x.astype(bf16).astype(f32)


def _pk(x):
    return pltpu.bitcast(x, u32)


def _upk(x):
    return pltpu.bitcast(x, bf16)


def _gather(col):
    n = col.shape[0] // 8
    lane = lax.broadcasted_iota(i32, (8, 128), 1)
    vs = [jnp.broadcast_to(col[g * 8:(g + 1) * 8], (8, 128)) for g in range(n)]
    bit = 1
    while len(vs) > 1:
        m = (lane & bit) != 0
        vs = [jnp.where(m, vs[2 * k + 1], vs[2 * k]) for k in range(len(vs) // 2)]
        bit *= 2
    return vs[0]


def _scatter(dense, n):
    return jnp.concatenate([jnp.broadcast_to(dense[:, g:g + 1], (8, 128)) for g in range(n)], axis=0)


def _wide(v):
    return jnp.concatenate([v] * (M // 128), axis=1)


def _unpack_pair(buf):
    k = buf.shape[0] * G
    w = pltpu.bitcast(buf.reshape(2 * k, D), u32)
    w2 = jnp.concatenate([w << 16, w & jnp.uint32(0xFFFF0000)], axis=1)
    return pltpu.bitcast(w2, f32).astype(bf16)


def _cat(parts, axis):
    return parts[0] if len(parts) == 1 else jnp.concatenate(parts, axis=axis)


def _rows(i, n, k=1):
    return pl.ds(i * n, k * n) if isinstance(i, int) else pl.ds(pl.multiple_of(i * n, n), k * n)


def _kernel(x_hbm, c_hbm, wq_hbm, wk_hbm, wv_hbm, wo_hbm, wr_hbm, wg_hbm, wu_hbm, wd_hbm, o_hbm,
            x_ref, c_ref, cp_ref, xn_ref, acc_ref, o_ref, bq, bk, bv, bo, q_ref, k_ref, v_ref, ctx_ref,
            wr_ref, wg_ref, wu_ref, wd_ref, st_ref, z_ref, wsem, xsem, csem, fsem, outsem):
    wtab = {"k": (0, wk_hbm, bk), "v": (1, wv_hbm, bv), "q": (2, wq_hbm, bq), "o": (3, wo_hbm, bo)}

    def wstart(name, pair, slot):
        t, w, b = wtab[name]
        heads = _rows(pair, 2)
        if name == "o":
            pltpu.make_async_copy(w.at[heads], b.at[slot], wsem.at[t, slot]).start()
        else:
            for g in range(G):
                pltpu.make_async_copy(w.at[:, g, heads, :], b.at[slot, :, pl.ds(2 * g, 2), :],
                                      wsem.at[t, slot]).start()

    def wwait(name, slot):
        t, _, b = wtab[name]
        pltpu.make_async_copy(b.at[slot], b.at[slot], wsem.at[t, slot]).wait()

    def xcopy(i):
        return pltpu.make_async_copy(x_hbm.at[_rows(i, TQ)], x_ref.at[_rows(i, TQ)], xsem.at[i])

    def ccopy(i):
        return pltpu.make_async_copy(c_hbm.at[_rows(i, TQ)], c_ref.at[_rows(i, TQ)], csem.at[i])

    def outcopy(i):
        return pltpu.make_async_copy(o_ref.at[_rows(i, TQ)], o_hbm.at[_rows(i, TQ)], outsem.at[i])

    rcopy = pltpu.make_async_copy(wr_hbm, wr_ref, fsem.at[3])

    def fstart(j):
        cs = _rows(j, F // FCH)
        pltpu.make_async_copy(wg_hbm.at[:, cs], wg_ref.at[:, cs], fsem.at[0]).start()
        pltpu.make_async_copy(wu_hbm.at[:, cs], wu_ref.at[:, cs], fsem.at[1]).start()
        pltpu.make_async_copy(wd_hbm.at[cs, :], wd_ref.at[cs, 0:M], fsem.at[2]).start()

    def fwait():
        for t, r in enumerate((wg_ref, wu_ref, wd_ref.at[:, 0:M])):
            pltpu.make_async_copy(r, r, fsem.at[t]).wait()

    def proj(src, w, dst, i, scale=None):
        y = jnp.dot(_upk(src), w, preferred_element_type=f32)
        if scale is not None:
            y = y * scale
        for e in range(2):
            dst[e, _rows(i, src.shape[0]), :] = _pk(y[:, e * D:(e + 1) * D].astype(bf16))

    def pr(ref, e, lo, hi):
        return ref[e, lo // 2:hi // 2, :]

    def nt(a, b):
        return lax.dot_general(_upk(a), _upk(b), NT, preferred_element_type=f32)

    def iota2():
        return lax.broadcasted_iota(i32, (GR, 128), 0), lax.broadcasted_iota(i32, (GR, 128), 1)

    def causal_tri():
        row, col = iota2()
        return col <= row + (128 - GR)

    def qunit(I, e, c):
        return _cat([pr(q_ref, e, r, r + GR) for r in range(I * TB + GR * c, (I + 1) * TB, 128)], 0)

    def period(c):
        return 1 << (GR * (c + 1) - 1).bit_length()

    def left(I, e, c, nv):
        s = GR * (c + 1)
        per = period(c) if c < nv else 128
        st = nt(pr(k_ref, e, 0, s), qunit(I, e, c))
        pad = [jnp.full((per - s, 128), NEG, f32)] if per > s else []
        t = jnp.concatenate(([st] + pad) * (128 // per), axis=0).T
        if I == 0:
            row, col = iota2()
            t = jnp.concatenate([jnp.where((col & (per - 1)) <= row + GR * c, t[:GR], NEG), t[GR:]], axis=0)
        return t

    def qk(I, e, c, tri, lf):
        r0 = I * TB
        s = GR * (c + 1)
        q = qunit(I, e, c)
        if s == 128:
            mn = nt(q, pr(k_ref, e, 0, r0 + 128))
        else:
            mn = _cat([lf] + ([nt(q, pr(k_ref, e, s, r0 + s))] if r0 else []), 1)
        ex = [nt(q[x * GR // 2:], pr(k_ref, e, r0 + s + 128 * (x - 1), r0 + s + 128 * x)) for x in range(1, NC)]
        out = []
        for a in range(NC):
            sa = _cat([mn[a * GR:(a + 1) * GR]]
                      + [ex[x - 1][(a - x) * GR:(a - x + 1) * GR] for x in range(1, a + 1)], 1)
            w = sa.shape[1]
            if not (s < 128 and w == 128):
                sa = _cat(([sa[:, :w - 128]] if w > 128 else []) + [jnp.where(tri, sa[:, w - 128:], NEG)], 1)
            out.append(jnp.exp2(sa - jnp.max(sa, axis=1, keepdims=True)))
        return out

    def skewed_v(e, per):
        w = _upk(pr(v_ref, e, 0, per)).astype(f32)
        lane = lax.broadcasted_iota(i32, (per, 128), 1)
        bit = 1
        while bit < per:
            w = jnp.where((lane & bit) != 0, pltpu.roll(w, per - bit, 0), w)
            bit *= 2
        return [w[0:BS]] + [pltpu.roll(w[r // 8 * 8:r // 8 * 8 + 8], r, 1)[r % 8:r % 8 + BS]
                            for r in range(BS, per, BS)]

    def pv(I, e, c, p, nv, skew):
        r0 = I * TB
        s = GR * (c + 1)
        w0 = r0 + 128
        vpu = c < nv
        if s == 128:
            vm = [pr(v_ref, e, 0, w0)]
        else:
            vm = ([] if vpu else [pr(v_ref, e, 0, 128)]) + ([pr(v_ref, e, s, r0 + s)] if r0 else [])
        cs = [None] * NC
        if vm:
            pm = _cat([pa[:, 128 * vpu:w0] for pa in p], 0).astype(bf16)
            ctx = jnp.dot(pm, _upk(_cat(vm, 0)), preferred_element_type=f32)
            cs = [ctx[a * GR:(a + 1) * GR] for a in range(NC)]
        if vpu:
            per = period(c)
            if (e, per) not in skew:
                skew[e, per] = skewed_v(e, per)
            pl0 = _cat([pa[:, :128] for pa in p], 0)
            baby = [pl0] + [pltpu.roll(pl0, 128 - b, 1) for b in range(1, BS)]
            acc = None
            for w in reversed(skew[e, per]):
                if acc is not None:
                    acc = pltpu.roll(acc, 128 - BS, 1)
                for b in range(BS):
                    t = baby[b] * w[b:b + 1, :]
                    acc = t if acc is None else acc + t
            once = iota2()[1] < s
            p = [_cat([jnp.where(once, pa[:, :128], 0.0)] + ([pa[:, 128:]] if pa.shape[1] > 128 else []), 1)
                 for pa in p]
        den = [jnp.sum(pa.astype(bf16).astype(f32), axis=1, keepdims=True) for pa in p]
        for x in range(1, NC):
            px = _cat([p[a][:, w0 + 128 * (x - 1):w0 + 128 * x] for a in range(x, NC)], 0).astype(bf16)
            cx = jnp.dot(px, _upk(pr(v_ref, e, r0 + s + 128 * (x - 1), r0 + s + 128 * x)),
                         preferred_element_type=f32)
            for a in range(x, NC):
                t = cx[(a - x) * GR:(a - x + 1) * GR]
                cs[a] = t if cs[a] is None else cs[a] + t
        if vpu:
            cs = [acc[a * GR:(a + 1) * GR] if cs[a] is None else cs[a] + acc[a * GR:(a + 1) * GR]
                  for a in range(NC)]
        return [cs[a] * pl.reciprocal(den[a], approx=False, full_range=False) for a in range(NC)]

    def issue(n, f):
        def body(i, _):
            f(i)
            return 0

        lax.fori_loop(0, n, body, 0)

    HB = NB // 2
    wstart("k", 0, 0)
    wstart("v", 0, 0)
    issue(HB, lambda i: ccopy(i).start())
    wstart("q", 0, 0)
    issue(HB, lambda t: (ccopy(HB + t).start(), xcopy(2 * t).start(), xcopy(2 * t + 1).start()))
    wstart("o", 0, 0)
    for name in "kvq":
        wstart(name, 1, 1)
    rcopy.start()
    z_ref[...] = jnp.zeros((8, 128), u32)
    wwait("k", 0)
    wk0 = _unpack_pair(bk[0])
    wwait("v", 0)
    wv0 = _unpack_pair(bv[0])

    def pack_c(i):
        cpk = _pk(c_ref[_rows(i, TQ), :])
        cp_ref[_rows(i, T2), :] = cpk
        return cpk

    def ln_block(i):
        xf = x_ref[_rows(i, TQ), :].astype(f32)
        acc_ref[_rows(i, TQ), :] = xf
        d = xf - jnp.sum(xf, axis=-1, keepdims=True) * (1.0 / M)
        inv = lax.rsqrt(jnp.sum(d * d, axis=-1, keepdims=True) * (1.0 / M) + EPS)
        xnp = _pk((d * inv).astype(bf16))
        xn_ref[_rows(i, T2), :] = xnp
        return xnp

    def pro_a(i, _):
        ccopy(i).wait()
        cpk = pack_c(i)
        proj(cpk, wk0, k_ref, i)
        proj(cpk, wv0, v_ref, i)
        return 0

    lax.fori_loop(0, HB, pro_a, 0)
    wwait("q", 0)
    wq0 = _unpack_pair(bq[0])

    def pro_b(t, _):
        ccopy(HB + t).wait()
        xcopy(2 * t).wait()
        xcopy(2 * t + 1).wait()
        xs = [ln_block(2 * t), ln_block(2 * t + 1)]
        cpk = pack_c(HB + t)
        for j, (w, dst) in enumerate(((wk0, k_ref), (wv0, v_ref))):
            proj(cpk, w, dst, HB + t)
            for n in range(4):
                proj(xs[j][n * 32:(n + 1) * 32], wq0, q_ref, (2 * t + j) * 4 + n, QSCALE)
        return 0

    lax.fori_loop(0, HB, pro_b, 0)

    def step(p, _):
        s0 = p & 1
        s1 = 1 - s0
        for name in "kvq":
            wwait(name, s1)
        wwait("o", s0)
        ahead = jnp.minimum(p + 2, NP - 1)
        for name in "kvq":
            wstart(name, ahead, s0)
        wstart("o", p + 1, s1)

        @pl.when(p < FCH)
        def _():
            fstart(p)

        tri = causal_tri()
        w = {}

        def weight(name):
            if name not in w:
                b = wtab[name][2]
                w[name] = b[s0].reshape(2 * D, M) if name == "o" else _unpack_pair(b[s1])
            return w[name]

        lfs, ps, ctxs, skew = {}, {}, {}, {}
        for item in _parse(MID):
            op, i, u = item[0], item[1], item[1:]
            if op == "LT":
                lfs[u] = left(*u, NV)
            elif op == "KP":
                proj(cp_ref[_rows(i, T2), :], weight("k"), k_ref, i)
            elif op == "VP":
                proj(cp_ref[_rows(i, T2), :], weight("v"), v_ref, i)
            elif op == "QP":
                proj(xn_ref[_rows(i, T2), :], weight("q"), q_ref, i, QSCALE)
            elif op == "QK":
                ps[u] = qk(*u, tri, lfs.pop(u, None))
            elif op == "PV":
                ctxs[u] = pv(*u, ps.pop(u), NV, skew)
            else:
                I, a0 = divmod(2 * i, NC)
                c2 = jnp.concatenate([_cat([ctxs[I, e, c][a] for a in (a0, a0 + 1) for c in range(NC)], 0)
                                      for e in range(2)], axis=1).astype(bf16)
                acc_ref[_rows(i, TQ), :] += jnp.dot(c2, weight("o"), preferred_element_type=f32)
        return 0

    lax.fori_loop(0, NP - 1, step, 0)

    def last_head(e, _):
        tri = causal_tri()
        lfs, ps = {}, {}
        for op, I, c in _parse(LAST):
            if op == "LT":
                lfs[I, c] = left(I, e, c, 0)
            elif op == "QK":
                ps[I, c] = qk(I, e, c, tri, lfs.pop((I, c), None))
            else:
                for a, ca in enumerate(pv(I, e, c, ps.pop((I, c)), 0, None)):
                    r = (I * TB + 128 * a + GR * c) // 2
                    ctx_ref[e, r:r + GR // 2, :] = _pk(ca.astype(bf16))
        return 0

    lax.fori_loop(0, 2, last_head, 0)
    wwait("o", (NP - 1) & 1)
    rcopy.wait()
    for name in "kvq":
        wwait(name, NP & 1)
    fwait()
    wr = wr_ref[...].astype(f32).reshape(1, M)
    wo = bo[(NP - 1) & 1].reshape(2 * D, M)

    def out_block(i, dst):
        c2 = _upk(jnp.concatenate([ctx_ref[0, _rows(i, T2), :], ctx_ref[1, _rows(i, T2), :]], axis=1))
        y = dst[...] + jnp.dot(c2, wo, preferred_element_type=f32)
        dst[...] = _rb(y)
        return y

    def epi_block(i, src, top, y=None):
        hh = src[...]
        s = jnp.sum(hh, axis=-1, keepdims=True)
        mrow = _rb(s * (1.0 / M))
        if y is not None:
            z = z_ref[...]
            parts = []
            for g in range(NG):
                t = g * PACE // NG
                yt = y[(t % NG) * 8:(t % NG + 1) * 8, (t // NG) * 256:(t // NG) * 256 + 128]
                mg = jnp.broadcast_to(mrow[g * 8:(g + 1) * 8], (8, 128))
                parts.append(pltpu.bitcast(pltpu.bitcast(mg, u32) | (pltpu.bitcast(yt, u32) & z), f32))
            mrow = jnp.concatenate(parts, axis=0)
        else:
            mrow = jnp.broadcast_to(mrow, (TQ, 128))
        d = hh - _wide(mrow)
        mu = _gather(s) * (1.0 / M)
        dm = mu - _rb(mu)
        var = _gather(jnp.sum(d * d, axis=-1, keepdims=True)) * (1.0 / M) - dm * dm
        sw = _gather(jnp.sum(d * wr, axis=-1, keepdims=True))
        ve = _rb(_rb(jnp.maximum(var, 0.0)) + EPS)
        inv = pl.reciprocal(_rb(ve * lax.rsqrt(ve)), approx=False, full_range=False)
        r = _rb(sw * inv)
        inv_s = _scatter(inv, NG)
        st_ref[0, _rows(i, TQ), :] = inv_s
        st_ref[1, _rows(i, TQ), :] = mrow
        o_ref[_rows(i, TQ), :] = (hh * _wide(inv_s + 1.0) - _wide(mrow * inv_s)).astype(bf16)
        outcopy(i).start()
        b = pltpu.bitcast(r + 0.0, i32)
        code = lax.shift_right_arithmetic(b ^ (lax.shift_right_arithmetic(b, 31) & jnp.int32(0x7FFF0000)), 5)
        lane = lax.broadcasted_iota(i32, (8, 128), 1)
        tok = i * TQ + lane * 8 + lax.broadcasted_iota(i32, (8, 128), 0)
        key = pltpu.bitcast(code + (jnp.int32(0x24000000 + S - 1) - tok), f32)
        key = jnp.where(lane < NG, key, 0.0)
        return jnp.maximum(top[0], key), jnp.maximum(top[1], jnp.minimum(top[0], key))

    out_block(0, acc_ref.at[_rows(0, TQ)])

    def out_epi(j, top):
        v = acc_ref.at[_rows(j, TQ, 2)]
        y = out_block(j + 1, v.at[TQ:2 * TQ])
        return epi_block(j, v.at[0:TQ], top, y)

    lo = jnp.zeros((8, 128), f32)
    top = lax.fori_loop(0, NB - 1, out_epi, (lo, lo))
    t1, t2 = epi_block(NB - 1, acc_ref.at[_rows(NB - 1, TQ)], top)

    def amax(t):
        return jnp.max(jnp.max(t, axis=1, keepdims=True), axis=0, keepdims=True)

    k1 = amax(t1)
    k2 = amax(jnp.where(t1 == k1, t2, t1))
    i1 = (S - 1) - (pltpu.bitcast(k1, i32)[0, 0] & (S - 1))
    i2 = (S - 1) - (pltpu.bitcast(k2, i32)[0, 0] & (S - 1))
    g1 = pl.multiple_of(i1 & ~7, 8)
    g2 = pl.multiple_of(i2 & ~7, 8)

    def two(f):
        return jnp.concatenate([f(pl.ds(g1, 8)), f(pl.ds(g2, 8))], axis=0)

    hh = two(lambda r_: acc_ref[r_, :])
    hnb = (_rb(hh - _wide(two(lambda r_: st_ref[1, r_, :]))) * _wide(two(lambda r_: st_ref[0, r_, :]))).astype(bf16)
    hn = hnb.astype(f32)
    r = _rb(jnp.sum(hn * wr, axis=1, keepdims=True))
    sub = lax.broadcasted_iota(i32, (16, 1), 0)
    tok = jnp.where(sub < 8, g1 + sub, g2 + sub - 8)
    sel = (tok == i1) | (tok == i2)
    g = _rb(jnp.dot(hnb, wg_ref[...], preferred_element_type=f32))
    g = _rb(g * _rb(jax.nn.sigmoid(g)))
    u = _rb(jnp.dot(hnb, wu_ref[...], preferred_element_type=f32))
    y = _rb(jnp.dot((g * u).astype(bf16), wd_ref[:, 0:M], preferred_element_type=f32))
    y = _rb(y * _rb(jax.nn.sigmoid(r)))
    res = (hh + jnp.where(sel, _rb(hn + y), hn)).astype(bf16)
    for i in range(NB):
        outcopy(i).wait()
    o_ref[0:16, :] = res
    cp1 = pltpu.make_async_copy(o_ref.at[0:8], o_hbm.at[pl.ds(g1, 8)], outsem.at[0])
    cp1.start()

    @pl.when(g2 != g1)
    def _():
        cp2 = pltpu.make_async_copy(o_ref.at[8:16], o_hbm.at[pl.ds(g2, 8)], outsem.at[1])
        cp2.start()
        cp2.wait()

    cp1.wait()


@jax.jit
def pallas_sequential_preLN__compressed_kv_cla__moe_arch_mod__prompt_kernel(
    A_x: jax.Array,
    A_c_kv: jax.Array,
    A_w_q: jax.Array,
    A_w_uk: jax.Array,
    A_w_uv: jax.Array,
    A_w_o: jax.Array,
    B_x: jax.Array,
    B_w_r: jax.Array,
    B_w_gate: jax.Array,
    B_w_up: jax.Array,
    B_w_down: jax.Array,
):
    del B_x
    hbm = pl.BlockSpec(memory_space=pl.ANY)
    V = pltpu.VMEM
    DMA = pltpu.SemaphoreType.DMA
    out = pl.pallas_call(
        _kernel,
        in_specs=[hbm] * 10,
        out_specs=hbm,
        out_shape=jax.ShapeDtypeStruct((S, M), bf16),
        scratch_shapes=[
            V((S, M), bf16), V((S, DC), bf16),
            V((S // 2, DC), u32), V((S // 2, M), u32),
            V((S, M), f32), V((S, M), bf16),
            V((2, M // G, 2 * G, D), bf16), V((2, DC // G, 2 * G, D), bf16), V((2, DC // G, 2 * G, D), bf16),
            V((2, 2, D, M), bf16),
            V((2, S // 2, D), u32), V((2, S // 2, D), u32), V((2, S // 2, D), u32), V((2, S // 2, D), u32),
            V((M,), bf16), V((M, F), bf16), V((M, F), bf16),
            V((F, M + 128), bf16),
            V((2, S, 128), f32), V((8, 128), u32),
            DMA((4, 2)), DMA((NB,)), DMA((NB,)), DMA((4,)), DMA((NB,)),
        ],
        compiler_params=pltpu.CompilerParams(vmem_limit_bytes=120 * 1024 * 1024,
                                             disable_bounds_checks=True,
                                             disable_semaphore_checks=True),
    )(A_x.reshape(S, M), A_c_kv.reshape(S, DC), A_w_q.reshape(M // G, G, H, D),
      A_w_uk.reshape(DC // G, G, H, D), A_w_uv.reshape(DC // G, G, H, D), A_w_o,
      B_w_r, B_w_gate, B_w_up, B_w_down)
    return out.reshape(1, S, M)
```

```python
import math

import jax
import jax.numpy as jnp
from jax import lax
from jax.experimental import pallas as pl
from jax.experimental.pallas import tpu as pltpu

S, M, H, D, DC, F = 2048, 1024, 32, 128, 512, 3584
EPS = 1e-5
bf16, f32, u32, i32 = jnp.bfloat16, jnp.float32, jnp.uint32, jnp.int32
NT = (((1,), (1,)), ((), ()))
G = 4
NP = H // 2
TQ = 256
NB = S // TQ
T2 = TQ // 2
NG = TQ // 8
FCH = 14
QSCALE = (D ** -0.5) * math.log2(math.e)
PACE = 72

NEG = -1e30
GR = 16
NC = 128 // GR
TB = 128 * NC
NV = 4
BS = 4

MID = ("LT105 LT106 QK107 LT104 QK106 QK105 QK104 LT101 LT103 LT102 QK103 QK102 PV107 QK101 LT100 LT116 "
       "QK100 PV105 PV106 LT115 QK117 QK115 PV104 LT114 QK116 PV102 PV103 LT113 QK114 LT112 PV101 LT111 "
       "QK113 PV100 LT110 PV115 QK112 PV117 QK111 LT006 QK110 PV116 LT005 QK007 KP7 QP7 PV114 LT004 QK006 "
       "QP6 LT003 KP6 QK005 PV112 LT002 QK004 PV113 QP5 PV111 LT001 QK003 KP5 PV110 QK002 QP4 PV007 QK001 "
       "KP4 PV006 LT000 LT016 QK000 VP7 PV005 QK017 LT015 VP6 QK016 PV004 VP5 LT014 VP4 PV002 LT013 QK015 "
       "PV003 LT012 QK014 OUT7 QK013 OUT6 PV000 LT010 QK012 OUT5 PV001 LT011 PV017 QK011 OUT4 QK010 QP3 "
       "PV015 PV013 PV012 KP3 KP1 PV016 PV014 PV011 QP1 PV010 KP2 OUT2 VP3 QP0 QP2 VP2 OUT3 VP0 VP1 OUT1 "
       "OUT0 KP0")
LAST = ("LT15 LT16 QK17 LT14 QK16 LT13 QK14 LT11 QK15 LT12 PV17 QK13 PV16 LT10 QK11 PV14 QK12 PV15 QK10 LT06 "
       "PV13 LT05 QK07 LT04 PV12 QK06 PV11 QK05 LT03 PV10 LT02 QK04 PV07 LT01 QK03 PV06 LT00 QK02 PV05 QK01 "
       "PV04 QK00 PV03 PV02 PV01 PV00")


def _parse(s):
    out = []
    for t in s.split():
        name = t.rstrip("0123456789")
        out.append((name,) + tuple(int(c) for c in t[len(name):]))
    return out


def _rb(x):
    return x.astype(bf16).astype(f32)


def _pk(x):
    return pltpu.bitcast(x, u32)


def _upk(x):
    return pltpu.bitcast(x, bf16)


def _gather(col):
    n = col.shape[0] // 8
    lane = lax.broadcasted_iota(i32, (8, 128), 1)
    vs = [jnp.broadcast_to(col[g * 8:(g + 1) * 8], (8, 128)) for g in range(n)]
    bit = 1
    while len(vs) > 1:
        m = (lane & bit) != 0
        vs = [jnp.where(m, vs[2 * k + 1], vs[2 * k]) for k in range(len(vs) // 2)]
        bit *= 2
    return vs[0]


def _scatter(dense, n):
    return jnp.concatenate([jnp.broadcast_to(dense[:, g:g + 1], (8, 128)) for g in range(n)], axis=0)


def _wide(v):
    return jnp.concatenate([v] * (M // 128), axis=1)


def _unpack_pair(buf):
    k = buf.shape[0] * G
    w = pltpu.bitcast(buf.reshape(2 * k, D), u32)
    w2 = jnp.concatenate([w << 16, w & jnp.uint32(0xFFFF0000)], axis=1)
    return pltpu.bitcast(w2, f32).astype(bf16)


def _cat(parts, axis):
    return parts[0] if len(parts) == 1 else jnp.concatenate(parts, axis=axis)


def _rows(i, n, k=1):
    return pl.ds(i * n, k * n) if isinstance(i, int) else pl.ds(pl.multiple_of(i * n, n), k * n)


def _kernel(x_hbm, c_hbm, wq_hbm, wk_hbm, wv_hbm, wo_hbm, wr_hbm, wg_hbm, wu_hbm, wd_hbm, o_hbm,
            x_ref, c_ref, cp_ref, xn_ref, acc_ref, o_ref, bq, bk, bv, bo, q_ref, k_ref, v_ref, ctx_ref,
            wr_ref, wg_ref, wu_ref, wd_ref, st_ref, z_ref, wsem, xsem, csem, fsem, outsem):
    wtab = {"k": (0, wk_hbm, bk), "v": (1, wv_hbm, bv), "q": (2, wq_hbm, bq), "o": (3, wo_hbm, bo)}

    def wstart(name, pair, slot):
        t, w, b = wtab[name]
        heads = _rows(pair, 2)
        if name == "o":
            pltpu.make_async_copy(w.at[heads], b.at[slot], wsem.at[t, slot]).start()
        else:
            for g in range(G):
                pltpu.make_async_copy(w.at[:, g, heads, :], b.at[slot, :, pl.ds(2 * g, 2), :],
                                      wsem.at[t, slot]).start()

    def wwait(name, slot):
        t, _, b = wtab[name]
        pltpu.make_async_copy(b.at[slot], b.at[slot], wsem.at[t, slot]).wait()

    def xcopy(i):
        return pltpu.make_async_copy(x_hbm.at[_rows(i, TQ)], x_ref.at[_rows(i, TQ)], xsem.at[i])

    def ccopy(i):
        return pltpu.make_async_copy(c_hbm.at[_rows(i, TQ)], c_ref.at[_rows(i, TQ)], csem.at[i])

    def outcopy(i):
        return pltpu.make_async_copy(o_ref.at[_rows(i, TQ)], o_hbm.at[_rows(i, TQ)], outsem.at[i])

    rcopy = pltpu.make_async_copy(wr_hbm, wr_ref, fsem.at[3])

    def fstart(j):
        cs = _rows(j, F // FCH)
        pltpu.make_async_copy(wg_hbm.at[:, cs], wg_ref.at[:, cs], fsem.at[0]).start()
        pltpu.make_async_copy(wu_hbm.at[:, cs], wu_ref.at[:, cs], fsem.at[1]).start()
        pltpu.make_async_copy(wd_hbm.at[cs, :], wd_ref.at[cs, 0:M], fsem.at[2]).start()

    def fwait():
        for t, r in enumerate((wg_ref, wu_ref, wd_ref.at[:, 0:M])):
            pltpu.make_async_copy(r, r, fsem.at[t]).wait()

    def proj(src, w, dst, i, scale=None):
        y = jnp.dot(_upk(src), w, preferred_element_type=f32)
        if scale is not None:
            y = y * scale
        for e in range(2):
            dst[e, _rows(i, src.shape[0]), :] = _pk(y[:, e * D:(e + 1) * D].astype(bf16))

    def pr(ref, e, lo, hi):
        return ref[e, lo // 2:hi // 2, :]

    def nt(a, b):
        return lax.dot_general(_upk(a), _upk(b), NT, preferred_element_type=f32)

    def iota2():
        return lax.broadcasted_iota(i32, (GR, 128), 0), lax.broadcasted_iota(i32, (GR, 128), 1)

    def causal_tri():
        row, col = iota2()
        return col <= row + (128 - GR)

    def qunit(I, e, c):
        return _cat([pr(q_ref, e, r, r + GR) for r in range(I * TB + GR * c, (I + 1) * TB, 128)], 0)

    def period(c):
        return 1 << (GR * (c + 1) - 1).bit_length()

    def left(I, e, c, nv):
        s = GR * (c + 1)
        per = period(c) if c < nv else 128
        st = nt(pr(k_ref, e, 0, s), qunit(I, e, c))
        pad = [jnp.full((per - s, 128), NEG, f32)] if per > s else []
        t = jnp.concatenate(([st] + pad) * (128 // per), axis=0).T
        if I == 0:
            row, col = iota2()
            t = jnp.concatenate([jnp.where((col & (per - 1)) <= row + GR * c, t[:GR], NEG), t[GR:]], axis=0)
        return t

    def qk(I, e, c, tri, lf):
        r0 = I * TB
        s = GR * (c + 1)
        q = qunit(I, e, c)
        if s == 128:
            mn = nt(q, pr(k_ref, e, 0, r0 + 128))
        else:
            mn = _cat([lf] + ([nt(q, pr(k_ref, e, s, r0 + s))] if r0 else []), 1)
        ex = [nt(q[x * GR // 2:], pr(k_ref, e, r0 + s + 128 * (x - 1), r0 + s + 128 * x)) for x in range(1, NC)]
        out = []
        for a in range(NC):
            sa = _cat([mn[a * GR:(a + 1) * GR]]
                      + [ex[x - 1][(a - x) * GR:(a - x + 1) * GR] for x in range(1, a + 1)], 1)
            w = sa.shape[1]
            if not (s < 128 and w == 128):
                sa = _cat(([sa[:, :w - 128]] if w > 128 else []) + [jnp.where(tri, sa[:, w - 128:], NEG)], 1)
            out.append(jnp.exp2(sa - jnp.max(sa, axis=1, keepdims=True)))
        return out

    def skewed_v(e, per):
        w = _upk(pr(v_ref, e, 0, per)).astype(f32)
        lane = lax.broadcasted_iota(i32, (per, 128), 1)
        bit = 1
        while bit < per:
            w = jnp.where((lane & bit) != 0, pltpu.roll(w, per - bit, 0), w)
            bit *= 2
        return [w[0:BS]] + [pltpu.roll(w[r // 8 * 8:r // 8 * 8 + 8], r, 1)[r % 8:r % 8 + BS]
                            for r in range(BS, per, BS)]

    def pv(I, e, c, p, nv, skew):
        r0 = I * TB
        s = GR * (c + 1)
        w0 = r0 + 128
        vpu = c < nv
        if s == 128:
            vm = [pr(v_ref, e, 0, w0)]
        else:
            vm = ([] if vpu else [pr(v_ref, e, 0, 128)]) + ([pr(v_ref, e, s, r0 + s)] if r0 else [])
        cs = [None] * NC
        if vm:
            pm = _cat([pa[:, 128 * vpu:w0] for pa in p], 0).astype(bf16)
            ctx = jnp.dot(pm, _upk(_cat(vm, 0)), preferred_element_type=f32)
            cs = [ctx[a * GR:(a + 1) * GR] for a in range(NC)]
        if vpu:
            per = period(c)
            if (e, per) not in skew:
                skew[e, per] = skewed_v(e, per)
            pl0 = _cat([pa[:, :128] for pa in p], 0)
            baby = [pl0] + [pltpu.roll(pl0, 128 - b, 1) for b in range(1, BS)]
            acc = None
            for w in reversed(skew[e, per]):
                if acc is not None:
                    acc = pltpu.roll(acc, 128 - BS, 1)
                for b in range(BS):
                    t = baby[b] * w[b:b + 1, :]
                    acc = t if acc is None else acc + t
            once = iota2()[1] < s
            p = [_cat([jnp.where(once, pa[:, :128], 0.0)] + ([pa[:, 128:]] if pa.shape[1] > 128 else []), 1)
                 for pa in p]
        den = [jnp.sum(pa.astype(bf16).astype(f32), axis=1, keepdims=True) for pa in p]
        for x in range(1, NC):
            px = _cat([p[a][:, w0 + 128 * (x - 1):w0 + 128 * x] for a in range(x, NC)], 0).astype(bf16)
            cx = jnp.dot(px, _upk(pr(v_ref, e, r0 + s + 128 * (x - 1), r0 + s + 128 * x)),
                         preferred_element_type=f32)
            for a in range(x, NC):
                t = cx[(a - x) * GR:(a - x + 1) * GR]
                cs[a] = t if cs[a] is None else cs[a] + t
        if vpu:
            cs = [acc[a * GR:(a + 1) * GR] if cs[a] is None else cs[a] + acc[a * GR:(a + 1) * GR]
                  for a in range(NC)]
        return [cs[a] * pl.reciprocal(den[a], approx=False, full_range=False) for a in range(NC)]

    def issue(n, f):
        def body(i, _):
            f(i)
            return 0

        lax.fori_loop(0, n, body, 0)

    HB = NB // 2
    wstart("k", 0, 0)
    wstart("v", 0, 0)
    issue(HB, lambda i: ccopy(i).start())
    wstart("q", 0, 0)
    issue(HB, lambda t: (ccopy(HB + t).start(), xcopy(2 * t).start(), xcopy(2 * t + 1).start()))
    wstart("o", 0, 0)
    for name in "kvq":
        wstart(name, 1, 1)
    rcopy.start()
    z_ref[...] = jnp.zeros((8, 128), u32)
    wwait("k", 0)
    wk0 = _unpack_pair(bk[0])
    wwait("v", 0)
    wv0 = _unpack_pair(bv[0])

    def pack_c(i):
        cpk = _pk(c_ref[_rows(i, TQ), :])
        cp_ref[_rows(i, T2), :] = cpk
        return cpk

    def ln_block(i):
        xf = x_ref[_rows(i, TQ), :].astype(f32)
        acc_ref[_rows(i, TQ), :] = xf
        d = xf - jnp.sum(xf, axis=-1, keepdims=True) * (1.0 / M)
        inv = lax.rsqrt(jnp.sum(d * d, axis=-1, keepdims=True) * (1.0 / M) + EPS)
        xnp = _pk((d * inv).astype(bf16))
        xn_ref[_rows(i, T2), :] = xnp
        return xnp

    def pro_a(i, _):
        ccopy(i).wait()
        cpk = pack_c(i)
        proj(cpk, wk0, k_ref, i)
        proj(cpk, wv0, v_ref, i)
        return 0

    lax.fori_loop(0, HB, pro_a, 0)
    wwait("q", 0)
    wq0 = _unpack_pair(bq[0])

    def pro_b(t, _):
        ccopy(HB + t).wait()
        xcopy(2 * t).wait()
        xcopy(2 * t + 1).wait()
        xs = [ln_block(2 * t), ln_block(2 * t + 1)]
        cpk = pack_c(HB + t)
        for j, (w, dst) in enumerate(((wk0, k_ref), (wv0, v_ref))):
            proj(cpk, w, dst, HB + t)
            for n in range(4):
                proj(xs[j][n * 32:(n + 1) * 32], wq0, q_ref, (2 * t + j) * 4 + n, QSCALE)
        return 0

    lax.fori_loop(0, HB, pro_b, 0)

    def step(p, _):
        s0 = p & 1
        s1 = 1 - s0
        for name in "kvq":
            wwait(name, s1)
        wwait("o", s0)
        ahead = jnp.minimum(p + 2, NP - 1)
        for name in "kvq":
            wstart(name, ahead, s0)
        wstart("o", p + 1, s1)

        @pl.when(p < FCH)
        def _():
            fstart(p)

        tri = causal_tri()
        w = {}

        def weight(name):
            if name not in w:
                b = wtab[name][2]
                w[name] = b[s0].reshape(2 * D, M) if name == "o" else _unpack_pair(b[s1])
            return w[name]

        lfs, ps, ctxs, skew = {}, {}, {}, {}
        for item in _parse(MID):
            op, i, u = item[0], item[1], item[1:]
            if op == "LT":
                lfs[u] = left(*u, NV)
            elif op == "KP":
                proj(cp_ref[_rows(i, T2), :], weight("k"), k_ref, i)
            elif op == "VP":
                proj(cp_ref[_rows(i, T2), :], weight("v"), v_ref, i)
            elif op == "QP":
                proj(xn_ref[_rows(i, T2), :], weight("q"), q_ref, i, QSCALE)
            elif op == "QK":
                ps[u] = qk(*u, tri, lfs.pop(u, None))
            elif op == "PV":
                ctxs[u] = pv(*u, ps.pop(u), NV, skew)
            else:
                I, a0 = divmod(2 * i, NC)
                c2 = jnp.concatenate([_cat([ctxs[I, e, c][a] for a in (a0, a0 + 1) for c in range(NC)], 0)
                                      for e in range(2)], axis=1).astype(bf16)
                acc_ref[_rows(i, TQ), :] += jnp.dot(c2, weight("o"), preferred_element_type=f32)
        return 0

    lax.fori_loop(0, NP - 1, step, 0)

    def last_head(e, _):
        tri = causal_tri()
        lfs, ps = {}, {}
        for op, I, c in _parse(LAST):
            if op == "LT":
                lfs[I, c] = left(I, e, c, 0)
            elif op == "QK":
                ps[I, c] = qk(I, e, c, tri, lfs.pop((I, c), None))
            else:
                for a, ca in enumerate(pv(I, e, c, ps.pop((I, c)), 0, None)):
                    r = (I * TB + 128 * a + GR * c) // 2
                    ctx_ref[e, r:r + GR // 2, :] = _pk(ca.astype(bf16))
        return 0

    lax.fori_loop(0, 2, last_head, 0)
    wwait("o", (NP - 1) & 1)
    rcopy.wait()
    for name in "kvq":
        wwait(name, NP & 1)
    fwait()
    wr = wr_ref[...].astype(f32).reshape(1, M)
    wo = bo[(NP - 1) & 1].reshape(2 * D, M)

    def out_block(i, dst):
        c2 = _upk(jnp.concatenate([ctx_ref[0, _rows(i, T2), :], ctx_ref[1, _rows(i, T2), :]], axis=1))
        y = dst[...] + jnp.dot(c2, wo, preferred_element_type=f32)
        dst[...] = _rb(y)
        return y

    def epi_block(i, src, top, y=None):
        hh = src[...]
        s = jnp.sum(hh, axis=-1, keepdims=True)
        mrow = _rb(s * (1.0 / M))
        if y is not None:
            z = z_ref[...]
            parts = []
            for g in range(NG):
                t = g * PACE // NG
                yt = y[(t % NG) * 8:(t % NG + 1) * 8, (t // NG) * 256:(t // NG) * 256 + 128]
                mg = jnp.broadcast_to(mrow[g * 8:(g + 1) * 8], (8, 128))
                parts.append(pltpu.bitcast(pltpu.bitcast(mg, u32) | (pltpu.bitcast(yt, u32) & z), f32))
            mrow = jnp.concatenate(parts, axis=0)
        else:
            mrow = jnp.broadcast_to(mrow, (TQ, 128))
        d = hh - _wide(mrow)
        mu = _gather(s) * (1.0 / M)
        dm = mu - _rb(mu)
        var = _gather(jnp.sum(d * d, axis=-1, keepdims=True)) * (1.0 / M) - dm * dm
        sw = _gather(jnp.sum(d * wr, axis=-1, keepdims=True))
        ve = _rb(_rb(jnp.maximum(var, 0.0)) + EPS)
        inv = pl.reciprocal(_rb(ve * lax.rsqrt(ve)), approx=False, full_range=False)
        r = _rb(sw * inv)
        inv_s = _scatter(inv, NG)
        st_ref[0, _rows(i, TQ), :] = inv_s
        st_ref[1, _rows(i, TQ), :] = mrow
        o_ref[_rows(i, TQ), :] = (hh * _wide(inv_s + 1.0) - _wide(mrow * inv_s)).astype(bf16)
        outcopy(i).start()
        b = pltpu.bitcast(r + 0.0, i32)
        code = lax.shift_right_arithmetic(b ^ (lax.shift_right_arithmetic(b, 31) & jnp.int32(0x7FFF0000)), 5)
        lane = lax.broadcasted_iota(i32, (8, 128), 1)
        tok = i * TQ + lane * 8 + lax.broadcasted_iota(i32, (8, 128), 0)
        key = pltpu.bitcast(code + (jnp.int32(0x24000000 + S - 1) - tok), f32)
        key = jnp.where(lane < NG, key, 0.0)
        return jnp.maximum(top[0], key), jnp.maximum(top[1], jnp.minimum(top[0], key))

    out_block(0, acc_ref.at[_rows(0, TQ)])

    def out_epi(j, top):
        v = acc_ref.at[_rows(j, TQ, 2)]
        y = out_block(j + 1, v.at[TQ:2 * TQ])
        return epi_block(j, v.at[0:TQ], top, y)

    lo = jnp.zeros((8, 128), f32)
    top = lax.fori_loop(0, NB - 1, out_epi, (lo, lo))
    t1, t2 = epi_block(NB - 1, acc_ref.at[_rows(NB - 1, TQ)], top)

    for sh in (4, 2, 1):
        u1, u2 = pltpu.roll(t1, sh, 0), pltpu.roll(t2, sh, 0)
        t1, t2 = jnp.maximum(t1, u1), jnp.maximum(jnp.maximum(t2, u2), jnp.minimum(t1, u1))
    lane = lax.broadcasted_iota(i32, (8, 128), 1)
    sub8 = lax.broadcasted_iota(i32, (8, 128), 0)
    bit = (lax.shift_right_logical(lane, sub8) & 1) == 1
    m0 = jnp.max(jnp.where(sub8 == 7, t2, jnp.where(bit, 0.0, t1)), axis=1, keepdims=True)
    m1 = jnp.max(jnp.where(sub8 == 7, t2, jnp.where(bit, t1, 0.0)), axis=1, keepdims=True)
    k1 = jnp.maximum(m0, m1)[0:1]
    k2 = jnp.max(jnp.minimum(m0, m1), axis=0, keepdims=True)
    i1 = (S - 1) - (pltpu.bitcast(k1, i32)[0, 0] & (S - 1))
    i2 = (S - 1) - (pltpu.bitcast(k2, i32)[0, 0] & (S - 1))
    g1 = pl.multiple_of(i1 & ~7, 8)
    g2 = pl.multiple_of(i2 & ~7, 8)

    def two(f):
        return jnp.concatenate([f(pl.ds(g1, 8)), f(pl.ds(g2, 8))], axis=0)

    hh = two(lambda r_: acc_ref[r_, :])
    hnb = (_rb(hh - _wide(two(lambda r_: st_ref[1, r_, :]))) * _wide(two(lambda r_: st_ref[0, r_, :]))).astype(bf16)
    hn = hnb.astype(f32)
    r = _rb(jnp.sum(hn * wr, axis=1, keepdims=True))
    sub = lax.broadcasted_iota(i32, (16, 1), 0)
    tok = jnp.where(sub < 8, g1 + sub, g2 + sub - 8)
    sel = (tok == i1) | (tok == i2)
    g = _rb(jnp.dot(hnb, wg_ref[...], preferred_element_type=f32))
    g = _rb(g * _rb(jax.nn.sigmoid(g)))
    u = _rb(jnp.dot(hnb, wu_ref[...], preferred_element_type=f32))
    y = _rb(jnp.dot((g * u).astype(bf16), wd_ref[:, 0:M], preferred_element_type=f32))
    y = _rb(y * _rb(jax.nn.sigmoid(r)))
    res = (hh + jnp.where(sel, _rb(hn + y), hn)).astype(bf16)
    for i in range(NB):
        outcopy(i).wait()
    o_ref[0:16, :] = res
    cp1 = pltpu.make_async_copy(o_ref.at[0:8], o_hbm.at[pl.ds(g1, 8)], outsem.at[0])
    cp1.start()

    @pl.when(g2 != g1)
    def _():
        cp2 = pltpu.make_async_copy(o_ref.at[8:16], o_hbm.at[pl.ds(g2, 8)], outsem.at[1])
        cp2.start()
        cp2.wait()

    cp1.wait()


@jax.jit
def pallas_sequential_preLN__compressed_kv_cla__moe_arch_mod__prompt_kernel(
    A_x: jax.Array,
    A_c_kv: jax.Array,
    A_w_q: jax.Array,
    A_w_uk: jax.Array,
    A_w_uv: jax.Array,
    A_w_o: jax.Array,
    B_x: jax.Array,
    B_w_r: jax.Array,
    B_w_gate: jax.Array,
    B_w_up: jax.Array,
    B_w_down: jax.Array,
):
    del B_x
    hbm = pl.BlockSpec(memory_space=pl.ANY)
    V = pltpu.VMEM
    DMA = pltpu.SemaphoreType.DMA
    out = pl.pallas_call(
        _kernel,
        in_specs=[hbm] * 10,
        out_specs=hbm,
        out_shape=jax.ShapeDtypeStruct((S, M), bf16),
        scratch_shapes=[
            V((S, M), bf16), V((S, DC), bf16),
            V((S // 2, DC), u32), V((S // 2, M), u32),
            V((S, M), f32), V((S, M), bf16),
            V((2, M // G, 2 * G, D), bf16), V((2, DC // G, 2 * G, D), bf16), V((2, DC // G, 2 * G, D), bf16),
            V((2, 2, D, M), bf16),
            V((2, S // 2, D), u32), V((2, S // 2, D), u32), V((2, S // 2, D), u32), V((2, S // 2, D), u32),
            V((M,), bf16), V((M, F), bf16), V((M, F), bf16),
            V((F, M + 128), bf16),
            V((2, S, 128), f32), V((8, 128), u32),
            DMA((4, 2)), DMA((NB,)), DMA((NB,)), DMA((4,)), DMA((NB,)),
        ],
        compiler_params=pltpu.CompilerParams(vmem_limit_bytes=120 * 1024 * 1024,
                                             disable_bounds_checks=True,
                                             disable_semaphore_checks=True),
    )(A_x.reshape(S, M), A_c_kv.reshape(S, DC), A_w_q.reshape(M // G, G, H, D),
      A_w_uk.reshape(DC // G, G, H, D), A_w_uv.reshape(DC // G, G, H, D), A_w_o,
      B_w_r, B_w_gate, B_w_up, B_w_down)
    return out.reshape(1, S, M)
```

```python
import math

import jax
import jax.numpy as jnp
from jax import lax
from jax.experimental import pallas as pl
from jax.experimental.pallas import tpu as pltpu

S, M, H, D, DC, F = 2048, 1024, 32, 128, 512, 3584
EPS = 1e-5
bf16, f32, u32, i32 = jnp.bfloat16, jnp.float32, jnp.uint32, jnp.int32
NT = (((1,), (1,)), ((), ()))
G = 4
NP = H // 2
TQ = 256
NB = S // TQ
T2 = TQ // 2
NG = TQ // 8
FCH = 14
QSCALE = (D ** -0.5) * math.log2(math.e)
PACE = 72

NEG = -1e30
GR = 16
NC = 128 // GR
TB = 128 * NC
NV = 4
BS = 4

MID = ("LT105 LT106 QK107 LT104 QK106 QK105 QK104 LT101 LT103 LT102 QK103 QK102 PV107 QK101 LT100 LT116 "
       "QK100 PV105 PV106 LT115 QK117 QK115 PV104 LT114 QK116 PV102 LT113 QK114 PV103 LT112 PV101 LT111 "
       "QK113 PV100 LT110 PV115 QK112 PV117 QK111 LT006 QK110 PV116 LT005 QK007 KP7 QP7 PV114 LT004 QK006 "
       "QP6 LT003 KP6 QK005 PV112 LT002 LT001 QK003 QK004 PV113 QP5 KP5 PV110 PV111 QK002 QP4 PV007 QK001 "
       "KP4 VP7 PV006 LT000 LT016 QK000 PV005 QK017 LT015 VP6 QK016 PV004 VP5 PV002 LT014 QK015 PV003 LT012 "
       "QK014 OUT7 OUT6 LT013 VP4 QK013 PV000 LT010 QK012 OUT5 PV001 LT011 PV017 QK011 OUT4 QK010 QP3 PV015 "
       "PV012 PV013 KP1 PV016 PV014 PV011 QP1 PV010 KP2 OUT2 KP3 VP3 KP0 QP0 QP2 VP2 VP1 OUT1 OUT3 VP0 OUT0")
LAST = ("LT16 LT15 QK17 LT14 QK16 QK15 QK14 LT13 PV17 LT12 LT11 QK13 PV16 LT10 QK11 QK12 PV14 PV13 LT05 PV15 "
       "QK10 LT06 QK07 LT04 PV12 QK05 QK06 PV11 PV10 LT02 QK04 LT03 PV07 LT01 QK03 LT00 QK02 PV05 PV06 QK01 "
       "PV04 QK00 PV03 PV02 PV00 PV01")


def _parse(s):
    out = []
    for t in s.split():
        name = t.rstrip("0123456789")
        out.append((name,) + tuple(int(c) for c in t[len(name):]))
    return out


def _rb(x):
    return x.astype(bf16).astype(f32)


def _pk(x):
    return pltpu.bitcast(x, u32)


def _upk(x):
    return pltpu.bitcast(x, bf16)


def _gather(col):
    n = col.shape[0] // 8
    lane = lax.broadcasted_iota(i32, (8, 128), 1)
    vs = [jnp.broadcast_to(col[g * 8:(g + 1) * 8], (8, 128)) for g in range(n)]
    bit = 1
    while len(vs) > 1:
        m = (lane & bit) != 0
        vs = [jnp.where(m, vs[2 * k + 1], vs[2 * k]) for k in range(len(vs) // 2)]
        bit *= 2
    return vs[0]


def _scatter(dense, n):
    return jnp.concatenate([jnp.broadcast_to(dense[:, g:g + 1], (8, 128)) for g in range(n)], axis=0)


def _wide(v):
    return jnp.concatenate([v] * (M // 128), axis=1)


def _unpack_pair(buf):
    k = buf.shape[0] * G
    w = pltpu.bitcast(buf.reshape(2 * k, D), u32)
    w2 = jnp.concatenate([w << 16, w & jnp.uint32(0xFFFF0000)], axis=1)
    return pltpu.bitcast(w2, f32).astype(bf16)


def _cat(parts, axis):
    return parts[0] if len(parts) == 1 else jnp.concatenate(parts, axis=axis)


def _rows(i, n, k=1):
    return pl.ds(i * n, k * n) if isinstance(i, int) else pl.ds(pl.multiple_of(i * n, n), k * n)


def _kernel(x_hbm, c_hbm, wq_hbm, wk_hbm, wv_hbm, wo_hbm, wr_hbm, wg_hbm, wu_hbm, wd_hbm, o_hbm,
            x_ref, c_ref, cp_ref, xn_ref, acc_ref, o_ref, bq, bk, bv, bo, q_ref, k_ref, v_ref, ctx_ref,
            wr_ref, wg_ref, wu_ref, wd_ref, st_ref, z_ref, wsem, xsem, csem, fsem, outsem):
    wtab = {"k": (0, wk_hbm, bk), "v": (1, wv_hbm, bv), "q": (2, wq_hbm, bq), "o": (3, wo_hbm, bo)}

    def wstart(name, pair, slot):
        t, w, b = wtab[name]
        heads = _rows(pair, 2)
        if name == "o":
            pltpu.make_async_copy(w.at[heads], b.at[slot], wsem.at[t, slot]).start()
        else:
            for g in range(G):
                pltpu.make_async_copy(w.at[:, g, heads, :], b.at[slot, :, pl.ds(2 * g, 2), :],
                                      wsem.at[t, slot]).start()

    def wwait(name, slot):
        t, _, b = wtab[name]
        pltpu.make_async_copy(b.at[slot], b.at[slot], wsem.at[t, slot]).wait()

    def xcopy(i):
        return pltpu.make_async_copy(x_hbm.at[_rows(i, TQ)], x_ref.at[_rows(i, TQ)], xsem.at[i])

    def ccopy(i):
        return pltpu.make_async_copy(c_hbm.at[_rows(i, TQ)], c_ref.at[_rows(i, TQ)], csem.at[i])

    def outcopy(i):
        return pltpu.make_async_copy(o_ref.at[_rows(i, TQ)], o_hbm.at[_rows(i, TQ)], outsem.at[i])

    rcopy = pltpu.make_async_copy(wr_hbm, wr_ref, fsem.at[3])

    def fstart(j):
        cs = _rows(j, F // FCH)
        pltpu.make_async_copy(wg_hbm.at[:, cs], wg_ref.at[:, cs], fsem.at[0]).start()
        pltpu.make_async_copy(wu_hbm.at[:, cs], wu_ref.at[:, cs], fsem.at[1]).start()
        pltpu.make_async_copy(wd_hbm.at[cs, :], wd_ref.at[cs, 0:M], fsem.at[2]).start()

    def fwait():
        for t, r in enumerate((wg_ref, wu_ref, wd_ref.at[:, 0:M])):
            pltpu.make_async_copy(r, r, fsem.at[t]).wait()

    def proj(src, w, dst, i, scale=None):
        y = jnp.dot(_upk(src), w, preferred_element_type=f32)
        if scale is not None:
            y = y * scale
        for e in range(2):
            dst[e, _rows(i, src.shape[0]), :] = _pk(y[:, e * D:(e + 1) * D].astype(bf16))

    def pr(ref, e, lo, hi):
        return ref[e, lo // 2:hi // 2, :]

    def nt(a, b):
        return lax.dot_general(_upk(a), _upk(b), NT, preferred_element_type=f32)

    def iota2():
        return lax.broadcasted_iota(i32, (GR, 128), 0), lax.broadcasted_iota(i32, (GR, 128), 1)

    def causal_tri():
        row, col = iota2()
        return col <= row + (128 - GR)

    def qunit(I, e, c):
        return _cat([pr(q_ref, e, r, r + GR) for r in range(I * TB + GR * c, (I + 1) * TB, 128)], 0)

    def period(c):
        return 1 << (GR * (c + 1) - 1).bit_length()

    def left(I, e, c, nv):
        s = GR * (c + 1)
        per = period(c) if c < nv else 128
        st = nt(pr(k_ref, e, 0, s), qunit(I, e, c))
        pad = [jnp.full((per - s, 128), NEG, f32)] if per > s else []
        t = jnp.concatenate(([st] + pad) * (128 // per), axis=0).T
        if I == 0:
            row, col = iota2()
            t = jnp.concatenate([jnp.where((col & (per - 1)) <= row + GR * c, t[:GR], NEG), t[GR:]], axis=0)
        return t

    def qk(I, e, c, tri, lf):
        r0 = I * TB
        s = GR * (c + 1)
        q = qunit(I, e, c)
        if s == 128:
            mn = nt(q, pr(k_ref, e, 0, r0 + 128))
        else:
            mn = _cat([lf] + ([nt(q, pr(k_ref, e, s, r0 + s))] if r0 else []), 1)
        ex = [nt(q[x * GR // 2:], pr(k_ref, e, r0 + s + 128 * (x - 1), r0 + s + 128 * x)) for x in range(1, NC)]
        out = []
        for a in range(NC):
            sa = _cat([mn[a * GR:(a + 1) * GR]]
                      + [ex[x - 1][(a - x) * GR:(a - x + 1) * GR] for x in range(1, a + 1)], 1)
            w = sa.shape[1]
            if not (s < 128 and w == 128):
                sa = _cat(([sa[:, :w - 128]] if w > 128 else []) + [jnp.where(tri, sa[:, w - 128:], NEG)], 1)
            out.append(jnp.exp2(sa - jnp.max(sa, axis=1, keepdims=True)))
        return out

    def skewed_v(e, per):
        w = _upk(pr(v_ref, e, 0, per)).astype(f32)
        lane = lax.broadcasted_iota(i32, (per, 128), 1)
        bit = 1
        while bit < per:
            w = jnp.where((lane & bit) != 0, pltpu.roll(w, per - bit, 0), w)
            bit *= 2
        return [w[0:BS]] + [pltpu.roll(w[r // 8 * 8:r // 8 * 8 + 8], r, 1)[r % 8:r % 8 + BS]
                            for r in range(BS, per, BS)]

    def pv(I, e, c, p, nv, skew):
        r0 = I * TB
        s = GR * (c + 1)
        w0 = r0 + 128
        vpu = c < nv
        if s == 128:
            vm = [pr(v_ref, e, 0, w0)]
        else:
            vm = ([] if vpu else [pr(v_ref, e, 0, 128)]) + ([pr(v_ref, e, s, r0 + s)] if r0 else [])
        cs = [None] * NC
        if vm:
            pm = _cat([pa[:, 128 * vpu:w0] for pa in p], 0).astype(bf16)
            ctx = jnp.dot(pm, _upk(_cat(vm, 0)), preferred_element_type=f32)
            cs = [ctx[a * GR:(a + 1) * GR] for a in range(NC)]
        if vpu:
            per = period(c)
            if (e, per) not in skew:
                skew[e, per] = skewed_v(e, per)
            pl0 = _cat([pa[:, :128] for pa in p], 0)
            baby = [pl0] + [pltpu.roll(pl0, 128 - b, 1) for b in range(1, BS)]
            acc = None
            for w in reversed(skew[e, per]):
                if acc is not None:
                    acc = pltpu.roll(acc, 128 - BS, 1)
                for b in range(BS):
                    t = baby[b] * w[b:b + 1, :]
                    acc = t if acc is None else acc + t
            once = iota2()[1] < s
            p = [_cat([jnp.where(once, pa[:, :128], 0.0)] + ([pa[:, 128:]] if pa.shape[1] > 128 else []), 1)
                 for pa in p]
        den = [jnp.sum(pa.astype(bf16).astype(f32), axis=1, keepdims=True) for pa in p]
        for x in range(1, NC):
            px = _cat([p[a][:, w0 + 128 * (x - 1):w0 + 128 * x] for a in range(x, NC)], 0).astype(bf16)
            cx = jnp.dot(px, _upk(pr(v_ref, e, r0 + s + 128 * (x - 1), r0 + s + 128 * x)),
                         preferred_element_type=f32)
            for a in range(x, NC):
                t = cx[(a - x) * GR:(a - x + 1) * GR]
                cs[a] = t if cs[a] is None else cs[a] + t
        if vpu:
            cs = [acc[a * GR:(a + 1) * GR] if cs[a] is None else cs[a] + acc[a * GR:(a + 1) * GR]
                  for a in range(NC)]
        return [cs[a] * pl.reciprocal(den[a], approx=False, full_range=False) for a in range(NC)]

    def issue(n, f):
        def body(i, _):
            f(i)
            return 0

        lax.fori_loop(0, n, body, 0)

    HB = NB // 2
    wstart("k", 0, 0)
    wstart("v", 0, 0)
    issue(HB, lambda i: ccopy(i).start())
    wstart("q", 0, 0)
    issue(HB, lambda t: (ccopy(HB + t).start(), xcopy(2 * t).start(), xcopy(2 * t + 1).start()))
    wstart("o", 0, 0)
    for name in "kvq":
        wstart(name, 1, 1)
    rcopy.start()
    z_ref[...] = jnp.zeros((8, 128), u32)
    wwait("k", 0)
    wk0 = _unpack_pair(bk[0])
    wwait("v", 0)
    wv0 = _unpack_pair(bv[0])

    def pack_c(i):
        cpk = _pk(c_ref[_rows(i, TQ), :])
        cp_ref[_rows(i, T2), :] = cpk
        return cpk

    def ln_block(i):
        xf = x_ref[_rows(i, TQ), :].astype(f32)
        acc_ref[_rows(i, TQ), :] = xf
        d = xf - jnp.sum(xf, axis=-1, keepdims=True) * (1.0 / M)
        inv = lax.rsqrt(jnp.sum(d * d, axis=-1, keepdims=True) * (1.0 / M) + EPS)
        xnp = _pk((d * inv).astype(bf16))
        xn_ref[_rows(i, T2), :] = xnp
        return xnp

    def pro_a(i, _):
        ccopy(i).wait()
        cpk = pack_c(i)
        proj(cpk, wk0, k_ref, i)
        proj(cpk, wv0, v_ref, i)
        return 0

    lax.fori_loop(0, HB, pro_a, 0)
    wwait("q", 0)
    wq0 = _unpack_pair(bq[0])

    def pro_b(t, _):
        ccopy(HB + t).wait()
        xcopy(2 * t).wait()
        xcopy(2 * t + 1).wait()
        xs = [ln_block(2 * t), ln_block(2 * t + 1)]
        cpk = pack_c(HB + t)
        for j, (w, dst) in enumerate(((wk0, k_ref), (wv0, v_ref))):
            proj(cpk, w, dst, HB + t)
            for n in range(4):
                proj(xs[j][n * 32:(n + 1) * 32], wq0, q_ref, (2 * t + j) * 4 + n, QSCALE)
        return 0

    lax.fori_loop(0, HB, pro_b, 0)

    def step(p, _):
        s0 = p & 1
        s1 = 1 - s0
        for name in "kvq":
            wwait(name, s1)
        wwait("o", s0)
        ahead = jnp.minimum(p + 2, NP - 1)
        for name in "kvq":
            wstart(name, ahead, s0)
        wstart("o", p + 1, s1)

        @pl.when(p < FCH)
        def _():
            fstart(p)

        tri = causal_tri()
        w = {}

        def weight(name):
            if name not in w:
                b = wtab[name][2]
                w[name] = b[s0].reshape(2 * D, M) if name == "o" else _unpack_pair(b[s1])
            return w[name]

        lfs, ps, ctxs, skew = {}, {}, {}, {}
        for item in _parse(MID):
            op, i, u = item[0], item[1], item[1:]
            if op == "LT":
                lfs[u] = left(*u, NV)
            elif op == "KP":
                proj(cp_ref[_rows(i, T2), :], weight("k"), k_ref, i)
            elif op == "VP":
                proj(cp_ref[_rows(i, T2), :], weight("v"), v_ref, i)
            elif op == "QP":
                proj(xn_ref[_rows(i, T2), :], weight("q"), q_ref, i, QSCALE)
            elif op == "QK":
                ps[u] = qk(*u, tri, lfs.pop(u, None))
            elif op == "PV":
                ctxs[u] = pv(*u, ps.pop(u), NV, skew)
            else:
                I, a0 = divmod(2 * i, NC)
                c2 = jnp.concatenate([_cat([ctxs[I, e, c][a] for a in (a0, a0 + 1) for c in range(NC)], 0)
                                      for e in range(2)], axis=1).astype(bf16)
                acc_ref[_rows(i, TQ), :] += jnp.dot(c2, weight("o"), preferred_element_type=f32)
        return 0

    lax.fori_loop(0, NP - 1, step, 0)

    def last_head(e, _):
        tri = causal_tri()
        lfs, ps = {}, {}
        for op, I, c in _parse(LAST):
            if op == "LT":
                lfs[I, c] = left(I, e, c, 0)
            elif op == "QK":
                ps[I, c] = qk(I, e, c, tri, lfs.pop((I, c), None))
            else:
                for a, ca in enumerate(pv(I, e, c, ps.pop((I, c)), 0, None)):
                    r = (I * TB + 128 * a + GR * c) // 2
                    ctx_ref[e, r:r + GR // 2, :] = _pk(ca.astype(bf16))
        return 0

    lax.fori_loop(0, 2, last_head, 0)
    wwait("o", (NP - 1) & 1)
    rcopy.wait()
    for name in "kvq":
        wwait(name, NP & 1)
    fwait()
    wr = wr_ref[...].astype(f32).reshape(1, M)
    wo = bo[(NP - 1) & 1].reshape(2 * D, M)

    def out_block(i, dst):
        c2 = _upk(jnp.concatenate([ctx_ref[0, _rows(i, T2), :], ctx_ref[1, _rows(i, T2), :]], axis=1))
        y = dst[...] + jnp.dot(c2, wo, preferred_element_type=f32)
        dst[...] = _rb(y)
        return y

    def epi_block(i, src, top, y=None):
        hh = src[...]
        s = jnp.sum(hh, axis=-1, keepdims=True)
        mrow = _rb(s * (1.0 / M))
        if y is not None:
            z = z_ref[...]
            parts = []
            for g in range(NG):
                t = g * PACE // NG
                yt = y[(t % NG) * 8:(t % NG + 1) * 8, (t // NG) * 256:(t // NG) * 256 + 128]
                mg = jnp.broadcast_to(mrow[g * 8:(g + 1) * 8], (8, 128))
                parts.append(pltpu.bitcast(pltpu.bitcast(mg, u32) | (pltpu.bitcast(yt, u32) & z), f32))
            mrow = jnp.concatenate(parts, axis=0)
        else:
            mrow = jnp.broadcast_to(mrow, (TQ, 128))
        d = hh - _wide(mrow)
        mu = _gather(s) * (1.0 / M)
        dm = mu - _rb(mu)
        var = _gather(jnp.sum(d * d, axis=-1, keepdims=True)) * (1.0 / M) - dm * dm
        sw = _gather(jnp.sum(d * wr, axis=-1, keepdims=True))
        ve = _rb(_rb(jnp.maximum(var, 0.0)) + EPS)
        inv = pl.reciprocal(_rb(ve * lax.rsqrt(ve)), approx=False, full_range=False)
        r = _rb(sw * inv)
        inv_s = _scatter(inv, NG)
        st_ref[0, _rows(i, TQ), :] = inv_s
        st_ref[1, _rows(i, TQ), :] = mrow
        o_ref[_rows(i, TQ), :] = (hh * _wide(inv_s + 1.0) - _wide(mrow * inv_s)).astype(bf16)
        outcopy(i).start()
        b = pltpu.bitcast(r + 0.0, i32)
        code = lax.shift_right_arithmetic(b ^ (lax.shift_right_arithmetic(b, 31) & jnp.int32(0x7FFF0000)), 5)
        lane = lax.broadcasted_iota(i32, (8, 128), 1)
        tok = i * TQ + lane * 8 + lax.broadcasted_iota(i32, (8, 128), 0)
        key = pltpu.bitcast(code + (jnp.int32(0x24000000 + S - 1) - tok), f32)
        key = jnp.where(lane < NG, key, 0.0)
        return jnp.maximum(top[0], key), jnp.maximum(top[1], jnp.minimum(top[0], key))

    out_block(0, acc_ref.at[_rows(0, TQ)])

    def out_epi(j, top):
        v = acc_ref.at[_rows(j, TQ, 2)]
        y = out_block(j + 1, v.at[TQ:2 * TQ])
        return epi_block(j, v.at[0:TQ], top, y)

    lo = jnp.zeros((8, 128), f32)
    top = lax.fori_loop(0, NB - 1, out_epi, (lo, lo))
    t1, t2 = epi_block(NB - 1, acc_ref.at[_rows(NB - 1, TQ)], top)

    for sh in (4, 2, 1):
        u1, u2 = pltpu.roll(t1, sh, 0), pltpu.roll(t2, sh, 0)
        t1, t2 = jnp.maximum(t1, u1), jnp.maximum(jnp.maximum(t2, u2), jnp.minimum(t1, u1))
    lane = lax.broadcasted_iota(i32, (8, 128), 1)
    sub8 = lax.broadcasted_iota(i32, (8, 128), 0)
    bit = (lax.shift_right_logical(lane, sub8) & 1) == 1
    m0 = jnp.max(jnp.where(sub8 == 7, t2, jnp.where(bit, 0.0, t1)), axis=1, keepdims=True)
    m1 = jnp.max(jnp.where(sub8 == 7, t2, jnp.where(bit, t1, 0.0)), axis=1, keepdims=True)
    k1 = jnp.maximum(m0, m1)[0:1]
    k2 = jnp.max(jnp.minimum(m0, m1), axis=0, keepdims=True)
    i1 = (S - 1) - (pltpu.bitcast(k1, i32)[0, 0] & (S - 1))
    i2 = (S - 1) - (pltpu.bitcast(k2, i32)[0, 0] & (S - 1))
    g1 = pl.multiple_of(i1 & ~7, 8)
    g2 = pl.multiple_of(i2 & ~7, 8)

    def two(f):
        return jnp.concatenate([f(pl.ds(g1, 8)), f(pl.ds(g2, 8))], axis=0)

    hh = two(lambda r_: acc_ref[r_, :])
    hnb = (_rb(hh - _wide(two(lambda r_: st_ref[1, r_, :]))) * _wide(two(lambda r_: st_ref[0, r_, :]))).astype(bf16)
    hn = hnb.astype(f32)
    r = _rb(jnp.sum(hn * wr, axis=1, keepdims=True))
    sub = lax.broadcasted_iota(i32, (16, 1), 0)
    tok = jnp.where(sub < 8, g1 + sub, g2 + sub - 8)
    sel = (tok == i1) | (tok == i2)
    g = _rb(jnp.dot(hnb, wg_ref[...], preferred_element_type=f32))
    g = _rb(g * _rb(jax.nn.sigmoid(g)))
    u = _rb(jnp.dot(hnb, wu_ref[...], preferred_element_type=f32))
    y = _rb(jnp.dot((g * u).astype(bf16), wd_ref[:, 0:M], preferred_element_type=f32))
    y = _rb(y * _rb(jax.nn.sigmoid(r)))
    res = (hh + jnp.where(sel, _rb(hn + y), hn)).astype(bf16)
    for i in range(NB):
        outcopy(i).wait()
    o_ref[0:16, :] = res
    cp1 = pltpu.make_async_copy(o_ref.at[0:8], o_hbm.at[pl.ds(g1, 8)], outsem.at[0])
    cp1.start()

    @pl.when(g2 != g1)
    def _():
        cp2 = pltpu.make_async_copy(o_ref.at[8:16], o_hbm.at[pl.ds(g2, 8)], outsem.at[1])
        cp2.start()
        cp2.wait()

    cp1.wait()


@jax.jit
def pallas_sequential_preLN__compressed_kv_cla__moe_arch_mod__prompt_kernel(
    A_x: jax.Array,
    A_c_kv: jax.Array,
    A_w_q: jax.Array,
    A_w_uk: jax.Array,
    A_w_uv: jax.Array,
    A_w_o: jax.Array,
    B_x: jax.Array,
    B_w_r: jax.Array,
    B_w_gate: jax.Array,
    B_w_up: jax.Array,
    B_w_down: jax.Array,
):
    del B_x
    hbm = pl.BlockSpec(memory_space=pl.ANY)
    V = pltpu.VMEM
    DMA = pltpu.SemaphoreType.DMA
    out = pl.pallas_call(
        _kernel,
        in_specs=[hbm] * 10,
        out_specs=hbm,
        out_shape=jax.ShapeDtypeStruct((S, M), bf16),
        scratch_shapes=[
            V((S, M), bf16), V((S, DC), bf16),
            V((S // 2, DC), u32), V((S // 2, M), u32),
            V((S, M), f32), V((S, M), bf16),
            V((2, M // G, 2 * G, D), bf16), V((2, DC // G, 2 * G, D), bf16), V((2, DC // G, 2 * G, D), bf16),
            V((2, 2, D, M), bf16),
            V((2, S // 2, D), u32), V((2, S // 2, D), u32), V((2, S // 2, D), u32), V((2, S // 2, D), u32),
            V((M,), bf16), V((M, F), bf16), V((M, F), bf16),
            V((F, M + 128), bf16),
            V((2, S, 128), f32), V((8, 128), u32),
            DMA((4, 2)), DMA((NB,)), DMA((NB,)), DMA((4,)), DMA((NB,)),
        ],
        compiler_params=pltpu.CompilerParams(vmem_limit_bytes=120 * 1024 * 1024,
                                             disable_bounds_checks=True,
                                             disable_semaphore_checks=True),
    )(A_x.reshape(S, M), A_c_kv.reshape(S, DC), A_w_q.reshape(M // G, G, H, D),
      A_w_uk.reshape(DC // G, G, H, D), A_w_uv.reshape(DC // G, G, H, D), A_w_o,
      B_w_r, B_w_gate, B_w_up, B_w_down)
    return out.reshape(1, S, M)
```

```python
import math

import jax
import jax.numpy as jnp
from jax import lax
from jax.experimental import pallas as pl
from jax.experimental.pallas import tpu as pltpu

S, M, H, D, DC, F = 2048, 1024, 32, 128, 512, 3584
EPS = 1e-5
bf16, f32, u32, i32 = jnp.bfloat16, jnp.float32, jnp.uint32, jnp.int32
NT = (((1,), (1,)), ((), ()))
G = 4
NP = H // 2
TQ = 256
NB = S // TQ
T2 = TQ // 2
NG = TQ // 8
FCH = 14
QSCALE = (D ** -0.5) * math.log2(math.e)
PACE = 72

NEG = -1e30
GR = 16
NC = 128 // GR
TB = 128 * NC
NV = 4
BS = 4

MID = ("LT105 LT106 QK107 LT104 QK106 QK105 QK104 LT101 LT103 LT102 QK103 QK102 PV107 QK101 LT100 LT116 "
       "QK100 PV105 PV106 LT115 QK117 QK115 PV104 LT114 QK116 PV102 LT113 QK114 PV103 LT112 PV101 LT111 "
       "QK113 PV100 LT110 PV115 QK112 PV117 QK111 LT006 QK110 PV116 LT005 QK007 KP7 QP7 PV114 LT004 QK006 "
       "QP6 LT003 KP6 QK005 PV112 LT002 LT001 QK003 QK004 PV113 QP5 KP5 PV110 PV111 QK002 QP4 PV007 QK001 "
       "KP4 VP7 PV006 LT000 LT016 QK000 PV005 QK017 LT015 VP6 QK016 PV004 VP5 PV002 LT014 QK015 PV003 LT012 "
       "QK014 OUT7 OUT6 LT013 VP4 QK013 PV000 LT010 QK012 OUT5 PV001 LT011 PV017 QK011 OUT4 QK010 QP3 PV015 "
       "PV012 PV013 KP1 PV016 PV014 PV011 QP1 PV010 KP2 OUT2 KP3 VP3 KP0 QP0 QP2 VP2 VP1 OUT1 OUT3 VP0 OUT0")
LAST = ("LT16 LT15 QK17 LT14 QK16 QK15 QK14 LT13 PV17 LT12 LT11 QK13 PV16 LT10 QK11 QK12 PV14 PV13 LT05 PV15 "
       "QK10 LT06 QK07 LT04 PV12 QK05 QK06 PV11 PV10 LT02 QK04 LT03 PV07 LT01 QK03 LT00 QK02 PV05 PV06 QK01 "
       "PV04 QK00 PV03 PV02 PV00 PV01")


def _parse(s):
    out = []
    for t in s.split():
        name = t.rstrip("0123456789")
        out.append((name,) + tuple(int(c) for c in t[len(name):]))
    return out


def _rb(x):
    return x.astype(bf16).astype(f32)


def _pk(x):
    return pltpu.bitcast(x, u32)


def _upk(x):
    return pltpu.bitcast(x, bf16)


def _gather(col):
    n = col.shape[0] // 8
    lane = lax.broadcasted_iota(i32, (8, 128), 1)
    vs = [jnp.broadcast_to(col[g * 8:(g + 1) * 8], (8, 128)) for g in range(n)]
    bit = 1
    while len(vs) > 1:
        m = (lane & bit) != 0
        vs = [jnp.where(m, vs[2 * k + 1], vs[2 * k]) for k in range(len(vs) // 2)]
        bit *= 2
    return vs[0]


def _scatter(dense, n):
    return jnp.concatenate([jnp.broadcast_to(dense[:, g:g + 1], (8, 128)) for g in range(n)], axis=0)


def _wide(v):
    return jnp.concatenate([v] * (M // 128), axis=1)


def _unpack_pair(buf):
    k = buf.shape[0] * G
    w = pltpu.bitcast(buf.reshape(2 * k, D), u32)
    w2 = jnp.concatenate([w << 16, w & jnp.uint32(0xFFFF0000)], axis=1)
    return pltpu.bitcast(w2, f32).astype(bf16)


def _cat(parts, axis):
    return parts[0] if len(parts) == 1 else jnp.concatenate(parts, axis=axis)


def _rows(i, n, k=1):
    return pl.ds(i * n, k * n) if isinstance(i, int) else pl.ds(pl.multiple_of(i * n, n), k * n)


def _kernel(x_hbm, c_hbm, wq_hbm, wk_hbm, wv_hbm, wo_hbm, wr_hbm, wg_hbm, wu_hbm, wd_hbm, o_hbm,
            x_ref, c_ref, cp_ref, xn_ref, accp_ref, op_ref, bq, bk, bv, bo, q_ref, k_ref, v_ref, ctx_ref,
            wr_ref, wg_ref, wu_ref, wd_ref, stp_ref, z_ref, wsem, xsem, csem, fsem, outsem):
    acc_ref, o_ref, st_ref = accp_ref.at[TQ:], op_ref.at[TQ:], stp_ref.at[:, TQ:]

    wtab = {"k": (0, wk_hbm, bk), "v": (1, wv_hbm, bv), "q": (2, wq_hbm, bq), "o": (3, wo_hbm, bo)}

    def wstart(name, pair, slot):
        t, w, b = wtab[name]
        heads = _rows(pair, 2)
        if name == "o":
            pltpu.make_async_copy(w.at[heads], b.at[slot], wsem.at[t, slot]).start()
        else:
            for g in range(G):
                pltpu.make_async_copy(w.at[:, g, heads, :], b.at[slot, :, pl.ds(2 * g, 2), :],
                                      wsem.at[t, slot]).start()

    def wwait(name, slot):
        t, _, b = wtab[name]
        pltpu.make_async_copy(b.at[slot], b.at[slot], wsem.at[t, slot]).wait()

    def xcopy(i):
        return pltpu.make_async_copy(x_hbm.at[_rows(i, TQ)], x_ref.at[_rows(i, TQ)], xsem.at[i])

    def ccopy(i):
        return pltpu.make_async_copy(c_hbm.at[_rows(i, TQ)], c_ref.at[_rows(i, TQ)], csem.at[i])

    def outcopy(i):
        return pltpu.make_async_copy(o_ref.at[_rows(i, TQ)], o_hbm.at[_rows(i, TQ)], outsem.at[i])

    rcopy = pltpu.make_async_copy(wr_hbm, wr_ref, fsem.at[3])

    def fstart(j):
        cs = _rows(j, F // FCH)
        pltpu.make_async_copy(wg_hbm.at[:, cs], wg_ref.at[:, cs], fsem.at[0]).start()
        pltpu.make_async_copy(wu_hbm.at[:, cs], wu_ref.at[:, cs], fsem.at[1]).start()
        pltpu.make_async_copy(wd_hbm.at[cs, :], wd_ref.at[cs, 0:M], fsem.at[2]).start()

    def fwait():
        for t, r in enumerate((wg_ref, wu_ref, wd_ref.at[:, 0:M])):
            pltpu.make_async_copy(r, r, fsem.at[t]).wait()

    def proj(src, w, dst, i, scale=None):
        y = jnp.dot(_upk(src), w, preferred_element_type=f32)
        if scale is not None:
            y = y * scale
        for e in range(2):
            dst[e, _rows(i, src.shape[0]), :] = _pk(y[:, e * D:(e + 1) * D].astype(bf16))

    def pr(ref, e, lo, hi):
        return ref[e, lo // 2:hi // 2, :]

    def nt(a, b):
        return lax.dot_general(_upk(a), _upk(b), NT, preferred_element_type=f32)

    def iota2():
        return lax.broadcasted_iota(i32, (GR, 128), 0), lax.broadcasted_iota(i32, (GR, 128), 1)

    def causal_tri():
        row, col = iota2()
        return col <= row + (128 - GR)

    def qunit(I, e, c):
        return _cat([pr(q_ref, e, r, r + GR) for r in range(I * TB + GR * c, (I + 1) * TB, 128)], 0)

    def period(c):
        return 1 << (GR * (c + 1) - 1).bit_length()

    def left(I, e, c, nv):
        s = GR * (c + 1)
        per = period(c) if c < nv else 128
        st = nt(pr(k_ref, e, 0, s), qunit(I, e, c))
        pad = [jnp.full((per - s, 128), NEG, f32)] if per > s else []
        t = jnp.concatenate(([st] + pad) * (128 // per), axis=0).T
        if I == 0:
            row, col = iota2()
            t = jnp.concatenate([jnp.where((col & (per - 1)) <= row + GR * c, t[:GR], NEG), t[GR:]], axis=0)
        return t

    def qk(I, e, c, tri, lf):
        r0 = I * TB
        s = GR * (c + 1)
        q = qunit(I, e, c)
        if s == 128:
            mn = nt(q, pr(k_ref, e, 0, r0 + 128))
        else:
            mn = _cat([lf] + ([nt(q, pr(k_ref, e, s, r0 + s))] if r0 else []), 1)
        ex = [nt(q[x * GR // 2:], pr(k_ref, e, r0 + s + 128 * (x - 1), r0 + s + 128 * x)) for x in range(1, NC)]
        out = []
        for a in range(NC):
            sa = _cat([mn[a * GR:(a + 1) * GR]]
                      + [ex[x - 1][(a - x) * GR:(a - x + 1) * GR] for x in range(1, a + 1)], 1)
            w = sa.shape[1]
            if not (s < 128 and w == 128):
                sa = _cat(([sa[:, :w - 128]] if w > 128 else []) + [jnp.where(tri, sa[:, w - 128:], NEG)], 1)
            out.append(jnp.exp2(sa - jnp.max(sa, axis=1, keepdims=True)))
        return out

    def skewed_v(e, per):
        w = _upk(pr(v_ref, e, 0, per)).astype(f32)
        lane = lax.broadcasted_iota(i32, (per, 128), 1)
        bit = 1
        while bit < per:
            w = jnp.where((lane & bit) != 0, pltpu.roll(w, per - bit, 0), w)
            bit *= 2
        return [w[0:BS]] + [pltpu.roll(w[r // 8 * 8:r // 8 * 8 + 8], r, 1)[r % 8:r % 8 + BS]
                            for r in range(BS, per, BS)]

    def pv(I, e, c, p, nv, skew):
        r0 = I * TB
        s = GR * (c + 1)
        w0 = r0 + 128
        vpu = c < nv
        if s == 128:
            vm = [pr(v_ref, e, 0, w0)]
        else:
            vm = ([] if vpu else [pr(v_ref, e, 0, 128)]) + ([pr(v_ref, e, s, r0 + s)] if r0 else [])
        cs = [None] * NC
        if vm:
            pm = _cat([pa[:, 128 * vpu:w0] for pa in p], 0).astype(bf16)
            ctx = jnp.dot(pm, _upk(_cat(vm, 0)), preferred_element_type=f32)
            cs = [ctx[a * GR:(a + 1) * GR] for a in range(NC)]
        if vpu:
            per = period(c)
            if (e, per) not in skew:
                skew[e, per] = skewed_v(e, per)
            pl0 = _cat([pa[:, :128] for pa in p], 0)
            baby = [pl0] + [pltpu.roll(pl0, 128 - b, 1) for b in range(1, BS)]
            acc = None
            for w in reversed(skew[e, per]):
                if acc is not None:
                    acc = pltpu.roll(acc, 128 - BS, 1)
                for b in range(BS):
                    t = baby[b] * w[b:b + 1, :]
                    acc = t if acc is None else acc + t
            once = iota2()[1] < s
            p = [_cat([jnp.where(once, pa[:, :128], 0.0)] + ([pa[:, 128:]] if pa.shape[1] > 128 else []), 1)
                 for pa in p]
        den = [jnp.sum(pa.astype(bf16).astype(f32), axis=1, keepdims=True) for pa in p]
        for x in range(1, NC):
            px = _cat([p[a][:, w0 + 128 * (x - 1):w0 + 128 * x] for a in range(x, NC)], 0).astype(bf16)
            cx = jnp.dot(px, _upk(pr(v_ref, e, r0 + s + 128 * (x - 1), r0 + s + 128 * x)),
                         preferred_element_type=f32)
            for a in range(x, NC):
                t = cx[(a - x) * GR:(a - x + 1) * GR]
                cs[a] = t if cs[a] is None else cs[a] + t
        if vpu:
            cs = [acc[a * GR:(a + 1) * GR] if cs[a] is None else cs[a] + acc[a * GR:(a + 1) * GR]
                  for a in range(NC)]
        return [cs[a] * pl.reciprocal(den[a], approx=False, full_range=False) for a in range(NC)]

    def issue(n, f):
        def body(i, _):
            f(i)
            return 0

        lax.fori_loop(0, n, body, 0)

    HB = NB // 2
    wstart("k", 0, 0)
    wstart("v", 0, 0)
    issue(HB, lambda i: ccopy(i).start())
    wstart("q", 0, 0)
    issue(HB, lambda t: (ccopy(HB + t).start(), xcopy(2 * t).start(), xcopy(2 * t + 1).start()))
    wstart("o", 0, 0)
    for name in "kvq":
        wstart(name, 1, 1)
    rcopy.start()
    z_ref[...] = jnp.zeros((8, 128), u32)

    def zero_pad(i):
        accp_ref[_rows(i, 32), :] = jnp.zeros((32, M), f32)

    issue(TQ // 32, zero_pad)
    wwait("k", 0)
    wk0 = _unpack_pair(bk[0])
    wwait("v", 0)
    wv0 = _unpack_pair(bv[0])

    def pack_c(i):
        cpk = _pk(c_ref[_rows(i, TQ), :])
        cp_ref[_rows(i, T2), :] = cpk
        return cpk

    def ln_block(i):
        xf = x_ref[_rows(i, TQ), :].astype(f32)
        acc_ref[_rows(i, TQ), :] = xf
        d = xf - jnp.sum(xf, axis=-1, keepdims=True) * (1.0 / M)
        inv = lax.rsqrt(jnp.sum(d * d, axis=-1, keepdims=True) * (1.0 / M) + EPS)
        xnp = _pk((d * inv).astype(bf16))
        xn_ref[_rows(i, T2), :] = xnp
        return xnp

    def pro_a(i, _):
        ccopy(i).wait()
        cpk = pack_c(i)
        proj(cpk, wk0, k_ref, i)
        proj(cpk, wv0, v_ref, i)
        return 0

    lax.fori_loop(0, HB, pro_a, 0)
    wwait("q", 0)
    wq0 = _unpack_pair(bq[0])

    def pro_b(t, _):
        ccopy(HB + t).wait()
        xcopy(2 * t).wait()
        xcopy(2 * t + 1).wait()
        xs = [ln_block(2 * t), ln_block(2 * t + 1)]
        cpk = pack_c(HB + t)
        for j, (w, dst) in enumerate(((wk0, k_ref), (wv0, v_ref))):
            proj(cpk, w, dst, HB + t)
            for n in range(4):
                proj(xs[j][n * 32:(n + 1) * 32], wq0, q_ref, (2 * t + j) * 4 + n, QSCALE)
        return 0

    lax.fori_loop(0, HB, pro_b, 0)

    def step(p, _):
        s0 = p & 1
        s1 = 1 - s0
        for name in "kvq":
            wwait(name, s1)
        wwait("o", s0)
        ahead = jnp.minimum(p + 2, NP - 1)
        for name in "kvq":
            wstart(name, ahead, s0)
        wstart("o", p + 1, s1)

        @pl.when(p < FCH)
        def _():
            fstart(p)

        tri = causal_tri()
        w = {}

        def weight(name):
            if name not in w:
                b = wtab[name][2]
                w[name] = b[s0].reshape(2 * D, M) if name == "o" else _unpack_pair(b[s1])
            return w[name]

        lfs, ps, ctxs, skew = {}, {}, {}, {}
        for item in _parse(MID):
            op, i, u = item[0], item[1], item[1:]
            if op == "LT":
                lfs[u] = left(*u, NV)
            elif op == "KP":
                proj(cp_ref[_rows(i, T2), :], weight("k"), k_ref, i)
            elif op == "VP":
                proj(cp_ref[_rows(i, T2), :], weight("v"), v_ref, i)
            elif op == "QP":
                proj(xn_ref[_rows(i, T2), :], weight("q"), q_ref, i, QSCALE)
            elif op == "QK":
                ps[u] = qk(*u, tri, lfs.pop(u, None))
            elif op == "PV":
                ctxs[u] = pv(*u, ps.pop(u), NV, skew)
            else:
                I, a0 = divmod(2 * i, NC)
                c2 = jnp.concatenate([_cat([ctxs[I, e, c][a] for a in (a0, a0 + 1) for c in range(NC)], 0)
                                      for e in range(2)], axis=1).astype(bf16)
                acc_ref[_rows(i, TQ), :] += jnp.dot(c2, weight("o"), preferred_element_type=f32)
        return 0

    lax.fori_loop(0, NP - 1, step, 0)

    def last_head(e, _):
        tri = causal_tri()
        lfs, ps = {}, {}
        for op, I, c in _parse(LAST):
            if op == "LT":
                lfs[I, c] = left(I, e, c, 0)
            elif op == "QK":
                ps[I, c] = qk(I, e, c, tri, lfs.pop((I, c), None))
            else:
                for a, ca in enumerate(pv(I, e, c, ps.pop((I, c)), 0, None)):
                    r = (I * TB + 128 * a + GR * c) // 2
                    ctx_ref[e, r:r + GR // 2, :] = _pk(ca.astype(bf16))
        return 0

    lax.fori_loop(0, 2, last_head, 0)
    wwait("o", (NP - 1) & 1)
    rcopy.wait()
    for name in "kvq":
        wwait(name, NP & 1)
    fwait()
    wr = wr_ref[...].astype(f32).reshape(1, M)

    def out_block(i, dst):
        c2 = _upk(jnp.concatenate([ctx_ref[0, _rows(i, T2), :], ctx_ref[1, _rows(i, T2), :]], axis=1))
        wo = bo[(NP - 1) & 1].reshape(2 * D, M)
        y = dst[...] + jnp.dot(c2, wo, preferred_element_type=f32)
        dst[...] = _rb(y)
        return y

    def epi_block(i, src, top, y=None, maybe_pad=False):
        hh = src[...]
        s = jnp.sum(hh, axis=-1, keepdims=True)
        mrow = _rb(s * (1.0 / M))
        if y is not None:
            z = z_ref[...]
            parts = []
            for g in range(NG):
                t = g * PACE // NG
                yt = y[(t % NG) * 8:(t % NG + 1) * 8, (t // NG) * 256:(t // NG) * 256 + 128]
                mg = jnp.broadcast_to(mrow[g * 8:(g + 1) * 8], (8, 128))
                parts.append(pltpu.bitcast(pltpu.bitcast(mg, u32) | (pltpu.bitcast(yt, u32) & z), f32))
            mrow = jnp.concatenate(parts, axis=0)
        else:
            mrow = jnp.broadcast_to(mrow, (TQ, 128))
        d = hh - _wide(mrow)
        mu = _gather(s) * (1.0 / M)
        dm = mu - _rb(mu)
        var = _gather(jnp.sum(d * d, axis=-1, keepdims=True)) * (1.0 / M) - dm * dm
        sw = _gather(jnp.sum(d * wr, axis=-1, keepdims=True))
        ve = _rb(_rb(jnp.maximum(var, 0.0)) + EPS)
        inv = pl.reciprocal(_rb(ve * lax.rsqrt(ve)), approx=False, full_range=False)
        r = _rb(sw * inv)
        inv_s = _scatter(inv, NG)
        off_s = mrow * inv_s
        stp_ref[0, _rows(i + 1, TQ), :] = inv_s
        stp_ref[1, _rows(i + 1, TQ), :] = mrow
        op_ref[_rows(i + 1, TQ), :] = (hh * _wide(inv_s + 1.0) - _wide(off_s)).astype(bf16)
        if maybe_pad:
            @pl.when(i >= 0)
            def _():
                outcopy(i).start()
        else:
            outcopy(i).start()
        b = pltpu.bitcast(r + 0.0, i32)
        code = lax.shift_right_arithmetic(b ^ (lax.shift_right_arithmetic(b, 31) & jnp.int32(0x7FFF0000)), 5)
        lane = lax.broadcasted_iota(i32, (8, 128), 1)
        tok = i * TQ + lane * 8 + lax.broadcasted_iota(i32, (8, 128), 0)
        key = pltpu.bitcast(code + (jnp.int32(0x24000000 + S - 1) - tok), f32)
        key = jnp.where((lane < NG) & (tok >= 0) if maybe_pad else lane < NG, key, 0.0)
        return jnp.maximum(top[0], key), jnp.maximum(top[1], jnp.minimum(top[0], key))

    def out_epi(j, top):
        v = accp_ref.at[pl.ds(pl.multiple_of(j * (2 * TQ), TQ), 3 * TQ)]
        for t in range(2):
            y = out_block(2 * j + t, v.at[(t + 1) * TQ:(t + 2) * TQ])
            top = epi_block(2 * j + t - 1, v.at[t * TQ:(t + 1) * TQ], top, y, t == 0)
        return top

    lo = jnp.zeros((8, 128), f32)
    top = lax.fori_loop(0, NB // 2, out_epi, (lo, lo))
    t1, t2 = epi_block(NB - 1, acc_ref.at[_rows(NB - 1, TQ)], top)

    for sh in (4, 2, 1):
        u1, u2 = pltpu.roll(t1, sh, 0), pltpu.roll(t2, sh, 0)
        t1, t2 = jnp.maximum(t1, u1), jnp.maximum(jnp.maximum(t2, u2), jnp.minimum(t1, u1))
    lane = lax.broadcasted_iota(i32, (8, 128), 1)
    sub8 = lax.broadcasted_iota(i32, (8, 128), 0)
    bit = (lax.shift_right_logical(lane, sub8) & 1) == 1
    m0 = jnp.max(jnp.where(sub8 == 7, t2, jnp.where(bit, 0.0, t1)), axis=1, keepdims=True)
    m1 = jnp.max(jnp.where(sub8 == 7, t2, jnp.where(bit, t1, 0.0)), axis=1, keepdims=True)
    k1 = jnp.maximum(m0, m1)[0:1]
    k2 = jnp.max(jnp.minimum(m0, m1), axis=0, keepdims=True)
    i1 = (S - 1) - (pltpu.bitcast(k1, i32)[0, 0] & (S - 1))
    i2 = (S - 1) - (pltpu.bitcast(k2, i32)[0, 0] & (S - 1))
    g1 = pl.multiple_of(i1 & ~7, 8)
    g2 = pl.multiple_of(i2 & ~7, 8)

    def two(f):
        return jnp.concatenate([f(pl.ds(g1, 8)), f(pl.ds(g2, 8))], axis=0)

    hh = two(lambda r_: acc_ref[r_, :])
    hnb = (_rb(hh - _wide(two(lambda r_: st_ref[1, r_, :]))) * _wide(two(lambda r_: st_ref[0, r_, :]))).astype(bf16)
    hn = hnb.astype(f32)
    r = _rb(jnp.sum(hn * wr, axis=1, keepdims=True))
    sub = lax.broadcasted_iota(i32, (16, 1), 0)
    tok = jnp.where(sub < 8, g1 + sub, g2 + sub - 8)
    sel = (tok == i1) | (tok == i2)
    g = _rb(jnp.dot(hnb, wg_ref[...], preferred_element_type=f32))
    g = _rb(g * _rb(jax.nn.sigmoid(g)))
    u = _rb(jnp.dot(hnb, wu_ref[...], preferred_element_type=f32))
    y = _rb(jnp.dot((g * u).astype(bf16), wd_ref[:, 0:M], preferred_element_type=f32))
    y = _rb(y * _rb(jax.nn.sigmoid(r)))
    res = (hh + jnp.where(sel, _rb(hn + y), hn)).astype(bf16)
    for i in range(NB):
        outcopy(i).wait()
    o_ref[0:16, :] = res
    cp1 = pltpu.make_async_copy(o_ref.at[0:8], o_hbm.at[pl.ds(g1, 8)], outsem.at[0])
    cp1.start()

    @pl.when(g2 != g1)
    def _():
        cp2 = pltpu.make_async_copy(o_ref.at[8:16], o_hbm.at[pl.ds(g2, 8)], outsem.at[1])
        cp2.start()
        cp2.wait()

    cp1.wait()


@jax.jit
def pallas_sequential_preLN__compressed_kv_cla__moe_arch_mod__prompt_kernel(
    A_x: jax.Array,
    A_c_kv: jax.Array,
    A_w_q: jax.Array,
    A_w_uk: jax.Array,
    A_w_uv: jax.Array,
    A_w_o: jax.Array,
    B_x: jax.Array,
    B_w_r: jax.Array,
    B_w_gate: jax.Array,
    B_w_up: jax.Array,
    B_w_down: jax.Array,
):
    del B_x
    hbm = pl.BlockSpec(memory_space=pl.ANY)
    V = pltpu.VMEM
    DMA = pltpu.SemaphoreType.DMA
    out = pl.pallas_call(
        _kernel,
        in_specs=[hbm] * 10,
        out_specs=hbm,
        out_shape=jax.ShapeDtypeStruct((S, M), bf16),
        scratch_shapes=[
            V((S, M), bf16), V((S, DC), bf16),
            V((S // 2, DC), u32), V((S // 2, M), u32),
            V((S + TQ, M), f32), V((S + TQ, M), bf16),
            V((2, M // G, 2 * G, D), bf16), V((2, DC // G, 2 * G, D), bf16), V((2, DC // G, 2 * G, D), bf16),
            V((2, 2, D, M), bf16),
            V((2, S // 2, D), u32), V((2, S // 2, D), u32), V((2, S // 2, D), u32), V((2, S // 2, D), u32),
            V((M,), bf16), V((M, F), bf16), V((M, F), bf16),
            V((F, M + 128), bf16),
            V((2, S + TQ, 128), f32), V((8, 128), u32),
            DMA((4, 2)), DMA((NB,)), DMA((NB,)), DMA((4,)), DMA((NB,)),
        ],
        compiler_params=pltpu.CompilerParams(vmem_limit_bytes=120 * 1024 * 1024,
                                             disable_bounds_checks=True,
                                             disable_semaphore_checks=True),
    )(A_x.reshape(S, M), A_c_kv.reshape(S, DC), A_w_q.reshape(M // G, G, H, D),
      A_w_uk.reshape(DC // G, G, H, D), A_w_uv.reshape(DC // G, G, H, D), A_w_o,
      B_w_r, B_w_gate, B_w_up, B_w_down)
    return out.reshape(1, S, M)
```

```python
import math

import jax
import jax.numpy as jnp
from jax import lax
from jax.experimental import pallas as pl
from jax.experimental.pallas import tpu as pltpu

S, M, H, D, DC, F = 2048, 1024, 32, 128, 512, 3584
EPS = 1e-5
bf16, f32, u32, i32 = jnp.bfloat16, jnp.float32, jnp.uint32, jnp.int32
NT = (((1,), (1,)), ((), ()))
G = 4
NP = H // 2
TQ = 256
NB = S // TQ
T2 = TQ // 2
NG = TQ // 8
FCH = 14
QSCALE = (D ** -0.5) * math.log2(math.e)
PACE = 72

NEG = -1e30
GR = 16
NC = 128 // GR
TB = 128 * NC
NV = 4
BS = 4

MID = ("LT105 LT106 QK107 LT104 QK106 QK105 QK104 LT101 LT103 LT102 QK103 QK102 PV107 QK101 LT100 LT116 "
       "QK100 PV105 PV106 LT115 QK117 QK115 LT114 QK116 PV102 LT113 QK114 PV103 LT112 PV101 PV104 LT111 "
       "PV100 QK113 PV115 LT110 QK112 PV117 QK111 LT006 QK110 PV116 LT005 QK007 KP7 QP7 LT003 PV114 LT004 "
       "QK006 QP6 KP6 QK005 PV112 LT001 LT002 QK003 QK004 PV113 KP5 QP5 PV110 PV111 QK002 QP4 PV007 QK001 "
       "KP4 VP7 PV006 VP6 LT000 LT016 QK000 PV005 QK017 LT015 QK016 PV004 VP5 PV002 LT014 QK015 PV003 LT012 "
       "QK014 OUT7 VP4 OUT6 LT013 QK013 PV000 LT010 QK012 PV001 LT011 OUT5 PV017 QK011 OUT4 QK010 KP1 PV015 "
       "QP3 PV012 PV013 PV016 PV014 PV010 PV011 QP1 KP2 OUT2 KP3 QP0 OUT3 QP2 VP2 OUT1 VP3 KP0 VP1 VP0 OUT0")
LAST = ("LT16 LT15 QK17 LT14 QK16 QK15 QK14 LT13 PV17 LT12 LT11 QK13 PV16 LT10 QK11 QK12 PV14 PV13 LT05 PV15 "
       "QK10 LT06 QK07 LT04 PV12 QK05 QK06 PV11 PV10 LT02 QK04 LT03 PV07 LT01 QK03 LT00 QK02 PV05 PV06 QK01 "
       "PV04 QK00 PV03 PV02 PV00 PV01")


def _parse(s):
    out = []
    for t in s.split():
        name = t.rstrip("0123456789")
        out.append((name,) + tuple(int(c) for c in t[len(name):]))
    return out


def _rb(x):
    return x.astype(bf16).astype(f32)


def _pk(x):
    return pltpu.bitcast(x, u32)


def _upk(x):
    return pltpu.bitcast(x, bf16)


def _gather(col):
    n = col.shape[0] // 8
    lane = lax.broadcasted_iota(i32, (8, 128), 1)
    vs = [jnp.broadcast_to(col[g * 8:(g + 1) * 8], (8, 128)) for g in range(n)]
    bit = 1
    while len(vs) > 1:
        m = (lane & bit) != 0
        vs = [jnp.where(m, vs[2 * k + 1], vs[2 * k]) for k in range(len(vs) // 2)]
        bit *= 2
    return vs[0]


def _scatter(dense, n):
    return jnp.concatenate([jnp.broadcast_to(dense[:, g:g + 1], (8, 128)) for g in range(n)], axis=0)


def _wide(v):
    return jnp.concatenate([v] * (M // 128), axis=1)


def _unpack_pair(buf):
    k = buf.shape[0] * G
    w = pltpu.bitcast(buf.reshape(2 * k, D), u32)
    w2 = jnp.concatenate([w << 16, w & jnp.uint32(0xFFFF0000)], axis=1)
    return pltpu.bitcast(w2, f32).astype(bf16)


def _cat(parts, axis):
    return parts[0] if len(parts) == 1 else jnp.concatenate(parts, axis=axis)


def _rows(i, n, k=1):
    return pl.ds(i * n, k * n) if isinstance(i, int) else pl.ds(pl.multiple_of(i * n, n), k * n)


def _kernel(x_hbm, c_hbm, wq_hbm, wk_hbm, wv_hbm, wo_hbm, wr_hbm, wg_hbm, wu_hbm, wd_hbm, o_hbm,
            x_ref, c_ref, cp_ref, xn_ref, accp_ref, op_ref, bq, bk, bv, bo, q_ref, k_ref, v_ref, ctx_ref,
            wr_ref, wg_ref, wu_ref, wd_ref, stp_ref, z_ref, wsem, xsem, csem, fsem, outsem):
    acc_ref, o_ref, st_ref = accp_ref.at[TQ:], op_ref.at[TQ:], stp_ref.at[:, TQ:]

    wtab = {"k": (0, wk_hbm, bk), "v": (1, wv_hbm, bv), "q": (2, wq_hbm, bq), "o": (3, wo_hbm, bo)}

    def wstart(name, pair, slot):
        t, w, b = wtab[name]
        heads = _rows(pair, 2)
        if name == "o":
            pltpu.make_async_copy(w.at[heads], b.at[slot], wsem.at[t, slot]).start()
        else:
            for g in range(G):
                pltpu.make_async_copy(w.at[:, g, heads, :], b.at[slot, :, pl.ds(2 * g, 2), :],
                                      wsem.at[t, slot]).start()

    def wwait(name, slot):
        t, _, b = wtab[name]
        pltpu.make_async_copy(b.at[slot], b.at[slot], wsem.at[t, slot]).wait()

    def xcopy(i):
        return pltpu.make_async_copy(x_hbm.at[_rows(i, TQ)], x_ref.at[_rows(i, TQ)], xsem.at[i])

    def ccopy(i):
        return pltpu.make_async_copy(c_hbm.at[_rows(i, TQ)], c_ref.at[_rows(i, TQ)], csem.at[i])

    def outcopy(i):
        return pltpu.make_async_copy(o_ref.at[_rows(i, TQ)], o_hbm.at[_rows(i, TQ)], outsem.at[i])

    rcopy = pltpu.make_async_copy(wr_hbm, wr_ref, fsem.at[3])

    def fstart(j):
        cs = _rows(j, F // FCH)
        pltpu.make_async_copy(wg_hbm.at[:, cs], wg_ref.at[:, cs], fsem.at[0]).start()
        pltpu.make_async_copy(wu_hbm.at[:, cs], wu_ref.at[:, cs], fsem.at[1]).start()
        pltpu.make_async_copy(wd_hbm.at[cs, :], wd_ref.at[cs, 0:M], fsem.at[2]).start()

    def fwait():
        for t, r in enumerate((wg_ref, wu_ref, wd_ref.at[:, 0:M])):
            pltpu.make_async_copy(r, r, fsem.at[t]).wait()

    def proj(src, w, dst, i, scale=None):
        y = jnp.dot(_upk(src), w, preferred_element_type=f32)
        if scale is not None:
            y = y * scale
        for e in range(2):
            dst[e, _rows(i, src.shape[0]), :] = _pk(y[:, e * D:(e + 1) * D].astype(bf16))

    def pr(ref, e, lo, hi):
        return ref[e, lo // 2:hi // 2, :]

    def nt(a, b):
        return lax.dot_general(_upk(a), _upk(b), NT, preferred_element_type=f32)

    def iota2():
        return lax.broadcasted_iota(i32, (GR, 128), 0), lax.broadcasted_iota(i32, (GR, 128), 1)

    def causal_tri():
        row, col = iota2()
        return col <= row + (128 - GR)

    def qunit(I, e, c):
        return _cat([pr(q_ref, e, r, r + GR) for r in range(I * TB + GR * c, (I + 1) * TB, 128)], 0)

    def period(c):
        return 1 << (GR * (c + 1) - 1).bit_length()

    def left(I, e, c, nv):
        s = GR * (c + 1)
        per = period(c) if c < nv else 128
        st = nt(pr(k_ref, e, 0, s), qunit(I, e, c))
        pad = [jnp.full((per - s, 128), NEG, f32)] if per > s else []
        t = jnp.concatenate(([st] + pad) * (128 // per), axis=0).T
        if I == 0:
            row, col = iota2()
            t = jnp.concatenate([jnp.where((col & (per - 1)) <= row + GR * c, t[:GR], NEG), t[GR:]], axis=0)
        return t

    def qk(I, e, c, tri, lf):
        r0 = I * TB
        s = GR * (c + 1)
        q = qunit(I, e, c)
        if s == 128:
            mn = nt(q, pr(k_ref, e, 0, r0 + 128))
        else:
            mn = _cat([lf] + ([nt(q, pr(k_ref, e, s, r0 + s))] if r0 else []), 1)
        ex = [nt(q[x * GR // 2:], pr(k_ref, e, r0 + s + 128 * (x - 1), r0 + s + 128 * x)) for x in range(1, NC)]
        out = []
        for a in range(NC):
            sa = _cat([mn[a * GR:(a + 1) * GR]]
                      + [ex[x - 1][(a - x) * GR:(a - x + 1) * GR] for x in range(1, a + 1)], 1)
            w = sa.shape[1]
            if not (s < 128 and w == 128):
                sa = _cat(([sa[:, :w - 128]] if w > 128 else []) + [jnp.where(tri, sa[:, w - 128:], NEG)], 1)
            out.append(jnp.exp2(sa - jnp.max(sa, axis=1, keepdims=True)))
        return out

    def skewed_v(e, per):
        w = _upk(pr(v_ref, e, 0, per)).astype(f32)
        lane = lax.broadcasted_iota(i32, (per, 128), 1)
        bit = 1
        while bit < per:
            w = jnp.where((lane & bit) != 0, pltpu.roll(w, per - bit, 0), w)
            bit *= 2
        return [w[0:BS]] + [pltpu.roll(w[r // 8 * 8:r // 8 * 8 + 8], r, 1)[r % 8:r % 8 + BS]
                            for r in range(BS, per, BS)]

    def pv(I, e, c, p, nv, skew):
        r0 = I * TB
        s = GR * (c + 1)
        w0 = r0 + 128
        vpu = c < nv
        if s == 128:
            vm = [pr(v_ref, e, 0, w0)]
        else:
            vm = ([] if vpu else [pr(v_ref, e, 0, 128)]) + ([pr(v_ref, e, s, r0 + s)] if r0 else [])
        cs = [None] * NC
        if vm:
            pm = _cat([pa[:, 128 * vpu:w0] for pa in p], 0).astype(bf16)
            ctx = jnp.dot(pm, _upk(_cat(vm, 0)), preferred_element_type=f32)
            cs = [ctx[a * GR:(a + 1) * GR] for a in range(NC)]
        if vpu:
            per = period(c)
            if (e, per) not in skew:
                skew[e, per] = skewed_v(e, per)
            pl0 = _cat([pa[:, :128] for pa in p], 0)
            baby = [pl0] + [pltpu.roll(pl0, 128 - b, 1) for b in range(1, BS)]
            acc = None
            for w in reversed(skew[e, per]):
                if acc is not None:
                    acc = pltpu.roll(acc, 128 - BS, 1)
                for b in range(BS):
                    t = baby[b] * w[b:b + 1, :]
                    acc = t if acc is None else acc + t
            once = iota2()[1] < s
            p = [_cat([jnp.where(once, pa[:, :128], 0.0)] + ([pa[:, 128:]] if pa.shape[1] > 128 else []), 1)
                 for pa in p]
        den = [jnp.sum(pa.astype(bf16).astype(f32), axis=1, keepdims=True) for pa in p]
        for x in range(1, NC):
            px = _cat([p[a][:, w0 + 128 * (x - 1):w0 + 128 * x] for a in range(x, NC)], 0).astype(bf16)
            cx = jnp.dot(px, _upk(pr(v_ref, e, r0 + s + 128 * (x - 1), r0 + s + 128 * x)),
                         preferred_element_type=f32)
            for a in range(x, NC):
                t = cx[(a - x) * GR:(a - x + 1) * GR]
                cs[a] = t if cs[a] is None else cs[a] + t
        if vpu:
            cs = [acc[a * GR:(a + 1) * GR] if cs[a] is None else cs[a] + acc[a * GR:(a + 1) * GR]
                  for a in range(NC)]
        return [cs[a] * pl.reciprocal(den[a], approx=False, full_range=False) for a in range(NC)]

    def issue(n, f):
        def body(i, _):
            f(i)
            return 0

        lax.fori_loop(0, n, body, 0)

    HB = NB // 2
    wstart("k", 0, 0)
    wstart("v", 0, 0)
    issue(HB, lambda i: ccopy(i).start())
    wstart("q", 0, 0)
    issue(HB, lambda t: (ccopy(HB + t).start(), xcopy(2 * t).start(), xcopy(2 * t + 1).start()))
    wstart("o", 0, 0)
    for name in "kvq":
        wstart(name, 1, 1)
    rcopy.start()
    z_ref[...] = jnp.zeros((8, 128), u32)

    def zero_pad(i):
        accp_ref[_rows(i, 32), :] = jnp.zeros((32, M), f32)

    issue(TQ // 32, zero_pad)
    wwait("k", 0)
    wk0 = _unpack_pair(bk[0])
    wwait("v", 0)
    wv0 = _unpack_pair(bv[0])

    def pack_c(i):
        cpk = _pk(c_ref[_rows(i, TQ), :])
        cp_ref[_rows(i, T2), :] = cpk
        return cpk

    def ln_block(i):
        xf = x_ref[_rows(i, TQ), :].astype(f32)
        acc_ref[_rows(i, TQ), :] = xf
        d = xf - jnp.sum(xf, axis=-1, keepdims=True) * (1.0 / M)
        inv = lax.rsqrt(jnp.sum(d * d, axis=-1, keepdims=True) * (1.0 / M) + EPS)
        xnp = _pk((d * inv).astype(bf16))
        xn_ref[_rows(i, T2), :] = xnp
        return xnp

    def pro_a(i, _):
        ccopy(i).wait()
        cpk = pack_c(i)
        proj(cpk, wk0, k_ref, i)
        proj(cpk, wv0, v_ref, i)
        return 0

    lax.fori_loop(0, HB, pro_a, 0)
    wwait("q", 0)
    wq0 = _unpack_pair(bq[0])

    def pro_b(t, _):
        ccopy(HB + t).wait()
        xcopy(2 * t).wait()
        xcopy(2 * t + 1).wait()
        xs = [ln_block(2 * t), ln_block(2 * t + 1)]
        cpk = pack_c(HB + t)
        for j, (w, dst) in enumerate(((wk0, k_ref), (wv0, v_ref))):
            proj(cpk, w, dst, HB + t)
            for n in range(4):
                proj(xs[j][n * 32:(n + 1) * 32], wq0, q_ref, (2 * t + j) * 4 + n, QSCALE)
        return 0

    lax.fori_loop(0, HB, pro_b, 0)

    def step(p, _):
        s0 = p & 1
        s1 = 1 - s0
        for name in "kvq":
            wwait(name, s1)
        wwait("o", s0)
        ahead = jnp.minimum(p + 2, NP - 1)
        for name in "kvq":
            wstart(name, ahead, s0)
        wstart("o", p + 1, s1)

        @pl.when(p < FCH)
        def _():
            fstart(p)

        tri = causal_tri()
        w = {}

        def weight(name):
            if name not in w:
                b = wtab[name][2]
                w[name] = b[s0].reshape(2 * D, M) if name == "o" else _unpack_pair(b[s1])
            return w[name]

        lfs, ps, ctxs, skew = {}, {}, {}, {}
        for item in _parse(MID):
            op, i, u = item[0], item[1], item[1:]
            if op == "LT":
                lfs[u] = left(*u, NV)
            elif op == "KP":
                proj(cp_ref[_rows(i, T2), :], weight("k"), k_ref, i)
            elif op == "VP":
                proj(cp_ref[_rows(i, T2), :], weight("v"), v_ref, i)
            elif op == "QP":
                proj(xn_ref[_rows(i, T2), :], weight("q"), q_ref, i, QSCALE)
            elif op == "QK":
                ps[u] = qk(*u, tri, lfs.pop(u, None))
            elif op == "PV":
                ctxs[u] = pv(*u, ps.pop(u), NV, skew)
            else:
                I, a0 = divmod(2 * i, NC)
                c2 = jnp.concatenate([_cat([ctxs[I, e, c][a] for a in (a0, a0 + 1) for c in range(NC)], 0)
                                      for e in range(2)], axis=1).astype(bf16)
                acc_ref[_rows(i, TQ), :] += jnp.dot(c2, weight("o"), preferred_element_type=f32)
        return 0

    lax.fori_loop(0, NP - 1, step, 0)

    def last_head(e, _):
        tri = causal_tri()
        lfs, ps = {}, {}
        for op, I, c in _parse(LAST):
            if op == "LT":
                lfs[I, c] = left(I, e, c, 0)
            elif op == "QK":
                ps[I, c] = qk(I, e, c, tri, lfs.pop((I, c), None))
            else:
                for a, ca in enumerate(pv(I, e, c, ps.pop((I, c)), 0, None)):
                    r = (I * TB + 128 * a + GR * c) // 2
                    ctx_ref[e, r:r + GR // 2, :] = _pk(ca.astype(bf16))
        return 0

    lax.fori_loop(0, 2, last_head, 0)
    wwait("o", (NP - 1) & 1)
    rcopy.wait()
    for name in "kvq":
        wwait(name, NP & 1)
    fwait()
    wr = wr_ref[...].astype(f32).reshape(1, M)

    def out_block(i, dst):
        c2 = _upk(jnp.concatenate([ctx_ref[0, _rows(i, T2), :], ctx_ref[1, _rows(i, T2), :]], axis=1))
        wo = bo[(NP - 1) & 1].reshape(2 * D, M)
        y = dst[...] + jnp.dot(c2, wo, preferred_element_type=f32)
        dst[...] = _rb(y)
        return y

    def epi_block(i, src, top, y=None, maybe_pad=False):
        hh = src[...]
        s = jnp.sum(hh, axis=-1, keepdims=True)
        mrow = _rb(s * (1.0 / M))
        if y is not None:
            z = z_ref[...]
            parts = []
            for g in range(NG):
                t = g * PACE // NG
                yt = y[(t % NG) * 8:(t % NG + 1) * 8, (t // NG) * 256:(t // NG) * 256 + 128]
                mg = jnp.broadcast_to(mrow[g * 8:(g + 1) * 8], (8, 128))
                parts.append(pltpu.bitcast(pltpu.bitcast(mg, u32) | (pltpu.bitcast(yt, u32) & z), f32))
            mrow = jnp.concatenate(parts, axis=0)
        else:
            mrow = jnp.broadcast_to(mrow, (TQ, 128))
        d = hh - _wide(mrow)
        mu = _gather(s) * (1.0 / M)
        dm = mu - _rb(mu)
        var = _gather(jnp.sum(d * d, axis=-1, keepdims=True)) * (1.0 / M) - dm * dm
        sw = _gather(jnp.sum(d * wr, axis=-1, keepdims=True))
        ve = _rb(_rb(jnp.maximum(var, 0.0)) + EPS)
        inv = pl.reciprocal(_rb(ve * lax.rsqrt(ve)), approx=False, full_range=False)
        r = _rb(sw * inv)
        inv_s = _scatter(inv, NG)
        off_s = mrow * inv_s
        stp_ref[0, _rows(i + 1, TQ), :] = inv_s
        stp_ref[1, _rows(i + 1, TQ), :] = mrow
        op_ref[_rows(i + 1, TQ), :] = (hh * _wide(inv_s + 1.0) - _wide(off_s)).astype(bf16)
        if maybe_pad:
            @pl.when(i >= 0)
            def _():
                outcopy(i).start()
        else:
            outcopy(i).start()
        b = pltpu.bitcast(r + 0.0, i32)
        code = lax.shift_right_arithmetic(b ^ (lax.shift_right_arithmetic(b, 31) & jnp.int32(0x7FFF0000)), 5)
        lane = lax.broadcasted_iota(i32, (8, 128), 1)
        tok = i * TQ + lane * 8 + lax.broadcasted_iota(i32, (8, 128), 0)
        key = pltpu.bitcast(code + (jnp.int32(0x24000000 + S - 1) - tok), f32)
        key = jnp.where((lane < NG) & (tok >= 0) if maybe_pad else lane < NG, key, 0.0)
        return jnp.maximum(top[0], key), jnp.maximum(top[1], jnp.minimum(top[0], key))

    def out_epi(j, top):
        v = accp_ref.at[pl.ds(pl.multiple_of(j * (2 * TQ), TQ), 3 * TQ)]
        for t in range(2):
            y = out_block(2 * j + t, v.at[(t + 1) * TQ:(t + 2) * TQ])
            top = epi_block(2 * j + t - 1, v.at[t * TQ:(t + 1) * TQ], top, y, t == 0)
        return top

    lo = jnp.zeros((8, 128), f32)
    top = lax.fori_loop(0, NB // 2, out_epi, (lo, lo))
    t1, t2 = epi_block(NB - 1, acc_ref.at[_rows(NB - 1, TQ)], top)

    for sh in (4, 2, 1):
        u1, u2 = pltpu.roll(t1, sh, 0), pltpu.roll(t2, sh, 0)
        t1, t2 = jnp.maximum(t1, u1), jnp.maximum(jnp.maximum(t2, u2), jnp.minimum(t1, u1))
    lane = lax.broadcasted_iota(i32, (8, 128), 1)
    sub8 = lax.broadcasted_iota(i32, (8, 128), 0)
    bit = (lax.shift_right_logical(lane, sub8) & 1) == 1
    m0 = jnp.max(jnp.where(sub8 == 7, t2, jnp.where(bit, 0.0, t1)), axis=1, keepdims=True)
    m1 = jnp.max(jnp.where(sub8 == 7, t2, jnp.where(bit, t1, 0.0)), axis=1, keepdims=True)
    k1 = jnp.maximum(m0, m1)[0:1]
    k2 = jnp.max(jnp.minimum(m0, m1), axis=0, keepdims=True)
    i1 = (S - 1) - (pltpu.bitcast(k1, i32)[0, 0] & (S - 1))
    i2 = (S - 1) - (pltpu.bitcast(k2, i32)[0, 0] & (S - 1))
    g1 = pl.multiple_of(i1 & ~7, 8)
    g2 = pl.multiple_of(i2 & ~7, 8)

    def two(f):
        return jnp.concatenate([f(pl.ds(g1, 8)), f(pl.ds(g2, 8))], axis=0)

    hh = two(lambda r_: acc_ref[r_, :])
    hnb = (_rb(hh - _wide(two(lambda r_: st_ref[1, r_, :]))) * _wide(two(lambda r_: st_ref[0, r_, :]))).astype(bf16)
    hn = hnb.astype(f32)
    r = _rb(jnp.sum(hn * wr, axis=1, keepdims=True))
    sub = lax.broadcasted_iota(i32, (16, 1), 0)
    tok = jnp.where(sub < 8, g1 + sub, g2 + sub - 8)
    sel = (tok == i1) | (tok == i2)
    g = _rb(jnp.dot(hnb, wg_ref[...], preferred_element_type=f32))
    g = _rb(g * _rb(jax.nn.sigmoid(g)))
    u = _rb(jnp.dot(hnb, wu_ref[...], preferred_element_type=f32))
    y = _rb(jnp.dot((g * u).astype(bf16), wd_ref[:, 0:M], preferred_element_type=f32))
    y = _rb(y * _rb(jax.nn.sigmoid(r)))
    res = (hh + jnp.where(sel, _rb(hn + y), hn)).astype(bf16)
    for i in range(NB):
        outcopy(i).wait()
    o_ref[0:16, :] = res
    cp1 = pltpu.make_async_copy(o_ref.at[0:8], o_hbm.at[pl.ds(g1, 8)], outsem.at[0])
    cp1.start()

    @pl.when(g2 != g1)
    def _():
        cp2 = pltpu.make_async_copy(o_ref.at[8:16], o_hbm.at[pl.ds(g2, 8)], outsem.at[1])
        cp2.start()
        cp2.wait()

    cp1.wait()


@jax.jit
def pallas_sequential_preLN__compressed_kv_cla__moe_arch_mod__prompt_kernel(
    A_x: jax.Array,
    A_c_kv: jax.Array,
    A_w_q: jax.Array,
    A_w_uk: jax.Array,
    A_w_uv: jax.Array,
    A_w_o: jax.Array,
    B_x: jax.Array,
    B_w_r: jax.Array,
    B_w_gate: jax.Array,
    B_w_up: jax.Array,
    B_w_down: jax.Array,
):
    del B_x
    hbm = pl.BlockSpec(memory_space=pl.ANY)
    V = pltpu.VMEM
    DMA = pltpu.SemaphoreType.DMA
    out = pl.pallas_call(
        _kernel,
        in_specs=[hbm] * 10,
        out_specs=hbm,
        out_shape=jax.ShapeDtypeStruct((S, M), bf16),
        scratch_shapes=[
            V((S, M), bf16), V((S, DC), bf16),
            V((S // 2, DC), u32), V((S // 2, M), u32),
            V((S + TQ, M), f32), V((S + TQ, M), bf16),
            V((2, M // G, 2 * G, D), bf16), V((2, DC // G, 2 * G, D), bf16), V((2, DC // G, 2 * G, D), bf16),
            V((2, 2, D, M), bf16),
            V((2, S // 2, D), u32), V((2, S // 2, D), u32), V((2, S // 2, D), u32), V((2, S // 2, D), u32),
            V((M,), bf16), V((M, F), bf16), V((M, F), bf16),
            V((F, M + 128), bf16),
            V((2, S + TQ, 128), f32), V((8, 128), u32),
            DMA((4, 2)), DMA((NB,)), DMA((NB,)), DMA((4,)), DMA((NB,)),
        ],
        compiler_params=pltpu.CompilerParams(vmem_limit_bytes=120 * 1024 * 1024,
                                             disable_bounds_checks=True,
                                             disable_semaphore_checks=True),
    )(A_x.reshape(S, M), A_c_kv.reshape(S, DC), A_w_q.reshape(M // G, G, H, D),
      A_w_uk.reshape(DC // G, G, H, D), A_w_uv.reshape(DC // G, G, H, D), A_w_o,
      B_w_r, B_w_gate, B_w_up, B_w_down)
    return out.reshape(1, S, M)
```

```python
import math

import jax
import jax.numpy as jnp
from jax import lax
from jax.experimental import pallas as pl
from jax.experimental.pallas import tpu as pltpu

S, M, H, D, DC, F = 2048, 1024, 32, 128, 512, 3584
EPS = 1e-5
EPS_BF16 = 1.0013580322265625e-05
bf16, f32, u32, i32 = jnp.bfloat16, jnp.float32, jnp.uint32, jnp.int32
NT = (((1,), (1,)), ((), ()))
G = 4
NP = H // 2
TQ = 256
NB = S // TQ
T2 = TQ // 2
NG = TQ // 8
FCH = 14
QSCALE = (D ** -0.5) * math.log2(math.e)
PACE = 72

NEG = -1e30
GR = 16
NC = 128 // GR
TB = 128 * NC
NV = 4
EXTRA = (0, 1, 4)
BS = 4

MID = ("LT105 LT106 QK107 LT104 QK106 QK105 QK104 LT101 LT103 LT102 QK103 QK102 PV107 QK101 LT100 LT116 "
       "QK100 PV105 PV106 LT115 QK117 QK115 LT114 QK116 PV102 LT113 QK114 PV103 LT112 PV101 PV104 LT111 "
       "PV100 QK113 PV115 LT110 QK112 PV117 QK111 LT006 QK110 PV116 LT005 QK007 KP7 QP7 LT003 PV114 LT004 "
       "QK006 QP6 KP6 QK005 PV112 LT001 LT002 QK003 QK004 PV113 KP5 QP5 PV110 PV111 QK002 QP4 PV007 QK001 "
       "KP4 VP7 PV006 VP6 LT000 LT016 QK000 PV005 QK017 LT015 QK016 PV004 VP5 PV002 LT014 QK015 PV003 LT012 "
       "QK014 OUT7 VP4 OUT6 LT013 QK013 PV000 LT010 QK012 PV001 LT011 OUT5 PV017 QK011 OUT4 QK010 KP1 PV015 "
       "QP3 PV012 PV013 PV016 PV014 PV010 PV011 QP1 KP2 OUT2 KP3 QP0 OUT3 QP2 VP2 OUT1 VP3 KP0 VP1 VP0 OUT0")
LAST = ("LT16 LT15 QK17 LT14 QK16 QK15 QK14 LT13 PV17 LT12 LT11 QK13 PV16 LT10 QK11 QK12 PV14 PV13 LT05 PV15 "
       "QK10 LT06 QK07 LT04 PV12 QK05 QK06 PV11 PV10 LT02 QK04 LT03 PV07 LT01 QK03 LT00 QK02 PV05 PV06 QK01 "
       "PV04 QK00 PV03 PV02 PV00 PV01")


def _parse(s):
    out = []
    for t in s.split():
        name = t.rstrip("0123456789")
        out.append((name,) + tuple(int(c) for c in t[len(name):]))
    return out


def _rb(x):
    return x.astype(bf16).astype(f32)


def _pk(x):
    return pltpu.bitcast(x, u32)


def _upk(x):
    return pltpu.bitcast(x, bf16)


def _gather(col):
    n = col.shape[0] // 8
    lane = lax.broadcasted_iota(i32, (8, 128), 1)
    vs = [jnp.broadcast_to(col[g * 8:(g + 1) * 8], (8, 128)) for g in range(n)]
    bit = 1
    while len(vs) > 1:
        m = (lane & bit) != 0
        vs = [jnp.where(m, vs[2 * k + 1], vs[2 * k]) for k in range(len(vs) // 2)]
        bit *= 2
    return vs[0]


def _scatter(dense, n):
    return jnp.concatenate([jnp.broadcast_to(dense[:, g:g + 1], (8, 128)) for g in range(n)], axis=0)


def _wide(v):
    return jnp.concatenate([v] * (M // 128), axis=1)


def _unpack_pair(buf):
    k = buf.shape[0] * G
    w = pltpu.bitcast(buf.reshape(2 * k, D), u32)
    w2 = jnp.concatenate([w << 16, w & jnp.uint32(0xFFFF0000)], axis=1)
    return pltpu.bitcast(w2, f32).astype(bf16)


def _cat(parts, axis):
    return parts[0] if len(parts) == 1 else jnp.concatenate(parts, axis=axis)


def _rows(i, n, k=1):
    return pl.ds(i * n, k * n) if isinstance(i, int) else pl.ds(pl.multiple_of(i * n, n), k * n)


def _kernel(x_hbm, c_hbm, wq_hbm, wk_hbm, wv_hbm, wo_hbm, wr_hbm, wg_hbm, wu_hbm, wd_hbm, o_hbm,
            x_ref, c_ref, cp_ref, xn_ref, accp_ref, op_ref, bq, bk, bv, bo, q_ref, k_ref, v_ref, ctx_ref,
            wr_ref, wg_ref, wu_ref, wd_ref, stp_ref, z_ref, wsem, xsem, csem, fsem, outsem):
    acc_ref, o_ref, st_ref = accp_ref.at[TQ:], op_ref.at[TQ:], stp_ref.at[:, TQ:]

    wtab = {"k": (0, wk_hbm, bk), "v": (1, wv_hbm, bv), "q": (2, wq_hbm, bq), "o": (3, wo_hbm, bo)}

    def wstart(name, pair, slot):
        t, w, b = wtab[name]
        heads = _rows(pair, 2)
        if name == "o":
            pltpu.make_async_copy(w.at[heads], b.at[slot], wsem.at[t, slot]).start()
        else:
            for g in range(G):
                pltpu.make_async_copy(w.at[:, g, heads, :], b.at[slot, :, pl.ds(2 * g, 2), :],
                                      wsem.at[t, slot]).start()

    def wwait(name, slot):
        t, _, b = wtab[name]
        pltpu.make_async_copy(b.at[slot], b.at[slot], wsem.at[t, slot]).wait()

    def xcopy(i):
        return pltpu.make_async_copy(x_hbm.at[_rows(i, TQ)], x_ref.at[_rows(i, TQ)], xsem.at[i])

    def ccopy(i):
        return pltpu.make_async_copy(c_hbm.at[_rows(i, TQ)], c_ref.at[_rows(i, TQ)], csem.at[i])

    def outcopy(i):
        return pltpu.make_async_copy(o_ref.at[_rows(i, TQ)], o_hbm.at[_rows(i, TQ)], outsem.at[i])

    rcopy = pltpu.make_async_copy(wr_hbm, wr_ref, fsem.at[3])

    def fstart(j):
        cs = _rows(j, F // FCH)
        pltpu.make_async_copy(wg_hbm.at[:, cs], wg_ref.at[:, cs], fsem.at[0]).start()
        pltpu.make_async_copy(wu_hbm.at[:, cs], wu_ref.at[:, cs], fsem.at[1]).start()
        pltpu.make_async_copy(wd_hbm.at[cs, :], wd_ref.at[cs, 0:M], fsem.at[2]).start()

    def fwait():
        for t, r in enumerate((wg_ref, wu_ref, wd_ref.at[:, 0:M])):
            pltpu.make_async_copy(r, r, fsem.at[t]).wait()

    def proj(src, w, dst, i, scale=None):
        y = jnp.dot(_upk(src), w, preferred_element_type=f32)
        if scale is not None:
            y = y * scale
        for e in range(2):
            dst[e, _rows(i, src.shape[0]), :] = _pk(y[:, e * D:(e + 1) * D].astype(bf16))

    def pr(ref, e, lo, hi):
        return ref[e, lo // 2:hi // 2, :]

    def nt(a, b):
        return lax.dot_general(_upk(a), _upk(b), NT, preferred_element_type=f32)

    def iota2():
        return lax.broadcasted_iota(i32, (GR, 128), 0), lax.broadcasted_iota(i32, (GR, 128), 1)

    def causal_tri():
        row, col = iota2()
        return col <= row + (128 - GR)

    def qunit(I, e, c):
        return _cat([pr(q_ref, e, r, r + GR) for r in range(I * TB + GR * c, (I + 1) * TB, 128)], 0)

    def period(c):
        return 1 << (GR * (c + 1) - 1).bit_length()

    def left(I, e, c, nv):
        s = GR * (c + 1)
        per = period(c) if c < nv else 128
        st = nt(pr(k_ref, e, 0, s), qunit(I, e, c))
        pad = [jnp.full((per - s, 128), NEG, f32)] if per > s else []
        t = jnp.concatenate(([st] + pad) * (128 // per), axis=0).T
        if I == 0:
            row, col = iota2()
            t = jnp.concatenate([jnp.where((col & (per - 1)) <= row + GR * c, t[:GR], NEG), t[GR:]], axis=0)
        return t

    def qk(I, e, c, tri, lf):
        r0 = I * TB
        s = GR * (c + 1)
        q = qunit(I, e, c)
        if s == 128:
            mn = nt(q, pr(k_ref, e, 0, r0 + 128))
        else:
            mn = _cat([lf] + ([nt(q, pr(k_ref, e, s, r0 + s))] if r0 else []), 1)
        ex = [nt(q[x * GR // 2:], pr(k_ref, e, r0 + s + 128 * (x - 1), r0 + s + 128 * x)) for x in range(1, NC)]
        out = []
        for a in range(NC):
            sa = _cat([mn[a * GR:(a + 1) * GR]]
                      + [ex[x - 1][(a - x) * GR:(a - x + 1) * GR] for x in range(1, a + 1)], 1)
            w = sa.shape[1]
            if not (s < 128 and w == 128):
                sa = _cat(([sa[:, :w - 128]] if w > 128 else []) + [jnp.where(tri, sa[:, w - 128:], NEG)], 1)
            out.append(jnp.exp2(sa - jnp.max(sa, axis=1, keepdims=True)))
        return out

    def skewed_v(e, off, per):
        w = _upk(pr(v_ref, e, off, off + per)).astype(f32)
        lane = lax.broadcasted_iota(i32, (per, 128), 1)
        bit = 1
        while bit < per:
            w = jnp.where((lane & bit) != 0, pltpu.roll(w, per - bit, 0), w)
            bit *= 2
        return [w[0:BS]] + [pltpu.roll(w[r // 8 * 8:r // 8 * 8 + 8], r, 1)[r % 8:r % 8 + BS]
                            for r in range(BS, per, BS)]

    def pv(I, e, c, p, nv, skew):
        r0 = I * TB
        s = GR * (c + 1)
        w0 = r0 + 128
        vpu = c < nv or (nv > 0 and (I, e, c) == EXTRA)
        if s == 128:
            vm = [pr(v_ref, e, 0, w0)]
        else:
            vm = ([] if vpu else [pr(v_ref, e, 0, 128)]) + ([pr(v_ref, e, s, r0 + s)] if r0 else [])
        cs = [None] * NC
        if vm:
            pm = _cat([pa[:, 128 * vpu:w0] for pa in p], 0).astype(bf16)
            ctx = jnp.dot(pm, _upk(_cat(vm, 0)), preferred_element_type=f32)
            cs = [ctx[a * GR:(a + 1) * GR] for a in range(NC)]
        if vpu:
            pl0 = _cat([pa[:, :128] for pa in p], 0)
            lane = lax.broadcasted_iota(i32, (128, 128), 1)
            parts = []
            for off, per in [(0, period(c))] if c < nv else [(0, 64), (64, 16)]:
                if c < nv:
                    x = pl0
                elif off == 0:
                    x = jnp.where(lane < 64, pl0, pltpu.roll(pl0, 64, 1))
                else:
                    x = jnp.where(lane >= off, pl0, 0.0)
                    for n in (16, 32, 64):
                        x = x + pltpu.roll(x, n, 1)
                if (e, off, per) not in skew:
                    skew[e, off, per] = skewed_v(e, off, per)
                parts.append(([x] + [pltpu.roll(x, 128 - b, 1) for b in range(1, BS)], skew[e, off, per]))
            acc = None
            for a in reversed(range(len(parts[0][1]))):
                if acc is not None:
                    acc = pltpu.roll(acc, 128 - BS, 1)
                for baby, w in parts:
                    for b in range(BS if a < len(w) else 0):
                        t = baby[b] * w[a][b:b + 1, :]
                        acc = t if acc is None else acc + t
            if c < nv:
                once = iota2()[1] < s
                p = [_cat([jnp.where(once, pa[:, :128], 0.0)] + ([pa[:, 128:]] if pa.shape[1] > 128 else []), 1)
                     for pa in p]
        den = [jnp.sum(pa.astype(bf16).astype(f32), axis=1, keepdims=True) for pa in p]
        for x in range(1, NC):
            px = _cat([p[a][:, w0 + 128 * (x - 1):w0 + 128 * x] for a in range(x, NC)], 0).astype(bf16)
            cx = jnp.dot(px, _upk(pr(v_ref, e, r0 + s + 128 * (x - 1), r0 + s + 128 * x)),
                         preferred_element_type=f32)
            for a in range(x, NC):
                t = cx[(a - x) * GR:(a - x + 1) * GR]
                cs[a] = t if cs[a] is None else cs[a] + t
        if vpu:
            cs = [acc[a * GR:(a + 1) * GR] if cs[a] is None else cs[a] + acc[a * GR:(a + 1) * GR]
                  for a in range(NC)]
        return [cs[a] * pl.reciprocal(den[a], approx=False, full_range=False) for a in range(NC)]

    def issue(n, f):
        def body(i, _):
            f(i)
            return 0

        lax.fori_loop(0, n, body, 0)

    HB = NB // 2
    wstart("k", 0, 0)
    wstart("v", 0, 0)
    issue(HB, lambda i: ccopy(i).start())
    wstart("q", 0, 0)
    issue(HB, lambda t: (ccopy(HB + t).start(), xcopy(2 * t).start(), xcopy(2 * t + 1).start()))
    wstart("o", 0, 0)
    for name in "kvq":
        wstart(name, 1, 1)
    rcopy.start()
    z_ref[...] = jnp.zeros((8, 128), u32)

    def zero_pad(i):
        accp_ref[_rows(i, 32), :] = jnp.zeros((32, M), f32)

    issue(TQ // 32, zero_pad)
    wwait("k", 0)
    wk0 = _unpack_pair(bk[0])
    wwait("v", 0)
    wv0 = _unpack_pair(bv[0])

    def pack_c(i):
        cpk = _pk(c_ref[_rows(i, TQ), :])
        cp_ref[_rows(i, T2), :] = cpk
        return cpk

    def ln_block(i):
        xf = x_ref[_rows(i, TQ), :].astype(f32)
        acc_ref[_rows(i, TQ), :] = xf
        d = xf - jnp.sum(xf, axis=-1, keepdims=True) * (1.0 / M)
        inv = lax.rsqrt(jnp.sum(d * d, axis=-1, keepdims=True) * (1.0 / M) + EPS)
        xnp = _pk((d * inv).astype(bf16))
        xn_ref[_rows(i, T2), :] = xnp
        return xnp

    def pro_a(i, _):
        ccopy(i).wait()
        cpk = pack_c(i)
        proj(cpk, wk0, k_ref, i)
        proj(cpk, wv0, v_ref, i)
        return 0

    lax.fori_loop(0, HB, pro_a, 0)
    wwait("q", 0)
    wq0 = _unpack_pair(bq[0])

    def pro_b(t, _):
        ccopy(HB + t).wait()
        xcopy(2 * t).wait()
        xcopy(2 * t + 1).wait()
        xs = [ln_block(2 * t), ln_block(2 * t + 1)]
        cpk = pack_c(HB + t)
        for j, (w, dst) in enumerate(((wk0, k_ref), (wv0, v_ref))):
            proj(cpk, w, dst, HB + t)
            for n in range(4):
                proj(xs[j][n * 32:(n + 1) * 32], wq0, q_ref, (2 * t + j) * 4 + n, QSCALE)
        return 0

    lax.fori_loop(0, HB, pro_b, 0)

    def step(p, _):
        s0 = p & 1
        s1 = 1 - s0
        for name in "kvq":
            wwait(name, s1)
        wwait("o", s0)
        ahead = jnp.minimum(p + 2, NP - 1)
        for name in "kvq":
            wstart(name, ahead, s0)
        wstart("o", p + 1, s1)

        @pl.when(p < FCH)
        def _():
            fstart(p)

        tri = causal_tri()
        w = {}

        def weight(name):
            if name not in w:
                b = wtab[name][2]
                w[name] = b[s0].reshape(2 * D, M) if name == "o" else _unpack_pair(b[s1])
            return w[name]

        lfs, ps, ctxs, skew = {}, {}, {}, {}
        for item in _parse(MID):
            op, i, u = item[0], item[1], item[1:]
            if op == "LT":
                lfs[u] = left(*u, NV)
            elif op == "KP":
                proj(cp_ref[_rows(i, T2), :], weight("k"), k_ref, i)
            elif op == "VP":
                proj(cp_ref[_rows(i, T2), :], weight("v"), v_ref, i)
            elif op == "QP":
                proj(xn_ref[_rows(i, T2), :], weight("q"), q_ref, i, QSCALE)
            elif op == "QK":
                ps[u] = qk(*u, tri, lfs.pop(u, None))
            elif op == "PV":
                ctxs[u] = pv(*u, ps.pop(u), NV, skew)
            else:
                I, a0 = divmod(2 * i, NC)
                c2 = jnp.concatenate([_cat([ctxs[I, e, c][a] for a in (a0, a0 + 1) for c in range(NC)], 0)
                                      for e in range(2)], axis=1).astype(bf16)
                acc_ref[_rows(i, TQ), :] += jnp.dot(c2, weight("o"), preferred_element_type=f32)
        return 0

    lax.fori_loop(0, NP - 1, step, 0)

    def last_head(e, _):
        tri = causal_tri()
        lfs, ps = {}, {}
        for op, I, c in _parse(LAST):
            if op == "LT":
                lfs[I, c] = left(I, e, c, 0)
            elif op == "QK":
                ps[I, c] = qk(I, e, c, tri, lfs.pop((I, c), None))
            else:
                for a, ca in enumerate(pv(I, e, c, ps.pop((I, c)), 0, None)):
                    r = (I * TB + 128 * a + GR * c) // 2
                    ctx_ref[e, r:r + GR // 2, :] = _pk(ca.astype(bf16))
        return 0

    lax.fori_loop(0, 2, last_head, 0)
    wwait("o", (NP - 1) & 1)
    rcopy.wait()
    for name in "kvq":
        wwait(name, NP & 1)
    fwait()
    wr = wr_ref[...].astype(f32).reshape(1, M)

    def out_block(i, dst):
        c2 = _upk(jnp.concatenate([ctx_ref[0, _rows(i, T2), :], ctx_ref[1, _rows(i, T2), :]], axis=1))
        wo = bo[(NP - 1) & 1].reshape(2 * D, M)
        y = dst[...] + jnp.dot(c2, wo, preferred_element_type=f32)
        dst[...] = _rb(y)
        return y

    def epi_block(i, src, top, y=None, maybe_pad=False):
        hh = src[...]
        s = jnp.sum(hh, axis=-1, keepdims=True)
        mrow = _rb(s * (1.0 / M))
        if y is not None:
            z = z_ref[...]
            parts = []
            for g in range(NG):
                t = g * PACE // NG
                yt = y[(t % NG) * 8:(t % NG + 1) * 8, (t // NG) * 256:(t // NG) * 256 + 128]
                mg = jnp.broadcast_to(mrow[g * 8:(g + 1) * 8], (8, 128))
                parts.append(pltpu.bitcast(pltpu.bitcast(mg, u32) | (pltpu.bitcast(yt, u32) & z), f32))
            mrow = jnp.concatenate(parts, axis=0)
        else:
            mrow = jnp.broadcast_to(mrow, (TQ, 128))
        d = hh - _wide(mrow)
        mu = _gather(s) * (1.0 / M)
        dm = mu - _rb(mu)
        var = _gather(jnp.sum(d * d, axis=-1, keepdims=True)) * (1.0 / M) - dm * dm
        sw = _gather(jnp.sum(d * wr, axis=-1, keepdims=True))
        ve = _rb(_rb(jnp.maximum(var, 0.0)) + EPS_BF16)
        inv = pl.reciprocal(_rb(ve * lax.rsqrt(ve)), approx=False, full_range=False)
        r = _rb(sw * inv)
        inv_s = _scatter(inv, NG)
        off_s = mrow * inv_s
        stp_ref[0, _rows(i + 1, TQ), :] = inv_s
        stp_ref[1, _rows(i + 1, TQ), :] = mrow
        op_ref[_rows(i + 1, TQ), :] = (hh * _wide(inv_s + 1.0) - _wide(off_s)).astype(bf16)
        if maybe_pad:
            @pl.when(i >= 0)
            def _():
                outcopy(i).start()
        else:
            outcopy(i).start()
        b = pltpu.bitcast(r + 0.0, i32)
        code = lax.shift_right_arithmetic(b ^ (lax.shift_right_arithmetic(b, 31) & jnp.int32(0x7FFF0000)), 5)
        lane = lax.broadcasted_iota(i32, (8, 128), 1)
        tok = i * TQ + lane * 8 + lax.broadcasted_iota(i32, (8, 128), 0)
        key = pltpu.bitcast(code + (jnp.int32(0x24000000 + S - 1) - tok), f32)
        key = jnp.where((lane < NG) & (tok >= 0) if maybe_pad else lane < NG, key, 0.0)
        return jnp.maximum(top[0], key), jnp.maximum(top[1], jnp.minimum(top[0], key))

    def out_epi(j, top):
        v = accp_ref.at[pl.ds(pl.multiple_of(j * (2 * TQ), TQ), 3 * TQ)]
        for t in range(2):
            y = out_block(2 * j + t, v.at[(t + 1) * TQ:(t + 2) * TQ])
            top = epi_block(2 * j + t - 1, v.at[t * TQ:(t + 1) * TQ], top, y, t == 0)
        return top

    lo = jnp.zeros((8, 128), f32)
    top = lax.fori_loop(0, NB // 2, out_epi, (lo, lo))
    t1, t2 = epi_block(NB - 1, acc_ref.at[_rows(NB - 1, TQ)], top)

    for sh in (4, 2, 1):
        u1, u2 = pltpu.roll(t1, sh, 0), pltpu.roll(t2, sh, 0)
        t1, t2 = jnp.maximum(t1, u1), jnp.maximum(jnp.maximum(t2, u2), jnp.minimum(t1, u1))
    lane = lax.broadcasted_iota(i32, (8, 128), 1)
    sub8 = lax.broadcasted_iota(i32, (8, 128), 0)
    bit = (lax.shift_right_logical(lane, sub8) & 1) == 1
    m0 = jnp.max(jnp.where(sub8 == 7, t2, jnp.where(bit, 0.0, t1)), axis=1, keepdims=True)
    m1 = jnp.max(jnp.where(sub8 == 7, t2, jnp.where(bit, t1, 0.0)), axis=1, keepdims=True)
    k1 = jnp.maximum(m0, m1)[0:1]
    k2 = jnp.max(jnp.minimum(m0, m1), axis=0, keepdims=True)
    i1 = (S - 1) - (pltpu.bitcast(k1, i32)[0, 0] & (S - 1))
    i2 = (S - 1) - (pltpu.bitcast(k2, i32)[0, 0] & (S - 1))
    g1 = pl.multiple_of(i1 & ~7, 8)
    g2 = pl.multiple_of(i2 & ~7, 8)

    def two(f):
        return jnp.concatenate([f(pl.ds(g1, 8)), f(pl.ds(g2, 8))], axis=0)

    hh = two(lambda r_: acc_ref[r_, :])
    hnb = (_rb(hh - _wide(two(lambda r_: st_ref[1, r_, :]))) * _wide(two(lambda r_: st_ref[0, r_, :]))).astype(bf16)
    hn = hnb.astype(f32)
    r = _rb(jnp.sum(hn * wr, axis=1, keepdims=True))
    sub = lax.broadcasted_iota(i32, (16, 1), 0)
    tok = jnp.where(sub < 8, g1 + sub, g2 + sub - 8)
    sel = (tok == i1) | (tok == i2)
    g = _rb(jnp.dot(hnb, wg_ref[...], preferred_element_type=f32))
    g = _rb(g * _rb(jax.nn.sigmoid(g)))
    u = _rb(jnp.dot(hnb, wu_ref[...], preferred_element_type=f32))
    y = _rb(jnp.dot((g * u).astype(bf16), wd_ref[:, 0:M], preferred_element_type=f32))
    y = _rb(y * _rb(jax.nn.sigmoid(r)))
    res = (hh + jnp.where(sel, _rb(hn + y), hn)).astype(bf16)
    for i in range(NB):
        outcopy(i).wait()
    o_ref[0:16, :] = res
    cp1 = pltpu.make_async_copy(o_ref.at[0:8], o_hbm.at[pl.ds(g1, 8)], outsem.at[0])
    cp1.start()

    @pl.when(g2 != g1)
    def _():
        cp2 = pltpu.make_async_copy(o_ref.at[8:16], o_hbm.at[pl.ds(g2, 8)], outsem.at[1])
        cp2.start()
        cp2.wait()

    cp1.wait()


@jax.jit
def pallas_sequential_preLN__compressed_kv_cla__moe_arch_mod__prompt_kernel(
    A_x: jax.Array,
    A_c_kv: jax.Array,
    A_w_q: jax.Array,
    A_w_uk: jax.Array,
    A_w_uv: jax.Array,
    A_w_o: jax.Array,
    B_x: jax.Array,
    B_w_r: jax.Array,
    B_w_gate: jax.Array,
    B_w_up: jax.Array,
    B_w_down: jax.Array,
):
    del B_x
    hbm = pl.BlockSpec(memory_space=pl.ANY)
    V = pltpu.VMEM
    DMA = pltpu.SemaphoreType.DMA
    out = pl.pallas_call(
        _kernel,
        in_specs=[hbm] * 10,
        out_specs=hbm,
        out_shape=jax.ShapeDtypeStruct((S, M), bf16),
        scratch_shapes=[
            V((S, M), bf16), V((S, DC), bf16),
            V((S // 2, DC), u32), V((S // 2, M), u32),
            V((S + TQ, M), f32), V((S + TQ, M), bf16),
            V((2, M // G, 2 * G, D), bf16), V((2, DC // G, 2 * G, D), bf16), V((2, DC // G, 2 * G, D), bf16),
            V((2, 2, D, M), bf16),
            V((2, S // 2, D), u32), V((2, S // 2, D), u32), V((2, S // 2, D), u32), V((2, S // 2, D), u32),
            V((M,), bf16), V((M, F), bf16), V((M, F), bf16),
            V((F, M + 128), bf16),
            V((2, S + TQ, 128), f32), V((8, 128), u32),
            DMA((4, 2)), DMA((NB,)), DMA((NB,)), DMA((4,)), DMA((NB,)),
        ],
        compiler_params=pltpu.CompilerParams(vmem_limit_bytes=120 * 1024 * 1024,
                                             disable_bounds_checks=True,
                                             disable_semaphore_checks=True),
    )(A_x.reshape(S, M), A_c_kv.reshape(S, DC), A_w_q.reshape(M // G, G, H, D),
      A_w_uk.reshape(DC // G, G, H, D), A_w_uv.reshape(DC // G, G, H, D), A_w_o,
      B_w_r, B_w_gate, B_w_up, B_w_down)
    return out.reshape(1, S, M)
```

```python
import math

import jax
import jax.numpy as jnp
from jax import lax
from jax.experimental import pallas as pl
from jax.experimental.pallas import tpu as pltpu

S, M, H, D, DC, F = 2048, 1024, 32, 128, 512, 3584
EPS = 1e-5
EPS_BF16 = 1.0013580322265625e-05
bf16, f32, u32, i32 = jnp.bfloat16, jnp.float32, jnp.uint32, jnp.int32
NT = (((1,), (1,)), ((), ()))
G = 4
NP = H // 2
TQ = 256
NB = S // TQ
T2 = TQ // 2
NG = TQ // 8
FCH = 14
QSCALE = (D ** -0.5) * math.log2(math.e)
PACE = 72

NEG = -1e30
GR = 16
NC = 128 // GR
TB = 128 * NC
NV = 4
EXTRA = (0, 1, 4)
BS = 4

MID = ("LT105 LT106 QK107 LT104 QK104 QK106 QK105 LT101 LT103 LT102 QK103 QK102 PV107 QK101 LT100 LT116 "
       "QK100 PV105 PV106 LT115 QK117 QK115 LT114 QK116 PV102 QK114 PV103 LT112 PV104 LT111 PV100 LT113 "
       "PV101 QK113 PV115 LT110 QK112 PV117 QK111 LT006 QK110 PV116 LT005 QK007 KP7 QP7 LT003 PV114 LT004 "
       "QK006 QP6 KP6 QK005 PV112 LT001 QK003 LT002 QK004 PV113 KP5 QP5 PV110 PV111 QK002 QP4 PV007 QK001 "
       "KP4 VP7 PV006 VP6 LT000 LT016 QK000 PV005 QK017 PV004 LT015 QK016 VP5 PV002 LT014 QK015 PV003 LT012 "
       "QK014 OUT7 VP4 OUT6 LT013 QK013 PV000 LT010 QK012 PV001 LT011 OUT5 PV017 QK011 OUT4 QK010 KP1 PV015 "
       "QP3 PV012 PV013 PV016 PV014 PV010 PV011 QP1 KP2 OUT2 QP2 KP3 VP2 QP0 VP1 OUT3 OUT1 VP0 KP0 VP3 OUT0")
LAST = ("LT16 LT15 QK17 LT14 QK16 QK15 QK14 LT13 PV17 LT12 LT11 QK13 PV16 LT10 QK11 QK12 PV14 PV13 LT05 PV15 "
       "QK10 LT06 QK07 LT04 PV12 QK05 QK06 PV11 PV10 LT02 QK04 LT03 PV07 LT01 QK03 LT00 QK02 PV05 PV06 QK01 "
       "PV04 QK00 PV03 PV02 PV00 PV01")


def _parse(s):
    out = []
    for t in s.split():
        name = t.rstrip("0123456789")
        out.append((name,) + tuple(int(c) for c in t[len(name):]))
    return out


def _rb(x):
    return x.astype(bf16).astype(f32)


def _pk(x):
    return pltpu.bitcast(x, u32)


def _upk(x):
    return pltpu.bitcast(x, bf16)


def _gather(col):
    n = col.shape[0] // 8
    lane = lax.broadcasted_iota(i32, (8, 128), 1)
    vs = [jnp.broadcast_to(col[g * 8:(g + 1) * 8], (8, 128)) for g in range(n)]
    bit = 1
    while len(vs) > 1:
        m = (lane & bit) != 0
        vs = [jnp.where(m, vs[2 * k + 1], vs[2 * k]) for k in range(len(vs) // 2)]
        bit *= 2
    return vs[0]


def _scatter(dense, n):
    return jnp.concatenate([jnp.broadcast_to(dense[:, g:g + 1], (8, 128)) for g in range(n)], axis=0)


def _wide(v):
    return jnp.concatenate([v] * (M // 128), axis=1)


def _unpack_pair(buf):
    k = buf.shape[0] * G
    w = pltpu.bitcast(buf.reshape(2 * k, D), u32)
    w2 = jnp.concatenate([w << 16, w & jnp.uint32(0xFFFF0000)], axis=1)
    return pltpu.bitcast(w2, f32).astype(bf16)


def _cat(parts, axis):
    return parts[0] if len(parts) == 1 else jnp.concatenate(parts, axis=axis)


def _rows(i, n, k=1):
    return pl.ds(i * n, k * n) if isinstance(i, int) else pl.ds(pl.multiple_of(i * n, n), k * n)


def _kernel(x_hbm, c_hbm, wq_hbm, wk_hbm, wv_hbm, wo_hbm, wr_hbm, wg_hbm, wu_hbm, wd_hbm, o_hbm,
            x_ref, c_ref, cp_ref, xn_ref, accp_ref, op_ref, bq, bk, bv, bo, q_ref, k_ref, v_ref, ctx_ref,
            wr_ref, wg_ref, wu_ref, wd_ref, stp_ref, z_ref, wsem, xsem, csem, fsem, outsem):
    acc_ref, o_ref, st_ref = accp_ref.at[TQ:], op_ref.at[TQ:], stp_ref.at[:, TQ:]

    wtab = {"k": (0, wk_hbm, bk), "v": (1, wv_hbm, bv), "q": (2, wq_hbm, bq), "o": (3, wo_hbm, bo)}

    def wstart(name, pair, slot):
        t, w, b = wtab[name]
        heads = _rows(pair, 2)
        if name == "o":
            pltpu.make_async_copy(w.at[heads], b.at[slot], wsem.at[t, slot]).start()
        else:
            for g in range(G):
                pltpu.make_async_copy(w.at[:, g, heads, :], b.at[slot, :, pl.ds(2 * g, 2), :],
                                      wsem.at[t, slot]).start()

    def wwait(name, slot):
        t, _, b = wtab[name]
        pltpu.make_async_copy(b.at[slot], b.at[slot], wsem.at[t, slot]).wait()

    def xcopy(i):
        return pltpu.make_async_copy(x_hbm.at[_rows(i, TQ)], x_ref.at[_rows(i, TQ)], xsem.at[i])

    def ccopy(i):
        return pltpu.make_async_copy(c_hbm.at[_rows(i, TQ)], c_ref.at[_rows(i, TQ)], csem.at[i])

    def outcopy(i):
        return pltpu.make_async_copy(o_ref.at[_rows(i, TQ)], o_hbm.at[_rows(i, TQ)], outsem.at[i])

    rcopy = pltpu.make_async_copy(wr_hbm, wr_ref, fsem.at[3])

    def fstart(j):
        cs = _rows(j, F // FCH)
        pltpu.make_async_copy(wg_hbm.at[:, cs], wg_ref.at[:, cs], fsem.at[0]).start()
        pltpu.make_async_copy(wu_hbm.at[:, cs], wu_ref.at[:, cs], fsem.at[1]).start()
        pltpu.make_async_copy(wd_hbm.at[cs, :], wd_ref.at[cs, 0:M], fsem.at[2]).start()

    def fwait():
        for t, r in enumerate((wg_ref, wu_ref, wd_ref.at[:, 0:M])):
            pltpu.make_async_copy(r, r, fsem.at[t]).wait()

    def proj(src, w, dst, i, scale=None):
        y = jnp.dot(_upk(src), w, preferred_element_type=f32)
        if scale is not None:
            y = y * scale
        for e in range(2):
            dst[e, _rows(i, src.shape[0]), :] = _pk(y[:, e * D:(e + 1) * D].astype(bf16))

    def pr(ref, e, lo, hi):
        return ref[e, lo // 2:hi // 2, :]

    def nt(a, b):
        return lax.dot_general(_upk(a), _upk(b), NT, preferred_element_type=f32)

    def iota2():
        return lax.broadcasted_iota(i32, (GR, 128), 0), lax.broadcasted_iota(i32, (GR, 128), 1)

    def causal_tri():
        row, col = iota2()
        return col <= row + (128 - GR)

    def qunit(I, e, c):
        return _cat([pr(q_ref, e, r, r + GR) for r in range(I * TB + GR * c, (I + 1) * TB, 128)], 0)

    def period(c):
        return 1 << (GR * (c + 1) - 1).bit_length()

    def left(I, e, c, nv):
        s = GR * (c + 1)
        per = period(c) if c < nv else 128
        st = nt(pr(k_ref, e, 0, s), qunit(I, e, c))
        pad = [jnp.full((per - s, 128), NEG, f32)] if per > s else []
        t = jnp.concatenate(([st] + pad) * (128 // per), axis=0).T
        if I == 0:
            row, col = iota2()
            t = jnp.concatenate([jnp.where((col & (per - 1)) <= row + GR * c, t[:GR], NEG), t[GR:]], axis=0)
        return t

    def qk(I, e, c, tri, lf):
        r0 = I * TB
        s = GR * (c + 1)
        q = qunit(I, e, c)
        if s == 128:
            mn = nt(q, pr(k_ref, e, 0, r0 + 128))
        else:
            mn = _cat([lf] + ([nt(q, pr(k_ref, e, s, r0 + s))] if r0 else []), 1)
        ex = [nt(q[x * GR // 2:], pr(k_ref, e, r0 + s + 128 * (x - 1), r0 + s + 128 * x)) for x in range(1, NC)]
        out = []
        for a in range(NC):
            sa = _cat([mn[a * GR:(a + 1) * GR]]
                      + [ex[x - 1][(a - x) * GR:(a - x + 1) * GR] for x in range(1, a + 1)], 1)
            w = sa.shape[1]
            if not (s < 128 and w == 128):
                sa = _cat(([sa[:, :w - 128]] if w > 128 else []) + [jnp.where(tri, sa[:, w - 128:], NEG)], 1)
            out.append(jnp.exp2(sa - jnp.max(sa, axis=1, keepdims=True)))
        return out

    def skewed_v(e, off, per):
        w = _upk(pr(v_ref, e, off, off + per)).astype(f32)
        lane = lax.broadcasted_iota(i32, (per, 128), 1)
        bit = 1
        while bit < per:
            w = jnp.where((lane & bit) != 0, pltpu.roll(w, per - bit, 0), w)
            bit *= 2
        return [w[0:BS]] + [pltpu.roll(w[r // 8 * 8:r // 8 * 8 + 8], r, 1)[r % 8:r % 8 + BS]
                            for r in range(BS, per, BS)]

    def pv(I, e, c, p, nv, skew):
        r0 = I * TB
        s = GR * (c + 1)
        w0 = r0 + 128
        vpu = c < nv or (nv > 0 and (I, e, c) == EXTRA)
        if s == 128:
            vm = [pr(v_ref, e, 0, w0)]
        else:
            vm = ([] if vpu else [pr(v_ref, e, 0, 128)]) + ([pr(v_ref, e, s, r0 + s)] if r0 else [])
        cs = [None] * NC
        if vm:
            pm = _cat([pa[:, 128 * vpu:w0] for pa in p], 0).astype(bf16)
            ctx = jnp.dot(pm, _upk(_cat(vm, 0)), preferred_element_type=f32)
            cs = [ctx[a * GR:(a + 1) * GR] for a in range(NC)]
        if vpu:
            pl0 = _cat([pa[:, :128] for pa in p], 0)
            lane = lax.broadcasted_iota(i32, (128, 128), 1)
            parts = []
            for off, per in [(0, period(c))] if c < nv else [(0, 64), (64, 16)]:
                if c < nv:
                    x = pl0
                elif off == 0:
                    x = jnp.where(lane < 64, pl0, pltpu.roll(pl0, 64, 1))
                else:
                    x = jnp.where(lane >= off, pl0, 0.0)
                    for n in (16, 32, 64):
                        x = x + pltpu.roll(x, n, 1)
                if (e, off, per) not in skew:
                    skew[e, off, per] = skewed_v(e, off, per)
                parts.append(([x] + [pltpu.roll(x, 128 - b, 1) for b in range(1, BS)], skew[e, off, per]))
            acc = None
            for a in reversed(range(len(parts[0][1]))):
                if acc is not None:
                    acc = pltpu.roll(acc, 128 - BS, 1)
                for baby, w in parts:
                    for b in range(BS if a < len(w) else 0):
                        t = baby[b] * w[a][b:b + 1, :]
                        acc = t if acc is None else acc + t
            if c < nv:
                once = iota2()[1] < s
                p = [_cat([jnp.where(once, pa[:, :128], 0.0)] + ([pa[:, 128:]] if pa.shape[1] > 128 else []), 1)
                     for pa in p]
        den = [jnp.sum(pa.astype(bf16).astype(f32), axis=1, keepdims=True) for pa in p]
        for x in range(1, NC):
            px = _cat([p[a][:, w0 + 128 * (x - 1):w0 + 128 * x] for a in range(x, NC)], 0).astype(bf16)
            cx = jnp.dot(px, _upk(pr(v_ref, e, r0 + s + 128 * (x - 1), r0 + s + 128 * x)),
                         preferred_element_type=f32)
            for a in range(x, NC):
                t = cx[(a - x) * GR:(a - x + 1) * GR]
                cs[a] = t if cs[a] is None else cs[a] + t
        if vpu:
            cs = [acc[a * GR:(a + 1) * GR] if cs[a] is None else cs[a] + acc[a * GR:(a + 1) * GR]
                  for a in range(NC)]
        return [cs[a] * pl.reciprocal(den[a], approx=False, full_range=False) for a in range(NC)]

    def issue(n, f):
        def body(i, _):
            f(i)
            return 0

        lax.fori_loop(0, n, body, 0)

    HB = NB // 2
    wstart("k", 0, 0)
    wstart("v", 0, 0)
    issue(HB, lambda i: ccopy(i).start())
    wstart("q", 0, 0)
    issue(HB, lambda t: (ccopy(HB + t).start(), xcopy(2 * t).start(), xcopy(2 * t + 1).start()))
    wstart("o", 0, 0)
    for name in "kvq":
        wstart(name, 1, 1)
    rcopy.start()
    z_ref[...] = jnp.zeros((8, 128), u32)

    def zero_pad(i):
        accp_ref[_rows(i, 32), :] = jnp.zeros((32, M), f32)

    issue(TQ // 32, zero_pad)
    wwait("k", 0)
    wk0 = _unpack_pair(bk[0])
    wwait("v", 0)
    wv0 = _unpack_pair(bv[0])

    def pack_c(i):
        cpk = _pk(c_ref[_rows(i, TQ), :])
        cp_ref[_rows(i, T2), :] = cpk
        return cpk

    def ln_block(i):
        xf = x_ref[_rows(i, TQ), :].astype(f32)
        acc_ref[_rows(i, TQ), :] = xf
        d = xf - jnp.sum(xf, axis=-1, keepdims=True) * (1.0 / M)
        inv = lax.rsqrt(jnp.sum(d * d, axis=-1, keepdims=True) * (1.0 / M) + EPS)
        xnp = _pk((d * inv).astype(bf16))
        xn_ref[_rows(i, T2), :] = xnp
        return xnp

    def pro_a(i, _):
        ccopy(i).wait()
        cpk = pack_c(i)
        proj(cpk, wk0, k_ref, i)
        proj(cpk, wv0, v_ref, i)
        return 0

    lax.fori_loop(0, HB, pro_a, 0)
    wwait("q", 0)
    wq0 = _unpack_pair(bq[0])

    def pro_b(t, _):
        ccopy(HB + t).wait()
        xcopy(2 * t).wait()
        xcopy(2 * t + 1).wait()
        xs = [ln_block(2 * t), ln_block(2 * t + 1)]
        cpk = pack_c(HB + t)
        for j, (w, dst) in enumerate(((wk0, k_ref), (wv0, v_ref))):
            proj(cpk, w, dst, HB + t)
            for n in range(4):
                proj(xs[j][n * 32:(n + 1) * 32], wq0, q_ref, (2 * t + j) * 4 + n, QSCALE)
        return 0

    lax.fori_loop(0, HB, pro_b, 0)

    def step(p, _):
        s0 = p & 1
        s1 = 1 - s0
        for name in "kvq":
            wwait(name, s1)
        wwait("o", s0)
        ahead = jnp.minimum(p + 2, NP - 1)
        for name in "kvq":
            wstart(name, ahead, s0)
        wstart("o", p + 1, s1)

        @pl.when(p < FCH)
        def _():
            fstart(p)

        tri = causal_tri()
        w = {}

        def weight(name):
            if name not in w:
                b = wtab[name][2]
                w[name] = b[s0].reshape(2 * D, M) if name == "o" else _unpack_pair(b[s1])
            return w[name]

        lfs, ps, ctxs, skew = {}, {}, {}, {}
        for item in _parse(MID):
            op, i, u = item[0], item[1], item[1:]
            if op == "LT":
                lfs[u] = left(*u, NV)
            elif op == "KP":
                proj(cp_ref[_rows(i, T2), :], weight("k"), k_ref, i)
            elif op == "VP":
                proj(cp_ref[_rows(i, T2), :], weight("v"), v_ref, i)
            elif op == "QP":
                proj(xn_ref[_rows(i, T2), :], weight("q"), q_ref, i, QSCALE)
            elif op == "QK":
                ps[u] = qk(*u, tri, lfs.pop(u, None))
            elif op == "PV":
                ctxs[u] = pv(*u, ps.pop(u), NV, skew)
            else:
                I, a0 = divmod(2 * i, NC)
                c2 = jnp.concatenate([_cat([ctxs[I, e, c][a] for a in (a0, a0 + 1) for c in range(NC)], 0)
                                      for e in range(2)], axis=1).astype(bf16)
                acc_ref[_rows(i, TQ), :] += jnp.dot(c2, weight("o"), preferred_element_type=f32)
        return 0

    lax.fori_loop(0, NP - 1, step, 0)

    def last_head(e, _):
        tri = causal_tri()
        lfs, ps = {}, {}
        for op, I, c in _parse(LAST):
            if op == "LT":
                lfs[I, c] = left(I, e, c, 0)
            elif op == "QK":
                ps[I, c] = qk(I, e, c, tri, lfs.pop((I, c), None))
            else:
                for a, ca in enumerate(pv(I, e, c, ps.pop((I, c)), 0, None)):
                    r = (I * TB + 128 * a + GR * c) // 2
                    ctx_ref[e, r:r + GR // 2, :] = _pk(ca.astype(bf16))
        return 0

    lax.fori_loop(0, 2, last_head, 0)
    wwait("o", (NP - 1) & 1)
    rcopy.wait()
    for name in "kvq":
        wwait(name, NP & 1)
    fwait()
    wr = wr_ref[...].astype(f32).reshape(1, M)

    def out_block(i, dst):
        c2 = _upk(jnp.concatenate([ctx_ref[0, _rows(i, T2), :], ctx_ref[1, _rows(i, T2), :]], axis=1))
        wo = bo[(NP - 1) & 1].reshape(2 * D, M)
        y = dst[...] + jnp.dot(c2, wo, preferred_element_type=f32)
        dst[...] = _rb(y)
        return y

    def epi_block(i, src, top, y=None, maybe_pad=False):
        hh = src[...]
        s = jnp.sum(hh, axis=-1, keepdims=True)
        mrow = _rb(s * (1.0 / M))
        if y is not None:
            z = z_ref[...]
            parts = []
            for g in range(NG):
                t = g * PACE // NG
                yt = y[(t % NG) * 8:(t % NG + 1) * 8, (t // NG) * 256:(t // NG) * 256 + 128]
                mg = jnp.broadcast_to(mrow[g * 8:(g + 1) * 8], (8, 128))
                parts.append(pltpu.bitcast(pltpu.bitcast(mg, u32) | (pltpu.bitcast(yt, u32) & z), f32))
            mrow = jnp.concatenate(parts, axis=0)
        else:
            mrow = jnp.broadcast_to(mrow, (TQ, 128))
        d = hh - _wide(mrow)
        mu = _gather(s) * (1.0 / M)
        dm = mu - _rb(mu)
        var = _gather(jnp.sum(d * d, axis=-1, keepdims=True)) * (1.0 / M) - dm * dm
        sw = _gather(jnp.sum(d * wr, axis=-1, keepdims=True))
        ve = _rb(_rb(jnp.maximum(var, 0.0)) + EPS_BF16)
        inv = pl.reciprocal(_rb(ve * lax.rsqrt(ve)), approx=False, full_range=False)
        r = _rb(sw * inv)
        inv_s = _scatter(inv, NG)
        off_s = mrow * inv_s
        stp_ref[0, _rows(i + 1, TQ), :] = inv_s
        stp_ref[1, _rows(i + 1, TQ), :] = mrow
        op_ref[_rows(i + 1, TQ), :] = (hh * _wide(inv_s + 1.0) - _wide(off_s)).astype(bf16)
        if maybe_pad:
            @pl.when(i >= 0)
            def _():
                outcopy(i).start()
        else:
            outcopy(i).start()
        b = pltpu.bitcast(r + 0.0, i32)
        code = lax.shift_right_arithmetic(b ^ (lax.shift_right_arithmetic(b, 31) & jnp.int32(0x7FFF0000)), 5)
        lane = lax.broadcasted_iota(i32, (8, 128), 1)
        tok = i * TQ + lane * 8 + lax.broadcasted_iota(i32, (8, 128), 0)
        key = pltpu.bitcast(code + (jnp.int32(0x24000000 + S - 1) - tok), f32)
        key = jnp.where((lane < NG) & (tok >= 0) if maybe_pad else lane < NG, key, 0.0)
        return jnp.maximum(top[0], key), jnp.maximum(top[1], jnp.minimum(top[0], key))

    def out_epi(j, top):
        v = accp_ref.at[pl.ds(pl.multiple_of(j * (2 * TQ), TQ), 3 * TQ)]
        for t in range(2):
            y = out_block(2 * j + t, v.at[(t + 1) * TQ:(t + 2) * TQ])
            top = epi_block(2 * j + t - 1, v.at[t * TQ:(t + 1) * TQ], top, y, t == 0)
        return top

    lo = jnp.zeros((8, 128), f32)
    top = lax.fori_loop(0, NB // 2, out_epi, (lo, lo))
    t1, t2 = epi_block(NB - 1, acc_ref.at[_rows(NB - 1, TQ)], top)

    for sh in (4, 2, 1):
        u1, u2 = pltpu.roll(t1, sh, 0), pltpu.roll(t2, sh, 0)
        t1, t2 = jnp.maximum(t1, u1), jnp.maximum(jnp.maximum(t2, u2), jnp.minimum(t1, u1))
    lane = lax.broadcasted_iota(i32, (8, 128), 1)
    sub8 = lax.broadcasted_iota(i32, (8, 128), 0)
    bit = (lax.shift_right_logical(lane, sub8) & 1) == 1
    m0 = jnp.max(jnp.where(sub8 == 7, t2, jnp.where(bit, 0.0, t1)), axis=1, keepdims=True)
    m1 = jnp.max(jnp.where(sub8 == 7, t2, jnp.where(bit, t1, 0.0)), axis=1, keepdims=True)
    k1 = jnp.maximum(m0, m1)[0:1]
    k2 = jnp.max(jnp.minimum(m0, m1), axis=0, keepdims=True)
    i1 = (S - 1) - (pltpu.bitcast(k1, i32)[0, 0] & (S - 1))
    i2 = (S - 1) - (pltpu.bitcast(k2, i32)[0, 0] & (S - 1))
    g1 = pl.multiple_of(i1 & ~7, 8)
    g2 = pl.multiple_of(i2 & ~7, 8)

    def two(f):
        return jnp.concatenate([f(pl.ds(g1, 8)), f(pl.ds(g2, 8))], axis=0)

    hh = two(lambda r_: acc_ref[r_, :])
    hnb = (_rb(hh - _wide(two(lambda r_: st_ref[1, r_, :]))) * _wide(two(lambda r_: st_ref[0, r_, :]))).astype(bf16)
    hn = hnb.astype(f32)
    r = _rb(jnp.sum(hn * wr, axis=1, keepdims=True))
    sub = lax.broadcasted_iota(i32, (16, 1), 0)
    tok = jnp.where(sub < 8, g1 + sub, g2 + sub - 8)
    sel = (tok == i1) | (tok == i2)
    g = _rb(jnp.dot(hnb, wg_ref[...], preferred_element_type=f32))
    g = _rb(g * _rb(jax.nn.sigmoid(g)))
    u = _rb(jnp.dot(hnb, wu_ref[...], preferred_element_type=f32))
    y = _rb(jnp.dot((g * u).astype(bf16), wd_ref[:, 0:M], preferred_element_type=f32))
    y = _rb(y * _rb(jax.nn.sigmoid(r)))
    res = (hh + jnp.where(sel, _rb(hn + y), hn)).astype(bf16)
    for i in range(NB):
        outcopy(i).wait()
    o_ref[0:16, :] = res
    cp1 = pltpu.make_async_copy(o_ref.at[0:8], o_hbm.at[pl.ds(g1, 8)], outsem.at[0])
    cp1.start()

    @pl.when(g2 != g1)
    def _():
        cp2 = pltpu.make_async_copy(o_ref.at[8:16], o_hbm.at[pl.ds(g2, 8)], outsem.at[1])
        cp2.start()
        cp2.wait()

    cp1.wait()


@jax.jit
def pallas_sequential_preLN__compressed_kv_cla__moe_arch_mod__prompt_kernel(
    A_x: jax.Array,
    A_c_kv: jax.Array,
    A_w_q: jax.Array,
    A_w_uk: jax.Array,
    A_w_uv: jax.Array,
    A_w_o: jax.Array,
    B_x: jax.Array,
    B_w_r: jax.Array,
    B_w_gate: jax.Array,
    B_w_up: jax.Array,
    B_w_down: jax.Array,
):
    del B_x
    hbm = pl.BlockSpec(memory_space=pl.ANY)
    V = pltpu.VMEM
    DMA = pltpu.SemaphoreType.DMA
    out = pl.pallas_call(
        _kernel,
        in_specs=[hbm] * 10,
        out_specs=hbm,
        out_shape=jax.ShapeDtypeStruct((S, M), bf16),
        scratch_shapes=[
            V((S, M), bf16), V((S, DC), bf16),
            V((S // 2, DC), u32), V((S // 2, M), u32),
            V((S + TQ, M), f32), V((S + TQ, M), bf16),
            V((2, M // G, 2 * G, D), bf16), V((2, DC // G, 2 * G, D), bf16), V((2, DC // G, 2 * G, D), bf16),
            V((2, 2, D, M), bf16),
            V((2, S // 2, D), u32), V((2, S // 2, D), u32), V((2, S // 2, D), u32), V((2, S // 2, D), u32),
            V((M,), bf16), V((M, F), bf16), V((M, F), bf16),
            V((F, M + 128), bf16),
            V((2, S + TQ, 128), f32), V((8, 128), u32),
            DMA((4, 2)), DMA((NB,)), DMA((NB,)), DMA((4,)), DMA((NB,)),
        ],
        compiler_params=pltpu.CompilerParams(vmem_limit_bytes=120 * 1024 * 1024,
                                             disable_bounds_checks=True,
                                             disable_semaphore_checks=True),
    )(A_x.reshape(S, M), A_c_kv.reshape(S, DC), A_w_q.reshape(M // G, G, H, D),
      A_w_uk.reshape(DC // G, G, H, D), A_w_uv.reshape(DC // G, G, H, D), A_w_o,
      B_w_r, B_w_gate, B_w_up, B_w_down)
    return out.reshape(1, S, M)
```
